```python
import jax
import jax.numpy as jnp

def _softmax(x, axis=-1):
    return jax.nn.softmax(x, axis=axis)
def _gelu(x):
    return jax.nn.gelu(x, approximate=True)
def _silu(x):
    return jax.nn.silu(x)
def _sigmoid(x):
    return jax.nn.sigmoid(x)
def _layernorm(x, axis=-1, eps=1e-5):
    m = jnp.mean(x, axis=axis, keepdims=True)
    v = jnp.var(x, axis=axis, keepdims=True)
    return (x - m) / jnp.sqrt(v + eps)
def _scatter_add(tgt, idx, src, axis=0):
    return tgt.at[idx].add(src)
def _segment_sum(src, seg, n):
    return jax.ops.segment_sum(src, seg, n)
class _Rng:
    def __init__(self, key):
        self._k = key
    def _next(self):
        self._k, sub = jax.random.split(self._k)
        return sub
    def normal(self, shape):
        return jax.random.normal(self._next(), shape, dtype=jnp.bfloat16)
    def randint(self, lo, hi, shape):
        return jax.random.randint(self._next(), shape, lo, hi, dtype=jnp.int32)
    def uniform(self, shape, lo=0.0, hi=1.0):
        return jax.random.uniform(self._next(), shape, jnp.bfloat16, lo, hi)
    def permutation(self, n):
        return jax.random.permutation(self._next(), n)


kernel_name = 'recurrent_scan__mha_block_cached__moe_arch_mod__prompt'

def setup_inputs():
    _rng = _Rng(jax.random.key(int.from_bytes(__import__("os").urandom(4), "little")))
    _w = (lambda a: (lambda t: t.astype(jnp.bfloat16) if jnp.issubdtype(t.dtype, jnp.floating) else t)(jnp.asarray(a)))
    def _A_setup():
        B, Sq, D = 1, 2048, 640
        H, Sk, Dh = 32, 2048, 128
        return {
            "x": _w((lambda *s: _rng.normal(s) * 0.05)(B, Sq, D)),
            "k_cache": _w((lambda *s: _rng.normal(s) * 0.05)(B, H, Sk, Dh)),
            "v_cache": _w((lambda *s: _rng.normal(s) * 0.05)(B, H, Sk, Dh)),
            "wq": _w((lambda *s: _rng.normal(s) * 0.05)(D, H * Dh) * (D ** -0.5)),
            "wo": _w((lambda *s: _rng.normal(s) * 0.05)(H * Dh, D) * ((H * Dh) ** -0.5)),
        }
    _A_in = _A_setup()

    def _B_setup():
        B, S, D, F, C = 1, 2048, 640, 1728, 8
        return {
            "x": _w((lambda *s: _rng.normal(s) * 0.05)(B, S, D)),
            "w_r": _w((lambda *s: _rng.normal(s) * 0.05)(D)),
            "w_gate": _w((lambda *s: _rng.normal(s) * 0.05)(D, F)),
            "w_up": _w((lambda *s: _rng.normal(s) * 0.05)(D, F)),
            "w_down": _w((lambda *s: _rng.normal(s) * 0.05)(F, D)),
        }
    _B_in = _B_setup()

    return {
        "A_x": _A_in["x"],
        "A_k_cache": _A_in["k_cache"],
        "A_v_cache": _A_in["v_cache"],
        "A_wq": _A_in["wq"],
        "A_wo": _A_in["wo"],
        "B_x": _B_in["x"],
        "B_w_r": _B_in["w_r"],
        "B_w_gate": _B_in["w_gate"],
        "B_w_up": _B_in["w_up"],
        "B_w_down": _B_in["w_down"],
    }

def reference(A_x, A_k_cache, A_v_cache, A_wq, A_wo, B_x, B_w_r, B_w_gate, B_w_up, B_w_down):
    def _A_ref(x, k_cache, v_cache, wq, wo):
        B, Sq, D = x.shape
        H, Dh = 32, 128
        q = (lambda x, *d: x.transpose(*d))((x @ wq).reshape(B, Sq, H, Dh), 0, 2, 1, 3)
        scores = jnp.einsum("bhqd,bhkd->bhqk", q, k_cache) * (Dh ** -0.5)
        p = _softmax(scores, axis=-1)
        o = jnp.einsum("bhqk,bhkd->bhqd", p, v_cache)
        return (lambda x, *d: x.transpose(*d))(o, 0, 2, 1, 3).reshape(B, Sq, H * Dh) @ wo

    def _B_ref(x, w_r, w_gate, w_up, w_down):
        B, S, D = x.shape
        C = 8
        r = x @ w_r
        idx = jnp.argsort(-r, axis=-1)[:, :C]
        idx_e = jnp.repeat(idx.reshape(B, C, 1), D, axis=2)
        x_sel = jnp.take_along_axis(x, idx_e, axis=1)
        g = _silu(x_sel @ w_gate)
        u = x_sel @ w_up
        y = (g * u) @ w_down
        r_sel = _sigmoid(jnp.take_along_axis(r, idx, axis=1))
        y = y * r_sel.reshape(B, C, 1)
        b_off = (jnp.arange(B) * S).reshape(B, 1)
        flat_idx = (idx + b_off).reshape(B * C)
        zero = (x * 0.0).reshape(B * S, D)
        upd = _scatter_add(zero, flat_idx, y.reshape(B * C, D), axis=0)
        return x + upd.reshape(B, S, D)

    x = A_x
    xn = _layernorm(x, axis=-1)
    s = _A_ref(xn, A_k_cache, A_v_cache, A_wq, A_wo)
    g = _silu(_B_ref(xn, B_w_r, B_w_gate, B_w_up, B_w_down))
    return x + s * g
```

```python
import functools
import math
import jax
import jax.numpy as jnp
from jax import lax
import jax.experimental.pallas as pl
import jax.experimental.pallas.tpu as pltpu

S, D, H, DH, F, C = 2048, 640, 32, 128, 1728, 8
TQ = 512
NS = 2
NP = 0
BF = jnp.bfloat16
F32 = jnp.float32
QSCALE = (DH ** -0.5) * math.log2(math.e)


def _rb(a):
    return a.astype(BF).astype(F32)


def _kernel(x_ref, k_ref, v_ref, wq_ref, wo_ref, wr_ref, wg_hbm, wu_hbm, wd_hbm,
            o_ref, xn_ref, acc_ref, q_ref, r_ref, wg_ref, wu_ref, wd_ref, sems, xnp_ref, z_ref, vt_ref, *bufs):
    s_refs = bufs[:NS]
    p_refs = bufs[NS:NS + NP]
    l_refs = bufs[NS + NP:]
    h = pl.program_id(0)

    def wcopies():
        return [pltpu.make_async_copy(wg_hbm, wg_ref, sems.at[0]),
                pltpu.make_async_copy(wu_hbm, wu_ref, sems.at[1]),
                pltpu.make_async_copy(wd_hbm, wd_ref, sems.at[2])]

    @pl.when(h == 0)
    def _():
        for c in wcopies():
            c.start()
        z_ref[0] = 0
        z_ref[1] = 0
        CH = 256
        def body(i, _):
            r0 = pl.multiple_of(i * CH, CH)
            x = x_ref[pl.ds(r0, CH), :].astype(F32)
            mf = jnp.mean(x, axis=-1, keepdims=True)
            xc = x - mf
            v = _rb(jnp.mean(xc * xc, axis=-1, keepdims=True))
            den = _rb(jnp.sqrt(_rb(v + 1e-5)))
            xn = (_rb(x - _rb(mf)) / den).astype(BF)
            xn_ref[pl.ds(r0, CH), :] = xn
            xnp_ref[pl.ds(pl.multiple_of(i * (CH // 2), CH // 2), CH // 2), :] = pltpu.bitcast(xn, jnp.uint32)
            acc_ref[pl.ds(r0, CH), :] = jnp.zeros((CH, D), F32)
            return 0
        lax.fori_loop(0, S // CH, body, 0)

    U32 = jnp.uint32
    NB = S // TQ
    NG = TQ // 128
    z1 = pl.multiple_of(z_ref[0], 8)
    z2 = pl.multiple_of(z_ref[1], 8)
    zvec = jnp.full((8, 128), z_ref[0], jnp.int32).astype(U32)

    def tok(a):
        return pltpu.bitcast(a, U32) & zvec

    def dep_bf(a, t):
        if t is None:
            return a
        au = pltpu.bitcast(a, U32)
        first = au[0:8, 0:128] | t
        top = first if au.shape[1] == 128 else jnp.concatenate([first, au[0:8, 128:]], axis=1)
        return pltpu.bitcast(jnp.concatenate([top, au[8:]], axis=0), BF)

    vt_ref[pl.ds(z1, DH // 2), :] = pltpu.bitcast(v_ref[...].T, U32)

    def qproj(i, t=None):
        xn = pltpu.bitcast(xnp_ref[i * TQ // 2:(i + 1) * TQ // 2, :], BF)
        xn = dep_bf(xn, t)
        return (jnp.dot(xn, wq_ref[...], preferred_element_type=F32) * QSCALE).astype(BF)

    SL = 512
    NSL = S // SL
    def qk(i, q):
        s_ref = s_refs[i % NS]
        ms = []
        for j in range(NSL):
            kj = k_ref[j * SL:(j + 1) * SL, :]
            if j >= 2:
                t = tok(ms[j - 2][:, 0:128])
                for g in range(1, NG):
                    t = t | tok(ms[j - 2][:, g * 128:(g + 1) * 128])
                kj = dep_bf(kj, t)
            sT = lax.dot_general(kj, q, (((1,), (1,)), ((), ())), preferred_element_type=F32)
            s_ref[pl.ds(z1 + j * SL, SL), :] = sT
            mj = jnp.max(jnp.max(sT.reshape(4, SL // 32, 8, TQ), axis=1), axis=0)
            if j > 0:
                mj = jnp.maximum(mj, ms[j - 1])
            ms.append(mj)
        def alltok(a):
            t = tok(a[:, 0:128])
            for g in range(1, NG):
                t = t | tok(a[:, g * 128:(g + 1) * 128])
            return t
        m = jnp.broadcast_to(jnp.max(ms[-1], axis=0, keepdims=True), (8, TQ))
        return m, alltok(ms[-2]), alltok(m)

    def pv(i, m):
        s_ref = s_refs[i % NS]
        os = []
        NT = S // 128
        for g in range(NG):
            mg = m[:, g * 128:(g + 1) * 128]
            ls = []
            ps = []
            for t in range(NT):
                mt = mg
                if t >= 2:
                    mt = pltpu.bitcast(pltpu.bitcast(mg, U32) | tok(ls[t - 2]), F32)
                s = s_ref[pl.ds(z2 + t * 128, 128), g * 128:(g + 1) * 128]
                p = jnp.exp2(s - jnp.concatenate([mt] * 16, axis=0))
                lt = jnp.sum(jnp.sum(p.reshape(2, 8, 8, 128), axis=1), axis=0)
                if t > 0:
                    lt = lt + ls[t - 1]
                ls.append(lt)
                ps.append(p)
            l = jnp.sum(ls[-1], axis=0, keepdims=True)
            vT = pltpu.bitcast(vt_ref[pl.ds(z2, DH // 2), :], BF)
            oT = jnp.dot(vT, jnp.concatenate(ps, axis=0).astype(BF), preferred_element_type=F32)
            oT = oT * (1.0 / l)
            os.append(oT.T.astype(BF))
        return jnp.concatenate(os, axis=0)

    def oproj(i, o, t=None):
        o = dep_bf(o, t)
        acc_ref[i * TQ:(i + 1) * TQ, :] += jnp.dot(o, wo_ref[...], preferred_element_type=F32)

    qs = {0: qproj(0)}
    os = {}
    for t in range(NB):
        m, t2, t3 = qk(t, qs[t])
        if t + 1 < NB:
            qs[t + 1] = qproj(t + 1, t2)
        if t >= 1:
            oproj(t - 1, os[t - 1], t3 if t + 1 < NB else t2)
        os[t] = pv(t, m)
    oproj(NB - 1, os[NB - 1])

    @pl.when(h == H - 1)
    def _():
        for c in wcopies():
            c.wait()
        wr = wr_ref[...]
        r = lax.dot_general(wr, xn_ref[...], (((1,), (1,)), ((), ())), preferred_element_type=F32)
        r = _rb(r)
        col = lax.broadcasted_iota(jnp.int32, (8, S), 1).astype(F32)
        row = lax.broadcasted_iota(jnp.int32, (8, S), 0)
        sel = jnp.zeros((8, S), F32)
        rsel = jnp.zeros((8, 1), F32)
        row1 = lax.broadcasted_iota(jnp.int32, (8, 1), 0)
        alive = jnp.ones((8, S), F32)
        rw = r
        for j in range(C):
            mx = jnp.max(rw, axis=-1, keepdims=True)
            cand = jnp.where((rw == mx) & (alive > 0), col, float(S))
            ix = jnp.min(cand, axis=-1, keepdims=True)
            hit = col == ix
            sel = jnp.where(hit & (row == j), 1.0, sel)
            rsel = jnp.where(row1 == j, mx, rsel)
            rw = jnp.where(hit, -jnp.inf, rw)
            alive = jnp.where(hit, 0.0, alive)
        selb = sel.astype(BF)
        xs = jnp.dot(selb, xn_ref[...], preferred_element_type=F32).astype(BF)
        g = _rb(lax.dot_general(xs, wg_ref[...], (((1,), (1,)), ((), ())), preferred_element_type=F32))
        g = _rb(g * jax.nn.sigmoid(g))
        u = _rb(lax.dot_general(xs, wu_ref[...], (((1,), (1,)), ((), ())), preferred_element_type=F32))
        y = _rb(jnp.dot((g * u).astype(BF), wd_ref[...], preferred_element_type=F32))
        y = (y * _rb(jax.nn.sigmoid(rsel))).astype(BF)
        r_ref[...] = sel
        CH = 256
        def body(i, _):
            r0 = pl.multiple_of(i * CH, CH)
            st = r_ref[:, pl.ds(r0, CH)].astype(BF)
            upd = lax.dot_general(st, y, (((0,), (0,)), ((), ())), preferred_element_type=F32)
            b = _rb(xn_ref[pl.ds(r0, CH), :].astype(F32) + upd)
            g = _rb(b * jax.nn.sigmoid(b))
            sacc = _rb(acc_ref[pl.ds(r0, CH), :])
            o_ref[pl.ds(r0, CH), :] = (x_ref[pl.ds(r0, CH), :].astype(F32) + _rb(sacc * g)).astype(BF)
            return 0
        lax.fori_loop(0, S // CH, body, 0)


@jax.jit
def pallas_recurrent_scan__mha_block_cached__moe_arch_mod__prompt_kernel(
    A_x, A_k_cache, A_v_cache, A_wq, A_wo, B_x, B_w_r, B_w_gate, B_w_up, B_w_down):
    x = A_x.reshape(S, D)
    k = A_k_cache.reshape(H, S, DH)
    v = A_v_cache.reshape(H, S, DH)
    wr = jnp.broadcast_to(B_w_r.reshape(1, D), (8, D))
    out = pl.pallas_call(
        _kernel,
        grid=(H,),
        in_specs=[
            pl.BlockSpec((S, D), lambda h: (0, 0)),
            pl.BlockSpec((None, S, DH), lambda h: (h, 0, 0)),
            pl.BlockSpec((None, S, DH), lambda h: (h, 0, 0)),
            pl.BlockSpec((D, DH), lambda h: (0, h)),
            pl.BlockSpec((DH, D), lambda h: (h, 0)),
            pl.BlockSpec((8, D), lambda h: (0, 0)),
            pl.BlockSpec(memory_space=pl.ANY),
            pl.BlockSpec(memory_space=pl.ANY),
            pl.BlockSpec(memory_space=pl.ANY),
        ],
        out_specs=pl.BlockSpec((S, D), lambda h: (0, 0)),
        out_shape=jax.ShapeDtypeStruct((S, D), BF),
        scratch_shapes=[
            pltpu.VMEM((S, D), BF),
            pltpu.VMEM((S, D), F32),
            pltpu.VMEM((S // 2, DH), jnp.uint32),
            pltpu.VMEM((8, S), F32),
            pltpu.VMEM((F, D), BF),
            pltpu.VMEM((F, D), BF),
            pltpu.VMEM((F, D), BF),
            pltpu.SemaphoreType.DMA((3,)),
            pltpu.VMEM((S // 2, D), jnp.uint32),
            pltpu.SMEM((2,), jnp.int32),
            pltpu.VMEM((DH // 2, S), jnp.uint32),
        ] + [pltpu.VMEM((S, TQ), F32)] * NS + [pltpu.VMEM((TQ // 2, S), jnp.uint32)] * NP + [pltpu.VMEM((TQ, 1), F32)] * NP,
        compiler_params=pltpu.CompilerParams(
            dimension_semantics=("arbitrary",),
            vmem_limit_bytes=126 * 1024 * 1024,
        ),
    )(x, k, v, A_wq, A_wo, wr, B_w_gate.T, B_w_up.T, B_w_down)
    return out.reshape(1, S, D)
```

```python
import math
import jax
import jax.numpy as jnp
from jax import lax
import jax.experimental.pallas as pl
import jax.experimental.pallas.tpu as pltpu

S, D, H, DH, F, C = 2048, 640, 32, 128, 1728, 8
TQ = 512
NB = S // TQ
NG = TQ // 128
BF = jnp.bfloat16
F32 = jnp.float32
U32 = jnp.uint32
QSCALE = (DH ** -0.5) * math.log2(math.e)
E = lambda k, d: d
PV_CT = 4
PV_DIST = E('PV_DIST', 3)
HPI = E('HPI', 1)
LNC = E('LNC', 32)
ATOK = (0, 0, 0, 0)
LN_DIST = E('LN_DIST', 2)
GROWS = 80 * HPI
FINH = E('FINH', 6)
DTOK = (128, 256, 384, 504)
NT = (((1,), (1,)), ((), ()))


def _rb(a):
    return a.astype(BF).astype(F32)


def _kernel(x_hbm, k_hbm, v_hbm, wq_hbm, wo_hbm, wr_ref, wg_hbm, wu_hbm, wd_hbm,
            o_hbm,
            x_ref, k_ref, v_ref, wq_ref, wo_ref, wg_ref, wu_ref, wd_ref,
            xn_ref, g_ref, acc_ref, qn_ref, vt_ref, xs_ref, rs_ref, rc_ref, out_ref, z_ref, idx_ref,
            s0_ref, s1_ref, ot_ref, lr_ref, sem):
    s_refs = (s0_ref, s1_ref)

    SEM_A, SEM_B, SEM_C, SEM_D, SEM_H, SEM_F, SEM_O = range(7)

    def cp_k(h, s=SEM_H):
        return pltpu.make_async_copy(k_hbm.at[h], k_ref.at[h], sem.at[s])

    def cp_v(h, s=SEM_H):
        return pltpu.make_async_copy(v_hbm.at[h], v_ref.at[h], sem.at[s])

    def cp_wq(h, s=SEM_H):
        off = h * DH if isinstance(h, int) else pl.multiple_of(h * DH, DH)
        return pltpu.make_async_copy(wq_hbm.at[:, pl.ds(off, DH)], wq_ref.at[h], sem.at[s])

    def cp_wo(h, s=SEM_H):
        return pltpu.make_async_copy(wo_hbm.at[h], wo_ref.at[h], sem.at[s])

    def cp_x(i, s):
        return pltpu.make_async_copy(x_hbm.at[pl.ds(i * TQ, TQ)], x_ref.at[pl.ds(i * TQ, TQ)], sem.at[s])

    cp_ffn = [pltpu.make_async_copy(wg_hbm, wg_ref, sem.at[SEM_F]),
              pltpu.make_async_copy(wu_hbm, wu_ref, sem.at[SEM_F]),
              pltpu.make_async_copy(wd_hbm, wd_ref, sem.at[SEM_F])]

    out_pieces = [(i * TQ, TQ) for i in range(NB - 1)] + [(S - TQ + g * 128, 128) for g in range(NG)]

    def cp_out(j):
        r0, n = out_pieces[j]
        return pltpu.make_async_copy(out_ref.at[pl.ds(r0, n)], o_hbm.at[pl.ds(r0, n)], sem.at[SEM_O])

    def start_head(h):
        cp_k(h).start()
        cp_v(h).start()
        cp_wo(h).start()
        if isinstance(h, int):
            if h + 1 < H:
                cp_wq(h + 1).start()
        else:
            @pl.when(h + 1 < H)
            def _():
                cp_wq(h + 1).start()

    def wait_head(h):
        cp_k(h).wait()
        cp_v(h).wait()
        cp_wo(h).wait()
        if not isinstance(h, int) or h + 1 < H:
            cp_wq(h + 1).wait()

    lane = lax.broadcasted_iota(jnp.int32, (8, 128), 1)
    sub = lax.broadcasted_iota(jnp.int32, (8, 128), 0)

    class Ctx:
        def __init__(self):
            self.z1 = pl.multiple_of(z_ref[0], 8)
            self.z2 = pl.multiple_of(z_ref[1], 8)
            self.zvec = jnp.full((8, 128), z_ref[0], jnp.int32).astype(U32)
            self.hist = []
            self.lnh = []

        def tok(self, a):
            return pltpu.bitcast(a, U32) & self.zvec

        def memtok(self, ref):
            rows = 16 if ref.dtype == BF else 8
            z = pl.multiple_of(self.z2 * 2, 16)
            return self.tok(ref[pl.ds(z, rows), 0:128])

    def dep_bf(a, t):
        if t is None:
            return a
        au = pltpu.bitcast(a, U32)
        first = au[0:8, 0:128] | t
        top = first if au.shape[1] == 128 else jnp.concatenate([first, au[0:8, 128:]], axis=1)
        return pltpu.bitcast(jnp.concatenate([top, au[8:]], axis=0), BF)

    def dep_f32(a, t):
        return pltpu.bitcast(pltpu.bitcast(a, U32) | t, F32)

    def layernorm(cx, r0, n, gate_tok=None):
        xv1 = x_ref.at[pl.ds(pl.multiple_of(cx.z1 * 2, 16), S), :]
        xv2 = x_ref.at[pl.ds(pl.multiple_of(cx.z2 * 2, 16), S), :]
        xv3 = x_ref.at[pl.ds(pl.multiple_of((cx.z1 + cx.z2) * 2, 16), S), :]
        if gate_tok is not None:
            x_ref[S:S + 16, 0:128] = pltpu.bitcast(cx.tok(gate_tok), BF)
        for c in range(n // LNC):
            a = r0 + c * LNC
            mf = jnp.mean(xv1[a:a + LNC, :].astype(F32), axis=-1, keepdims=True)
            xc = xv2[a:a + LNC, :].astype(F32) - mf
            x = xv3[a:a + LNC, :].astype(F32)
            v = _rb(_rb(jnp.mean(xc * xc, axis=-1, keepdims=True)) + 1e-5)
            den = _rb(v * lax.rsqrt(v))
            inv = pl.reciprocal(den, approx=True)
            inv = inv * (2.0 - den * inv)
            xn = (_rb(x - _rb(mf)) * inv).astype(BF)
            xn_ref[a:a + LNC, :] = xn

    def silu(b):
        hb = 0.5 * b
        return hb + hb * jnp.tanh(hb)

    def gate(r0, n):
        xf = xn_ref[pl.ds(r0, n), :].astype(F32)
        g_ref[pl.ds(r0, n), :] = silu(xf)
        r = _rb(jnp.sum(xf * wr_ref[...].astype(F32), axis=-1, keepdims=True))
        slot = jnp.concatenate([lane, lane + 128], axis=0)
        rc = rc_ref[...]
        for j in range(n // 8):
            rj = r[j * 8:(j + 1) * 8, :]
            rc = jnp.where(slot == r0 // 8 + j, jnp.concatenate([rj, rj], axis=0), rc)
        rc_ref[...] = rc

    def route():
        r = rc_ref[...]
        tix = jnp.concatenate([(8 * (128 * a + lane) + sub) for a in range(2)], axis=0).astype(F32)
        rw = jnp.where(r != r, -jnp.inf, r)
        alive = jnp.ones((16, 128), F32)
        for j in range(C):
            mx = jnp.max(jnp.max(rw, axis=0, keepdims=True), axis=1, keepdims=True)
            cand = jnp.where((rw == mx) & (alive > 0), tix, float(S - 1))
            ixv = jnp.min(jnp.min(cand, axis=0, keepdims=True), axis=1, keepdims=True)
            hit = tix == ixv
            rsel = jnp.sum(jnp.sum(jnp.where(hit, r, 0.0), axis=0, keepdims=True), axis=1, keepdims=True)
            rw = jnp.where(hit, -jnp.inf, rw)
            alive = jnp.where(hit, 0.0, alive)
            ix = ixv.astype(jnp.int32)[0, 0]
            idx_ref[j] = ix
            blk = xn_ref[pl.ds(pl.multiple_of((ix // 16) * 16, 16), 16), :].astype(F32)
            pick = lax.broadcasted_iota(jnp.int32, (16, D), 0) == (ixv.astype(jnp.int32) & 15)
            xs_ref[j:j + 1, :] = jnp.sum(jnp.where(pick, blk, 0.0), axis=0, keepdims=True)
            rs_ref[j:j + 1, :] = jnp.broadcast_to(rsel, (1, 128))

    def ffn_up():
        xs = xs_ref[...].astype(BF)
        g = _rb(lax.dot_general(xs, wg_ref[...], NT, preferred_element_type=F32))
        g = _rb(g * jax.nn.sigmoid(g))
        u = _rb(lax.dot_general(xs, wu_ref[...], NT, preferred_element_type=F32))
        return (g * u).astype(BF)

    def ffn_down(hid):
        y = _rb(jnp.dot(hid, wd_ref[...], preferred_element_type=F32))
        y = _rb(y * _rb(jax.nn.sigmoid(rs_ref[:, 0:1])))
        b = _rb(xs_ref[...] + y)
        gs = b * jax.nn.sigmoid(b)
        for j in range(C):
            g_ref[pl.ds(idx_ref[j], 1), :] = gs[j:j + 1, :]

    def qproj(i, h, split=1, t=None, cx=None):
        parts = []
        n = TQ // split
        for c in range(split):
            r0 = i * TQ + c * n
            xn = dep_bf(xn_ref[r0:r0 + n, :], t)
            d = jnp.dot(xn, wq_ref[h], preferred_element_type=F32)
            if cx is not None:
                for r in ATOK:
                    cx.hist.append(d[r:r + 8, :])
            parts.append((d * QSCALE).astype(BF))
        return parts[0] if split == 1 else jnp.concatenate(parts, axis=0)

    def transpose_v(cx, hh, h):
        vt_ref[hh, pl.ds(cx.z1, DH // 2), :] = pltpu.bitcast(v_ref[h].T, U32)

    def qk(cx, n, h, q, jobs=(), after=()):
        sv = s_refs[n % 2].at[pl.ds(cx.z1, S), :]
        ns = max(len(jobs) + 1, len(after))
        sl = S // ns
        m = None
        for j in range(ns):
            t = jobs[j - 1]() if 0 < j <= len(jobs) else None
            kj = dep_bf(k_ref[h, j * sl:(j + 1) * sl, :], t)
            sT = lax.dot_general(kj, q, NT, preferred_element_type=F32)
            sv[j * sl:(j + 1) * sl, :] = sT
            mj = jnp.max(jnp.max(sT.reshape(sl // 128, 16, 8, TQ), axis=1), axis=0)
            m = mj if m is None else jnp.maximum(m, mj)
            if j < len(after) and after[j] is not None:
                after[j](sT[0:8, 0:128])
        return jnp.broadcast_to(jnp.max(m, axis=0, keepdims=True), (8, TQ))

    def pv(cx, n, hh, m, hooks=None, groups=tuple(range(NG)), after=None):
        sv = s_refs[n % 2].at[pl.ds(cx.z2, S), :]
        vv = vt_ref.at[hh, pl.ds(cx.z2, DH // 2), :]
        otv = ot_ref.at[pl.ds(cx.z1, NG * DH), :]
        lrv = lr_ref.at[pl.ds(cx.z1, NG * 8), :]
        CT = PV_CT
        for g in groups:
            mg = m[:, g * 128:(g + 1) * 128]
            l8 = None
            oT = None
            for c in range(S // 128 // CT):
                mc = mg
                if len(cx.hist) >= PV_DIST:
                    mc = dep_f32(mc, cx.tok(cx.hist[-PV_DIST]))
                if hooks and (g * 4 + c) in hooks:
                    mc = dep_f32(mc, hooks[g * 4 + c])
                ps = []
                for tt in range(CT):
                    r0 = (c * CT + tt) * 128
                    s = sv[r0:r0 + 128, g * 128:(g + 1) * 128]
                    p = jnp.exp2(s - jnp.concatenate([mc] * 16, axis=0))
                    lt = None
                    for j in reversed(range(16)):
                        pj = p[j * 8:(j + 1) * 8, :]
                        lt = pj if lt is None else lt + pj
                    l8 = lt if l8 is None else l8 + lt
                    ps.append(p)
                vT = pltpu.bitcast(vv[:, c * CT * 128:(c + 1) * CT * 128], BF)
                part = jnp.dot(vT, jnp.concatenate(ps, axis=0).astype(BF), preferred_element_type=F32)
                cx.hist.append(part[0:8, :])
                if after and (g * 4 + c) in after:
                    after[g * 4 + c](part[0:8, :])
                oT = part if oT is None else oT + part
            otv[g * DH:(g + 1) * DH, :] = oT
            lrv[g * 8:(g + 1) * 8, :] = l8

    def load_o(cx, groups):
        otv = ot_ref.at[pl.ds(cx.z2, NG * DH), :]
        lrv = lr_ref.at[pl.ds(cx.z2, NG * 8), :]
        parts = []
        for g in groups:
            l = jnp.sum(lrv[g * 8:(g + 1) * 8, :], axis=0, keepdims=True)
            parts.append((otv[g * DH:(g + 1) * DH, :] * (1.0 / l)).T.astype(BF))
        return parts[0] if len(parts) == 1 else jnp.concatenate(parts, axis=0)

    def oproj(cx, i, h, mode, groups=tuple(range(NG)), toks=True):
        r0 = i * TQ + groups[0] * 128
        r1 = r0 + len(groups) * 128
        d = jnp.dot(load_o(cx, groups), wo_ref[h], preferred_element_type=F32)
        if mode == 'set':
            acc_ref[r0:r1, :] = d
        elif mode == 'add':
            acc_ref[r0:r1, :] += d
        else:
            s = acc_ref[r0:r1, :] + d
            out_ref[r0:r1, :] = (x_ref[r0:r1, :].astype(F32) + s * g_ref[r0:r1, :]).astype(BF)
        if toks:
            for r in DTOK:
                cx.hist.append(d[r:r + 8, 0:128])

    cp_x(0, SEM_A).start()
    cp_wq(0, SEM_A).start()
    cp_k(0, SEM_B).start()
    cp_x(1, SEM_B).start()
    cp_v(0, SEM_C).start()
    cp_x(2, SEM_D).start()
    cp_x(3, SEM_D).start()
    cp_wo(0, SEM_D).start()
    cp_wq(1, SEM_D).start()
    z_ref[0] = 0
    z_ref[1] = 0
    acc_ref[S - TQ:, :] = jnp.zeros((TQ, D), F32)
    cx = Ctx()
    rc_ref[...] = jnp.zeros((16, 128), F32)

    def ln_job(i, c):
        n = TQ // 8
        return lambda t=None: layernorm(cx, i * TQ + c * n, n, t)

    def gate_job(cx, r0, n):
        def job():
            gate(r0, n)
            return cx.memtok(g_ref) | cx.memtok(rc_ref)
        return job

    cp_x(0, SEM_A).wait()
    cp_wq(0, SEM_A).wait()
    layernorm(cx, 0, TQ)
    q = qproj(0, 0, split=4)
    cp_k(0, SEM_B).wait()
    cp_x(1, SEM_B).wait()
    for hh in range(HPI):
        start_head(1 + hh)
    for n in range(NB):
        if n == 1:
            cp_x(2, SEM_D).wait()
            cp_x(3, SEM_D).wait()
            cp_wo(0, SEM_D).wait()
            cp_wq(1, SEM_D).wait()
            for c in cp_ffn:
                c.start()
        if n + 1 < NB:
            ln_job(n + 1, 0)()
            m = qk(cx, n, 0, q, after=[ln_job(n + 1, 1 + j) for j in range(7)] + [None])
        else:
            m = qk(cx, n, 0, q)
        if n == 0:
            cp_v(0, SEM_C).wait()
            transpose_v(cx, 0, 0)
            q = qproj(1, 0)
        elif n + 1 < NB:
            oproj(cx, n - 1, 0, 'set', toks=False)
            q = qproj(n + 1, 0, cx=cx)
        else:
            q = qproj(0, 1)
            oproj(cx, n - 1, 0, 'set')
        pv(cx, n, 0, m)
    qn_ref[...] = pltpu.bitcast(q, U32)

    def body(it, _):
        h0 = 1 + it * HPI
        for hh in range(HPI):
            wait_head(h0 + hh)
        for hh in range(HPI):
            if hh == 0:
                start_head(h0 + HPI)
            else:
                @pl.when(h0 + HPI + hh < H)
                def _():
                    start_head(h0 + HPI + hh)
        cx = Ctx()
        for hh in range(HPI):
            transpose_v(cx, hh, h0 + hh)
        q = pltpu.bitcast(qn_ref[...], BF)
        h_prev = h0 - 1
        for n in range(HPI * NB):
            hh, i = divmod(n, NB)
            hn, in_ = divmod(n + 1, NB)
            jobs = ()
            if n == 1:
                r0 = pl.multiple_of(jnp.minimum(it * GROWS, S - GROWS), 16)
                jobs = (gate_job(cx, r0, GROWS),)
            m = qk(cx, n, h0 + hh, q, jobs)
            q = qproj(in_, h0 + hn)
            oproj(cx, (i - 1) % NB, h_prev, 'add')
            pv(cx, n, hh, m)
            h_prev = h0 + hh
        qn_ref[...] = pltpu.bitcast(q, U32)
        return 0

    lax.fori_loop(0, (H - 2) // HPI, body, 0)

    h = H - 1
    wait_head(h)
    for c in cp_ffn:
        c.wait()
    cx = Ctx()
    transpose_v(cx, 0, h)
    q = pltpu.bitcast(qn_ref[...], BF)
    route()
    m = qk(cx, 0, h, q)
    hid = ffn_up()
    q = qproj(1, h)
    oproj(cx, NB - 1, h - 1, 'add')
    pv(cx, 0, 0, m)
    ffn_down(hid)
    for n in range(1, NB):
        m = qk(cx, n, h, q)
        if n + 1 < NB:
            q = qproj(n + 1, h, t=cx.memtok(g_ref) if n == 1 else None)
        oproj(cx, n - 1, h, 'fin')
        cp_out(n - 1).start()
        pv(cx, n, 0, m, {FINH: cx.memtok(out_ref)})
    for g in range(NG):
        oproj(cx, NB - 1, h, 'fin', groups=(g,), toks=False)
        cp_out(NB - 1 + g).start()
    for j in range(len(out_pieces)):
        cp_out(j).wait()


@jax.jit
def pallas_recurrent_scan__mha_block_cached__moe_arch_mod__prompt_kernel(
    A_x, A_k_cache, A_v_cache, A_wq, A_wo, B_x, B_w_r, B_w_gate, B_w_up, B_w_down):
    x = A_x.reshape(S, D)
    k = A_k_cache.reshape(H, S, DH)
    v = A_v_cache.reshape(H, S, DH)
    wo = A_wo.reshape(H, DH, D)
    wr = B_w_r.reshape(1, D)
    anyspec = pl.BlockSpec(memory_space=pl.ANY)
    out = pl.pallas_call(
        _kernel,
        in_specs=[anyspec] * 5 + [pl.BlockSpec(memory_space=pltpu.VMEM)] + [anyspec] * 3,
        out_specs=anyspec,
        out_shape=jax.ShapeDtypeStruct((S, D), BF),
        scratch_shapes=[
            pltpu.VMEM((S + 16, D), BF),
            pltpu.VMEM((H, S, DH), BF),
            pltpu.VMEM((H, S, DH), BF),
            pltpu.VMEM((H, D, DH), BF),
            pltpu.VMEM((H, DH, D), BF),
            pltpu.VMEM((F, D), BF),
            pltpu.VMEM((F, D), BF),
            pltpu.VMEM((F, D), BF),
            pltpu.VMEM((S, D), BF),
            pltpu.VMEM((S, D), F32),
            pltpu.VMEM((S, D), F32),
            pltpu.VMEM((TQ // 2, DH), U32),
            pltpu.VMEM((HPI, DH // 2, S), U32),
            pltpu.VMEM((C, D), F32),
            pltpu.VMEM((C, 128), F32),
            pltpu.VMEM((16, 128), F32),
            pltpu.VMEM((S, D), BF),
            pltpu.SMEM((2,), jnp.int32),
            pltpu.SMEM((C,), jnp.int32),
            pltpu.VMEM((S, TQ), F32),
            pltpu.VMEM((S, TQ), F32),
            pltpu.VMEM((NG * DH, 128), F32),
            pltpu.VMEM((NG * 8, 128), F32),
            pltpu.SemaphoreType.DMA((7,)),
        ],
        compiler_params=pltpu.CompilerParams(
            vmem_limit_bytes=126 * 1024 * 1024,
            disable_bounds_checks=True,
            disable_semaphore_checks=True,
        ),
    )(x, k, v, A_wq, wo, wr, B_w_gate.T, B_w_up.T, B_w_down)
    return out.reshape(1, S, D)
```

```python
import math
import jax
import jax.numpy as jnp
from jax import lax
import jax.experimental.pallas as pl
import jax.experimental.pallas.tpu as pltpu

S, D, H, DH, F, C = 2048, 640, 32, 128, 1728, 8
TQ = 512
NB = S // TQ
NG = TQ // 128
BF = jnp.bfloat16
F32 = jnp.float32
U32 = jnp.uint32
QSCALE = (DH ** -0.5) * math.log2(math.e)
E = lambda k, d: d
PV_CT = 4
PV_DIST = E('PV_DIST', 3)
HPI = E('HPI', 1)
LNC = E('LNC', 32)
ATOK = (0, 0, 0, 0)
NJOB = E('NJOB', 8)
AFIRST = E('AFIRST', 0)
ONLYF = E('ONLYF', 0)
LN_DIST = E('LN_DIST', 2)
GROWS = 80 * HPI
FINH = E('FINH', 6)
DTOK = (128, 256, 384, 504)
NT = (((1,), (1,)), ((), ()))


def _rb(a):
    return a.astype(BF).astype(F32)


def _kernel(x_hbm, k_hbm, v_hbm, wq_hbm, wo_hbm, wr_hbm, wg_hbm, wu_hbm, wd_hbm,
            o_hbm,
            s0_ref, s1_ref, vt_ref, ot_ref, acc_ref, qn_ref,
            k_ref, v_ref, wq_ref, wo_ref, xn_ref, g_ref, out_ref, wg_ref, wu_ref, wd_ref,
            x_ref, lr_ref, xs_ref, rs_ref, rc_ref, wrf_ref, wr_ref, z_ref, idx_ref, sem):
    s_refs = (s0_ref, s1_ref)

    SEM_A, SEM_B, SEM_C, SEM_D, SEM_H, SEM_F, SEM_O = range(7)

    def cp_k(h, s=SEM_H):
        return pltpu.make_async_copy(k_hbm.at[h], k_ref.at[h], sem.at[s])

    def cp_v(h, s=SEM_H):
        return pltpu.make_async_copy(v_hbm.at[h], v_ref.at[h], sem.at[s])

    def cp_wq(h, s=SEM_H):
        off = h * DH if isinstance(h, int) else pl.multiple_of(h * DH, DH)
        return pltpu.make_async_copy(wq_hbm.at[:, pl.ds(off, DH)], wq_ref.at[h], sem.at[s])

    def cp_wo(h, s=SEM_H):
        return pltpu.make_async_copy(wo_hbm.at[h], wo_ref.at[h], sem.at[s])

    def cp_x(i, s):
        return pltpu.make_async_copy(x_hbm.at[pl.ds(i * TQ, TQ)], x_ref.at[pl.ds(i * TQ, TQ)], sem.at[s])

    cp_ffn = [pltpu.make_async_copy(wg_hbm, wg_ref, sem.at[SEM_F]),
              pltpu.make_async_copy(wu_hbm, wu_ref, sem.at[SEM_F]),
              pltpu.make_async_copy(wd_hbm, wd_ref, sem.at[SEM_F])]

    cp_wr = pltpu.make_async_copy(wr_hbm, wr_ref, sem.at[SEM_D])

    out_pieces = [(i * TQ, TQ) for i in range(NB - 1)] + [(S - TQ + g * 128, 128) for g in range(NG)]

    def cp_out(j):
        r0, n = out_pieces[j]
        return pltpu.make_async_copy(out_ref.at[pl.ds(r0, n)], o_hbm.at[pl.ds(r0, n)], sem.at[SEM_O])

    def start_head(h):
        cp_k(h).start()
        cp_v(h).start()
        cp_wo(h).start()
        if isinstance(h, int):
            if h + 1 < H:
                cp_wq(h + 1).start()
        else:
            @pl.when(h + 1 < H)
            def _():
                cp_wq(h + 1).start()

    def wait_head(h):
        cp_k(h).wait()
        cp_v(h).wait()
        cp_wo(h).wait()
        if not isinstance(h, int) or h + 1 < H:
            cp_wq(h + 1).wait()

    lane = lax.broadcasted_iota(jnp.int32, (8, 128), 1)
    sub = lax.broadcasted_iota(jnp.int32, (8, 128), 0)

    class Ctx:
        def __init__(self):
            self.z1 = pl.multiple_of(z_ref[0], 8)
            self.z2 = pl.multiple_of(z_ref[1], 8)
            self.zvec = jnp.full((8, 128), z_ref[0], jnp.int32).astype(U32)
            self.hist = []
            self.lnh = []

        def tok(self, a):
            return pltpu.bitcast(a, U32) & self.zvec

        def memtok(self, ref):
            rows = 16 if ref.dtype == BF else 8
            z = pl.multiple_of(self.z2 * 2, 16)
            return self.tok(ref[pl.ds(z, rows), 0:128])

    def dep_bf(a, t):
        if t is None:
            return a
        au = pltpu.bitcast(a, U32)
        first = au[0:8, 0:128] | t
        top = first if au.shape[1] == 128 else jnp.concatenate([first, au[0:8, 128:]], axis=1)
        return pltpu.bitcast(jnp.concatenate([top, au[8:]], axis=0), BF)

    def dep_f32(a, t):
        return pltpu.bitcast(pltpu.bitcast(a, U32) | t, F32)

    def layernorm(cx, r0, n, gate_tok=None):
        xv1 = x_ref.at[pl.ds(pl.multiple_of(cx.z1 * 2, 16), S), :]
        xv2 = x_ref.at[pl.ds(pl.multiple_of(cx.z2 * 2, 16), S), :]
        xv3 = x_ref.at[pl.ds(pl.multiple_of((cx.z1 + cx.z2) * 2, 16), S), :]
        if gate_tok is not None:
            x_ref[S:S + 16, 0:128] = pltpu.bitcast(cx.tok(gate_tok), BF)
        for c in range(n // LNC):
            a = r0 + c * LNC
            mf = jnp.mean(xv1[a:a + LNC, :].astype(F32), axis=-1, keepdims=True)
            xc = xv2[a:a + LNC, :].astype(F32) - mf
            x = xv3[a:a + LNC, :].astype(F32)
            v = _rb(_rb(jnp.mean(xc * xc, axis=-1, keepdims=True)) + 1e-5)
            den = _rb(v * lax.rsqrt(v))
            inv = pl.reciprocal(den, approx=True)
            inv = inv * (2.0 - den * inv)
            xn = (_rb(x - _rb(mf)) * inv).astype(BF)
            xn_ref[a:a + LNC, :] = xn

    def silu(b):
        hb = 0.5 * b
        return hb + hb * jnp.tanh(hb)

    def gate(r0, n):
        xf = xn_ref[pl.ds(r0, n), :].astype(F32)
        g_ref[pl.ds(r0, n), :] = silu(xf)
        r = _rb(jnp.sum(xf * jnp.concatenate([wrf_ref[...]] * (n // 8), axis=0), axis=-1, keepdims=True))
        slot = jnp.concatenate([lane, lane + 128], axis=0)
        rc = rc_ref[...]
        for j in range(n // 8):
            rj = r[j * 8:(j + 1) * 8, :]
            rc = jnp.where(slot == r0 // 8 + j, jnp.concatenate([rj, rj], axis=0), rc)
        rc_ref[...] = rc

    def route():
        r = rc_ref[...]
        tix = jnp.concatenate([(8 * (128 * a + lane) + sub) for a in range(2)], axis=0).astype(F32)
        rw = jnp.where(r != r, -jnp.inf, r)
        alive = jnp.ones((16, 128), F32)
        for j in range(C):
            mx = jnp.max(jnp.max(rw, axis=0, keepdims=True), axis=1, keepdims=True)
            cand = jnp.where((rw == mx) & (alive > 0), tix, float(S - 1))
            ixv = jnp.min(jnp.min(cand, axis=0, keepdims=True), axis=1, keepdims=True)
            hit = tix == ixv
            rsel = jnp.sum(jnp.sum(jnp.where(hit, r, 0.0), axis=0, keepdims=True), axis=1, keepdims=True)
            rw = jnp.where(hit, -jnp.inf, rw)
            alive = jnp.where(hit, 0.0, alive)
            ix = ixv.astype(jnp.int32)[0, 0]
            idx_ref[j] = ix
            blk = xn_ref[pl.ds(pl.multiple_of((ix // 16) * 16, 16), 16), :].astype(F32)
            pick = lax.broadcasted_iota(jnp.int32, (16, D), 0) == (ixv.astype(jnp.int32) & 15)
            xs_ref[j:j + 1, :] = jnp.sum(jnp.where(pick, blk, 0.0), axis=0, keepdims=True)
            rs_ref[j:j + 1, :] = jnp.broadcast_to(rsel, (1, 128))

    def ffn_up():
        xs = xs_ref[...].astype(BF)
        g = _rb(lax.dot_general(xs, wg_ref[...], NT, preferred_element_type=F32))
        g = _rb(g * jax.nn.sigmoid(g))
        u = _rb(lax.dot_general(xs, wu_ref[...], NT, preferred_element_type=F32))
        return (g * u).astype(BF)

    def ffn_down(hid):
        y = _rb(jnp.dot(hid, wd_ref[...], preferred_element_type=F32))
        y = _rb(y * _rb(jax.nn.sigmoid(rs_ref[:, 0:1])))
        b = _rb(xs_ref[...] + y)
        gs = b * jax.nn.sigmoid(b)
        for j in range(C):
            g_ref[pl.ds(idx_ref[j], 1), :] = gs[j:j + 1, :]

    def qproj(i, h, split=1, t=None, cx=None):
        parts = []
        n = TQ // split
        for c in range(split):
            r0 = i * TQ + c * n
            xn = dep_bf(xn_ref[r0:r0 + n, :], t)
            d = jnp.dot(xn, wq_ref[h], preferred_element_type=F32)
            if cx is not None:
                for r in ATOK:
                    cx.hist.append(d[r:r + 8, :])
            parts.append((d * QSCALE).astype(BF))
        return parts[0] if split == 1 else jnp.concatenate(parts, axis=0)

    def transpose_v(cx, hh, h):
        vt_ref[hh, pl.ds(cx.z1, DH // 2), :] = pltpu.bitcast(v_ref[h].T, U32)

    def qk(cx, n, h, q, jobs=(), after=()):
        sv = s_refs[n % 2].at[pl.ds(cx.z1, S), :]
        ns = max(len(jobs) + 1, len(after))
        sl = S // ns
        m = None
        for j in range(ns):
            t = jobs[j - 1]() if 0 < j <= len(jobs) else None
            kj = dep_bf(k_ref[h, j * sl:(j + 1) * sl, :], t)
            sT = lax.dot_general(kj, q, NT, preferred_element_type=F32)
            sv[j * sl:(j + 1) * sl, :] = sT
            mj = jnp.max(jnp.max(sT.reshape(sl // 128, 16, 8, TQ), axis=1), axis=0)
            m = mj if m is None else jnp.maximum(m, mj)
            if j < len(after) and after[j] is not None:
                after[j](sT[0:8, 0:128])
        return jnp.broadcast_to(jnp.max(m, axis=0, keepdims=True), (8, TQ))

    def pv(cx, n, hh, m, hooks=None, groups=tuple(range(NG)), after=None):
        sv = s_refs[n % 2].at[pl.ds(cx.z2, S), :]
        vv = vt_ref.at[hh, pl.ds(cx.z2, DH // 2), :]
        otv = ot_ref.at[pl.ds(cx.z1, NG * DH), :]
        lrv = lr_ref.at[pl.ds(cx.z1, NG * 8), :]
        CT = PV_CT
        for g in groups:
            mg = m[:, g * 128:(g + 1) * 128]
            l8 = None
            oT = None
            for c in range(S // 128 // CT):
                mc = mg
                if len(cx.hist) >= PV_DIST:
                    mc = dep_f32(mc, cx.tok(cx.hist[-PV_DIST]))
                if hooks and (g * 4 + c) in hooks:
                    mc = dep_f32(mc, hooks[g * 4 + c])
                ps = []
                for tt in range(CT):
                    r0 = (c * CT + tt) * 128
                    s = sv[r0:r0 + 128, g * 128:(g + 1) * 128]
                    p = jnp.exp2(s - jnp.concatenate([mc] * 16, axis=0))
                    lt = None
                    for j in reversed(range(16)):
                        pj = p[j * 8:(j + 1) * 8, :]
                        lt = pj if lt is None else lt + pj
                    l8 = lt if l8 is None else l8 + lt
                    ps.append(p)
                vT = pltpu.bitcast(vv[:, c * CT * 128:(c + 1) * CT * 128], BF)
                part = jnp.dot(vT, jnp.concatenate(ps, axis=0).astype(BF), preferred_element_type=F32)
                cx.hist.append(part[0:8, :])
                if after and (g * 4 + c) in after:
                    after[g * 4 + c](part[0:8, :])
                oT = part if oT is None else oT + part
            otv[g * DH:(g + 1) * DH, :] = oT
            lrv[g * 8:(g + 1) * 8, :] = l8

    def load_o(cx, groups):
        otv = ot_ref.at[pl.ds(cx.z2, NG * DH), :]
        lrv = lr_ref.at[pl.ds(cx.z2, NG * 8), :]
        parts = []
        for g in groups:
            l = jnp.sum(lrv[g * 8:(g + 1) * 8, :], axis=0, keepdims=True)
            parts.append((otv[g * DH:(g + 1) * DH, :] * (1.0 / l)).T.astype(BF))
        return parts[0] if len(parts) == 1 else jnp.concatenate(parts, axis=0)

    def oproj(cx, i, h, mode, groups=tuple(range(NG)), toks=True):
        r0 = i * TQ + groups[0] * 128
        r1 = r0 + len(groups) * 128
        d = jnp.dot(load_o(cx, groups), wo_ref[h], preferred_element_type=F32)
        if mode == 'set':
            acc_ref[r0:r1, :] = d
        elif mode == 'add':
            acc_ref[r0:r1, :] += d
        else:
            s = acc_ref[r0:r1, :] + d
            out_ref[r0:r1, :] = (x_ref[r0:r1, :].astype(F32) + s * g_ref[r0:r1, :]).astype(BF)
        if toks:
            for r in DTOK:
                cx.hist.append(d[r:r + 8, 0:128])

    cp_x(0, SEM_A).start()
    cp_wq(0, SEM_A).start()
    cp_k(0, SEM_B).start()
    cp_x(1, SEM_B).start()
    cp_v(0, SEM_C).start()
    cp_x(2, SEM_D).start()
    cp_x(3, SEM_D).start()
    cp_wo(0, SEM_D).start()
    cp_wq(1, SEM_D).start()
    cp_wr.start()
    z_ref[0] = 0
    z_ref[1] = 0
    acc_ref[S - TQ:, :] = jnp.zeros((TQ, D), F32)
    cx = Ctx()
    rc_ref[...] = jnp.zeros((16, 128), F32)

    def ln_job(i, c):
        n = TQ // NJOB
        return lambda t=None: layernorm(cx, i * TQ + c * n, n, t)

    def gate_job(cx, r0, n):
        def job():
            gate(r0, n)
            return cx.memtok(g_ref) | cx.memtok(rc_ref)
        return job

    cp_x(0, SEM_A).wait()
    cp_wq(0, SEM_A).wait()
    layernorm(cx, 0, TQ)
    q = qproj(0, 0, split=4)
    cp_k(0, SEM_B).wait()
    cp_x(1, SEM_B).wait()
    for hh in range(HPI):
        start_head(1 + hh)
    for n in range(NB):
        if n == 1:
            cp_x(2, SEM_D).wait()
            cp_x(3, SEM_D).wait()
            cp_wo(0, SEM_D).wait()
            cp_wq(1, SEM_D).wait()
            cp_wr.wait()
            wrf_ref[...] = jnp.broadcast_to(wr_ref[...].astype(F32).reshape(1, D), (8, D))
            for c in cp_ffn:
                c.start()
        if n + 1 < NB:
            ln_job(n + 1, 0)()
            m = qk(cx, n, 0, q, after=[ln_job(n + 1, 1 + j) for j in range(NJOB - 1)] + [None])
        else:
            m = qk(cx, n, 0, q)
        if n == 0:
            cp_v(0, SEM_C).wait()
            transpose_v(cx, 0, 0)
            q = qproj(1, 0)
        elif n + 1 < NB:
            oproj(cx, n - 1, 0, 'set', toks=False)
            q = qproj(n + 1, 0, cx=cx)
        else:
            q = qproj(0, 1)
            oproj(cx, n - 1, 0, 'set')
        pv(cx, n, 0, m)
    qn_ref[...] = pltpu.bitcast(q, U32)

    if ONLYF:
        wait_head(1)
        for c in cp_ffn:
            c.wait()
        out_ref[0:16, 0:128] = pltpu.bitcast(qn_ref[0:8, :], BF) + ot_ref[0:16, :].astype(BF) + acc_ref[0:16, 0:128].astype(BF)
        cp_out(3).start()
        cp_out(3).wait()
        return
    def body(it, _):
        h0 = 1 + it * HPI
        for hh in range(HPI):
            wait_head(h0 + hh)
        for hh in range(HPI):
            if hh == 0:
                start_head(h0 + HPI)
            else:
                @pl.when(h0 + HPI + hh < H)
                def _():
                    start_head(h0 + HPI + hh)
        cx = Ctx()
        for hh in range(HPI):
            transpose_v(cx, hh, h0 + hh)
        q = pltpu.bitcast(qn_ref[...], BF)
        h_prev = h0 - 1
        for n in range(HPI * NB):
            hh, i = divmod(n, NB)
            hn, in_ = divmod(n + 1, NB)
            jobs = ()
            if n == 1:
                r0 = pl.multiple_of(jnp.minimum(it * GROWS, S - GROWS), 16)
                jobs = (gate_job(cx, r0, GROWS),)
            if n == 0 and AFIRST:
                q_next = qproj(in_, h0 + hn)
                m = qk(cx, n, h0 + hh, q, jobs)
                q = q_next
            else:
                m = qk(cx, n, h0 + hh, q, jobs)
                q = qproj(in_, h0 + hn)
            oproj(cx, (i - 1) % NB, h_prev, 'add')
            pv(cx, n, hh, m)
            h_prev = h0 + hh
        qn_ref[...] = pltpu.bitcast(q, U32)
        return 0

    lax.fori_loop(0, (H - 2) // HPI, body, 0)

    h = H - 1
    wait_head(h)
    for c in cp_ffn:
        c.wait()
    cx = Ctx()
    transpose_v(cx, 0, h)
    q = pltpu.bitcast(qn_ref[...], BF)
    route()
    m = qk(cx, 0, h, q)
    hid = ffn_up()
    q = qproj(1, h)
    oproj(cx, NB - 1, h - 1, 'add')
    pv(cx, 0, 0, m)
    ffn_down(hid)
    for n in range(1, NB):
        m = qk(cx, n, h, q)
        if n + 1 < NB:
            q = qproj(n + 1, h, t=cx.memtok(g_ref) if n == 1 else None)
        oproj(cx, n - 1, h, 'fin')
        cp_out(n - 1).start()
        pv(cx, n, 0, m, {FINH: cx.memtok(out_ref)})
    for g in range(NG):
        oproj(cx, NB - 1, h, 'fin', groups=(g,), toks=False)
        cp_out(NB - 1 + g).start()
    for j in range(len(out_pieces)):
        cp_out(j).wait()


@jax.jit
def pallas_recurrent_scan__mha_block_cached__moe_arch_mod__prompt_kernel(
    A_x, A_k_cache, A_v_cache, A_wq, A_wo, B_x, B_w_r, B_w_gate, B_w_up, B_w_down):
    x = A_x.reshape(S, D)
    k = A_k_cache.reshape(H, S, DH)
    v = A_v_cache.reshape(H, S, DH)
    wo = A_wo.reshape(H, DH, D)
    wr = B_w_r
    anyspec = pl.BlockSpec(memory_space=pl.ANY)
    out = pl.pallas_call(
        _kernel,
        in_specs=[anyspec] * 9,
        out_specs=anyspec,
        out_shape=jax.ShapeDtypeStruct((S, D), BF),
        scratch_shapes=[
            pltpu.VMEM((S, TQ), F32),
            pltpu.VMEM((S, TQ), F32),
            pltpu.VMEM((HPI, DH // 2, S), U32),
            pltpu.VMEM((NG * DH, 128), F32),
            pltpu.VMEM((S, D), F32),
            pltpu.VMEM((TQ // 2, DH), U32),
            pltpu.VMEM((H, S, DH), BF),
            pltpu.VMEM((H, S, DH), BF),
            pltpu.VMEM((H, D, DH), BF),
            pltpu.VMEM((H, DH, D), BF),
            pltpu.VMEM((S, D), BF),
            pltpu.VMEM((S, D), F32),
            pltpu.VMEM((S, D), BF),
            pltpu.VMEM((F, D), BF),
            pltpu.VMEM((F, D), BF),
            pltpu.VMEM((F, D), BF),
            pltpu.VMEM((S + 64, D), BF),
            pltpu.VMEM((NG * 8, 128), F32),
            pltpu.VMEM((C, D), F32),
            pltpu.VMEM((C, 128), F32),
            pltpu.VMEM((16, 128), F32),
            pltpu.VMEM((8, D), F32),
            pltpu.VMEM((D,), BF),
            pltpu.SMEM((2,), jnp.int32),
            pltpu.SMEM((C,), jnp.int32),
            pltpu.SemaphoreType.DMA((7,)),
        ],
        compiler_params=pltpu.CompilerParams(
            vmem_limit_bytes=126 * 1024 * 1024,
            internal_scratch_in_bytes=16 * 4096,
            disable_bounds_checks=True,
            disable_semaphore_checks=True,
        ),
    )(x, k, v, A_wq, wo, wr, B_w_gate.T, B_w_up.T, B_w_down)
    return out.reshape(1, S, D)
```

```python
import math
import jax
import jax.numpy as jnp
from jax import lax
import jax.experimental.pallas as pl
import jax.experimental.pallas.tpu as pltpu

S, D, H, DH, F, C = 2048, 640, 32, 128, 1728, 8
TQ = 512
NB = S // TQ
NG = TQ // 128
BF = jnp.bfloat16
F32 = jnp.float32
U32 = jnp.uint32
QSCALE = (DH ** -0.5) * math.log2(math.e)
E = lambda k, d: d
PV_CT = 4
PV_DIST = E('PV_DIST', 3)
HPI = E('HPI', 1)
LNC = E('LNC', 32)
ATOK = ()
NJOB = E('NJOB', 8)
AFIRST = E('AFIRST', 0)
ONLYF = E('ONLYF', 0)
TAILH = E('TAILH', 0)
FSL = E('FSL', 16)
FH0 = E('FH0', 9)
RTH = E('RTH', 12)
LASTONLY = E('LASTONLY', 0)
LOOPONLY = E('LOOPONLY', 0)
GSPL = E('GSPL', 1)
GUN = E('GUN', 1)
GMODE = E('GMODE', 0)
LN_DIST = E('LN_DIST', 2)
GROWS = 80 * HPI
FINH = E('FINH', 6)
DTOK = (128, 256, 384, 504)
NT = (((1,), (1,)), ((), ()))


def _rb(a):
    return a.astype(BF).astype(F32)


def _kernel(x_hbm, k_hbm, v_hbm, wq_hbm, wo_hbm, wr_hbm, wg_hbm, wu_hbm, wd_hbm,
            o_hbm,
            s0_ref, s1_ref, vt_ref, ot_ref, ot2_ref, acc_ref, qn_ref,
            k_ref, v_ref, wq_ref, wo_ref, xn_ref, g_ref, out_ref, wg_ref, wu_ref, wd_ref,
            x_ref, lr_ref, lr2_ref, xs_ref, rs_ref, wrf_ref, wr_ref, z_ref, idx_ref, sem):
    s_refs = (s0_ref, s1_ref)
    ot_refs = (ot_ref, ot2_ref)
    lr_refs = (lr_ref, lr2_ref)

    SEM_A, SEM_B, SEM_C, SEM_D, SEM_H, SEM_F, SEM_O = range(7)

    def cp_k(h, s=SEM_H):
        return pltpu.make_async_copy(k_hbm.at[h], k_ref.at[h], sem.at[s])

    def cp_v(h, s=SEM_H):
        return pltpu.make_async_copy(v_hbm.at[h], v_ref.at[h], sem.at[s])

    def cp_wq(h, s=SEM_H):
        off = h * DH if isinstance(h, int) else pl.multiple_of(h * DH, DH)
        return pltpu.make_async_copy(wq_hbm.at[:, pl.ds(off, DH)], wq_ref.at[h], sem.at[s])

    def cp_wo(h, s=SEM_H):
        return pltpu.make_async_copy(wo_hbm.at[h], wo_ref.at[h], sem.at[s])

    def cp_x(i, s):
        return pltpu.make_async_copy(x_hbm.at[pl.ds(i * TQ, TQ)], x_ref.at[pl.ds(i * TQ, TQ)], sem.at[s])

    cp_ffn = [pltpu.make_async_copy(wg_hbm, wg_ref, sem.at[SEM_F]),
              pltpu.make_async_copy(wu_hbm, wu_ref, sem.at[SEM_F]),
              pltpu.make_async_copy(wd_hbm, wd_ref, sem.at[SEM_F])]

    cp_wr = pltpu.make_async_copy(wr_hbm, wr_ref, sem.at[SEM_D])

    out_pieces = [(i * TQ, TQ) for i in range(NB - 1)] + [(S - TQ + g * 128, 128) for g in range(NG)]

    def cp_out(j):
        r0, n = out_pieces[j]
        return pltpu.make_async_copy(out_ref.at[pl.ds(r0, n)], o_hbm.at[pl.ds(r0, n)], sem.at[SEM_O])

    def start_head(h):
        cp_k(h).start()
        cp_v(h).start()
        cp_wo(h).start()
        if isinstance(h, int):
            if h + 1 < H:
                cp_wq(h + 1).start()
        else:
            @pl.when(h + 1 < H)
            def _():
                cp_wq(h + 1).start()

    def wait_head(h):
        cp_k(h).wait()
        cp_v(h).wait()
        cp_wo(h).wait()
        if not isinstance(h, int) or h + 1 < H:
            cp_wq(h + 1).wait()

    lane = lax.broadcasted_iota(jnp.int32, (8, 128), 1)
    sub = lax.broadcasted_iota(jnp.int32, (8, 128), 0)

    class Ctx:
        def __init__(self):
            self.z1 = pl.multiple_of(z_ref[0], 8)
            self.z2 = pl.multiple_of(z_ref[1], 8)
            self.zvec = jnp.full((8, 128), z_ref[0], jnp.int32).astype(U32)
            self.hist = []
            self.lnh = []

        def tok(self, a):
            return pltpu.bitcast(a, U32) & self.zvec

        def memtok(self, ref):
            rows = 16 if ref.dtype == BF else 8
            z = pl.multiple_of(self.z2 * 2, 16)
            return self.tok(ref[pl.ds(z, rows), 0:128])

    def dep_bf(a, t):
        if t is None:
            return a
        au = pltpu.bitcast(a, U32)
        first = au[0:8, 0:128] | t
        top = first if au.shape[1] == 128 else jnp.concatenate([first, au[0:8, 128:]], axis=1)
        return pltpu.bitcast(jnp.concatenate([top, au[8:]], axis=0), BF)

    def dep_f32(a, t):
        return pltpu.bitcast(pltpu.bitcast(a, U32) | t, F32)

    def layernorm(cx, r0, n, gate_tok=None):
        xv1 = x_ref.at[pl.ds(pl.multiple_of(cx.z1 * 2, 16), S), :]
        xv2 = x_ref.at[pl.ds(pl.multiple_of(cx.z2 * 2, 16), S), :]
        xv3 = x_ref.at[pl.ds(pl.multiple_of((cx.z1 + cx.z2) * 2, 16), S), :]
        if gate_tok is not None:
            x_ref[S:S + 16, 0:128] = pltpu.bitcast(cx.tok(gate_tok), BF)
        for c in range(n // LNC):
            a = r0 + c * LNC
            mf = jnp.mean(xv1[a:a + LNC, :].astype(F32), axis=-1, keepdims=True)
            xc = xv2[a:a + LNC, :].astype(F32) - mf
            x = xv3[a:a + LNC, :].astype(F32)
            v = _rb(_rb(jnp.mean(xc * xc, axis=-1, keepdims=True)) + 1e-5)
            den = _rb(v * lax.rsqrt(v))
            inv = pl.reciprocal(den, approx=True)
            inv = inv * (2.0 - den * inv)
            xn = (_rb(x - _rb(mf)) * inv).astype(BF)
            xn_ref[a:a + LNC, :] = xn

    def silu(b):
        hb = 0.5 * b
        return hb + hb * jnp.tanh(hb)

    def gate(r0, n):
        xf = xn_ref[pl.ds(r0, n), :].astype(F32)
        g_ref[pl.ds(r0, n), :] = silu(xf)
        return xf

    def router(cx, r0, n, rc, gate_tok=None):
        xv = xn_ref.at[pl.ds(pl.multiple_of(cx.z2 * 2, 16), S), :]
        if gate_tok is not None:
            xn_ref[S:S + 16, 0:128] = pltpu.bitcast(cx.tok(gate_tok), BF)
        for c in range(n // LNC):
            a = r0 + c * LNC
            xf = xv[a:a + LNC, :].astype(F32)
            r = _rb(jnp.sum(xf * jnp.concatenate([wrf_ref[...]] * (LNC // 8), axis=0), axis=-1, keepdims=True))
            for j in range(LNC // 8):
                gi = a // 8 + j
                rc[gi // 128] = jnp.where(lane == gi % 128, r[j * 8:(j + 1) * 8, :], rc[gi // 128])

    def route(rc):
        r = jnp.concatenate(rc, axis=0)
        tix = jnp.concatenate([(8 * (128 * a + lane) + sub) for a in range(2)], axis=0).astype(F32)
        rw = jnp.where(r != r, -jnp.inf, r)
        alive = jnp.ones((16, 128), F32)
        for j in range(C):
            mx = jnp.max(jnp.max(rw, axis=0, keepdims=True), axis=1, keepdims=True)
            cand = jnp.where((rw == mx) & (alive > 0), tix, float(S - 1))
            ixv = jnp.min(jnp.min(cand, axis=0, keepdims=True), axis=1, keepdims=True)
            hit = tix == ixv
            rsel = jnp.sum(jnp.sum(jnp.where(hit, r, 0.0), axis=0, keepdims=True), axis=1, keepdims=True)
            rw = jnp.where(hit, -jnp.inf, rw)
            alive = jnp.where(hit, 0.0, alive)
            ix = ixv.astype(jnp.int32)[0, 0]
            idx_ref[j] = ix
            blk = xn_ref[pl.ds(pl.multiple_of((ix // 16) * 16, 16), 16), :].astype(F32)
            pick = lax.broadcasted_iota(jnp.int32, (16, D), 0) == (ixv.astype(jnp.int32) & 15)
            xs_ref[j:j + 1, :] = jnp.sum(jnp.where(pick, blk, 0.0), axis=0, keepdims=True)
            rs_ref[j:j + 1, :] = jnp.broadcast_to(rsel, (1, 128))

    FT = [(f0, min(128, F - f0)) for f0 in range(0, F, 128)]

    class Ffn:
        def __init__(self):
            self.xs = xs_ref[...].astype(BF)
            self.acc = {}
            self.up = [(w, i, k) for i in range(len(FT)) for w in (0, 1) for k in range(D // 128)]
            self.down = [(i, k) for k in range(D // 128) for i in range(len(FT))]
            self.hid = None

        def add(self, key, d):
            self.acc[key] = d if key not in self.acc else self.acc[key] + d

        def run_up(self, n):
            for _ in range(min(n, len(self.up))):
                w, i, k = self.up.pop(0)
                f0, fn = FT[i]
                wt = (wg_ref, wu_ref)[w][f0:f0 + fn, k * 128:(k + 1) * 128]
                self.add((w, i), lax.dot_general(self.xs[:, k * 128:(k + 1) * 128], wt, NT, preferred_element_type=F32))

        def run_down(self, n):
            if self.hid is None:
                self.run_up(len(self.up))
                self.hid = []
                for i in range(len(FT)):
                    g = _rb(self.acc[(0, i)])
                    g = _rb(g * jax.nn.sigmoid(g))
                    self.hid.append((g * _rb(self.acc[(1, i)])).astype(BF))
            for _ in range(min(n, len(self.down))):
                i, k = self.down.pop(0)
                f0, fn = FT[i]
                self.add((2, k), jnp.dot(self.hid[i], wd_ref[f0:f0 + fn, k * 128:(k + 1) * 128], preferred_element_type=F32))

        def finish(self):
            self.run_down(len(self.down))
            y = _rb(jnp.concatenate([self.acc[(2, k)] for k in range(D // 128)], axis=1))
            y = _rb(y * _rb(jax.nn.sigmoid(rs_ref[:, 0:1])))
            b = _rb(xs_ref[...] + y)
            gs = b * jax.nn.sigmoid(b)
            for j in range(C):
                g_ref[pl.ds(idx_ref[j], 1), :] = gs[j:j + 1, :]

    def qproj(i, h, split=1, t=None, cx=None):
        parts = []
        n = TQ // split
        for c in range(split):
            r0 = i * TQ + c * n
            xn = dep_bf(xn_ref[r0:r0 + n, :], t)
            d = jnp.dot(xn, wq_ref[h], preferred_element_type=F32)
            if cx is not None:
                for r in ATOK:
                    cx.hist.append(d[r:r + 8, :])
            parts.append((d * QSCALE).astype(BF))
        return parts[0] if split == 1 else jnp.concatenate(parts, axis=0)

    def transpose_v(cx, hh, h):
        vt_ref[hh, pl.ds(cx.z1, DH // 2), :] = pltpu.bitcast(v_ref[h].T, U32)

    def qk(cx, n, h, q, jobs=(), after=()):
        sv = s_refs[n % 2].at[pl.ds(cx.z1, S), :]
        ns = max(len(jobs) + 1, len(after))
        sl = S // ns
        m = None
        for j in range(ns):
            t = jobs[j - 1]() if 0 < j <= len(jobs) else None
            kj = dep_bf(k_ref[h, j * sl:(j + 1) * sl, :], t)
            sT = lax.dot_general(kj, q, NT, preferred_element_type=F32)
            sv[j * sl:(j + 1) * sl, :] = sT
            mj = jnp.max(jnp.max(sT.reshape(sl // 128, 16, 8, TQ), axis=1), axis=0)
            m = mj if m is None else jnp.maximum(m, mj)
            if j < len(after) and after[j] is not None:
                after[j](sT[0:8, 0:128])
        return jnp.broadcast_to(jnp.max(m, axis=0, keepdims=True), (8, TQ))

    def pv(cx, n, hh, m, hooks=None, groups=tuple(range(NG)), after=None, buf=0):
        sv = s_refs[n % 2].at[pl.ds(cx.z2, S), :]
        vv = vt_ref.at[hh, pl.ds(cx.z2, DH // 2), :]
        otv = ot_refs[buf].at[pl.ds(cx.z1, NG * DH), :]
        lrv = lr_refs[buf].at[pl.ds(cx.z1, NG * 8), :]
        CT = PV_CT
        for g in groups:
            mg = m[:, g * 128:(g + 1) * 128]
            l8 = None
            oT = None
            for c in range(S // 128 // CT):
                mc = mg
                if len(cx.hist) >= PV_DIST:
                    mc = dep_f32(mc, cx.tok(cx.hist[-PV_DIST]))
                if hooks and (g * 4 + c) in hooks:
                    mc = dep_f32(mc, hooks[g * 4 + c])
                ps = []
                for tt in range(CT):
                    r0 = (c * CT + tt) * 128
                    s = sv[r0:r0 + 128, g * 128:(g + 1) * 128]
                    p = jnp.exp2(s - jnp.concatenate([mc] * 16, axis=0))
                    lt = None
                    for j in reversed(range(16)):
                        pj = p[j * 8:(j + 1) * 8, :]
                        lt = pj if lt is None else lt + pj
                    l8 = lt if l8 is None else l8 + lt
                    ps.append(p)
                vT = pltpu.bitcast(vv[:, c * CT * 128:(c + 1) * CT * 128], BF)
                part = jnp.dot(vT, jnp.concatenate(ps, axis=0).astype(BF), preferred_element_type=F32)
                cx.hist.append(part[0:8, :])
                if after and (g * 4 + c) in after:
                    after[g * 4 + c](part[0:8, :])
                oT = part if oT is None else oT + part
            otv[g * DH:(g + 1) * DH, :] = oT
            lrv[g * 8:(g + 1) * 8, :] = l8

    def load_o(cx, groups, buf=0):
        otv = ot_refs[buf].at[pl.ds(cx.z2, NG * DH), :]
        lrv = lr_refs[buf].at[pl.ds(cx.z2, NG * 8), :]
        parts = []
        for g in groups:
            l = jnp.sum(lrv[g * 8:(g + 1) * 8, :], axis=0, keepdims=True)
            parts.append((otv[g * DH:(g + 1) * DH, :] * (1.0 / l)).T.astype(BF))
        return parts[0] if len(parts) == 1 else jnp.concatenate(parts, axis=0)

    def oproj(cx, i, h, mode, groups=tuple(range(NG)), toks=True, o=None):
        r0 = i * TQ + groups[0] * 128
        r1 = r0 + len(groups) * 128
        if o is None:
            o = load_o(cx, groups)
        d = jnp.dot(o, wo_ref[h], preferred_element_type=F32)
        if mode == 'set':
            acc_ref[r0:r1, :] = d
        elif mode == 'add':
            acc_ref[r0:r1, :] += d
        else:
            s = acc_ref[r0:r1, :] + d
            out_ref[r0:r1, :] = (x_ref[r0:r1, :].astype(F32) + s * g_ref[r0:r1, :]).astype(BF)
        if toks:
            for r in DTOK:
                cx.hist.append(d[r:r + 8, 0:128])

    cp_x(0, SEM_A).start()
    cp_wq(0, SEM_A).start()
    cp_k(0, SEM_B).start()
    cp_x(1, SEM_B).start()
    cp_v(0, SEM_C).start()
    cp_x(2, SEM_D).start()
    cp_x(3, SEM_D).start()
    cp_wo(0, SEM_D).start()
    cp_wq(1, SEM_D).start()
    cp_wr.start()
    z_ref[0] = 0
    z_ref[1] = 0
    acc_ref[S - TQ:, :] = jnp.zeros((TQ, D), F32)
    cx = Ctx()
    rc = [jnp.zeros((8, 128), F32), jnp.zeros((8, 128), F32)]

    def ln_job(i, c):
        n = TQ // NJOB
        return lambda t=None: layernorm(cx, i * TQ + c * n, n, t)

    def gate_job(cx, r0, n):
        def job():
            xf = gate(r0, n)
            if GMODE == 2:
                return None
            t = cx.memtok(g_ref)
            if GMODE == 3:
                r = jnp.max(xf, axis=-1, keepdims=True)
                u = jnp.zeros((8, 128), F32)
                for j in range(n // 8):
                    u = jnp.where(lane == j, r[j * 8:(j + 1) * 8, :], u)
                t = t | cx.tok(u)
            return t
        return job

    if LASTONLY:
        start_head(H - 1)
        for c in cp_ffn:
            c.start()
        def _b(i, c_):
            z_ref[1] = z_ref[0] * i
            z_ref[0] = z_ref[1] * i
            return c_
        lax.fori_loop(0, 3, _b, 0)
    elif LOOPONLY:
        start_head(1)
        for c in cp_ffn:
            c.start()
    else:
        cp_x(0, SEM_A).wait()
        cp_wq(0, SEM_A).wait()
        layernorm(cx, 0, TQ)
        q = qproj(0, 0, split=4)
        cp_k(0, SEM_B).wait()
        cp_x(1, SEM_B).wait()
        for hh in range(HPI):
            start_head(1 + hh)
        for n in range(NB):
            if n == 1:
                cp_x(2, SEM_D).wait()
                cp_x(3, SEM_D).wait()
                cp_wo(0, SEM_D).wait()
                cp_wq(1, SEM_D).wait()
                cp_wr.wait()
                wrf_ref[...] = jnp.broadcast_to(wr_ref[...].astype(F32).reshape(1, D), (8, D))
                for c in cp_ffn:
                    c.start()
            if n + 1 < NB:
                ln_job(n + 1, 0)()
                m = qk(cx, n, 0, q, after=[ln_job(n + 1, 1 + j) for j in range(NJOB - 1)] + [None])
            else:
                rn = S // NJOB
                router(cx, 0, rn, rc)
                m = qk(cx, n, 0, q, after=[(lambda t, j=j: router(cx, (j + 1) * rn, rn, rc, t)) for j in range(NJOB - 1)] + [None])
                route(rc)
            if n == 0:
                cp_v(0, SEM_C).wait()
                transpose_v(cx, 0, 0)
                q = qproj(1, 0)
            elif n + 1 < NB:
                oproj(cx, n - 1, 0, 'set', toks=False)
                q = qproj(n + 1, 0, cx=cx)
            else:
                q = qproj(0, 1)
                oproj(cx, n - 1, 0, 'set')
            pv(cx, n, 0, m, {RTH: cx.memtok(xs_ref) | cx.memtok(rs_ref)} if n + 1 == NB else None)
        qn_ref[...] = pltpu.bitcast(q, U32)

        if ONLYF:
            wait_head(1)
            for c in cp_ffn:
                c.wait()
            out_ref[0:16, 0:128] = pltpu.bitcast(qn_ref[0:8, :], BF) + ot_ref[0:16, :].astype(BF) + acc_ref[0:16, 0:128].astype(BF)
            cp_out(3).start()
            cp_out(3).wait()
            return
    if not LASTONLY:
        def body(it, _):
            h0 = 1 + it * HPI
            for hh in range(HPI):
                wait_head(h0 + hh)
            for hh in range(HPI):
                if hh == 0:
                    start_head(h0 + HPI)
                else:
                    @pl.when(h0 + HPI + hh < H)
                    def _():
                        start_head(h0 + HPI + hh)
            cx = Ctx()
            for hh in range(HPI):
                transpose_v(cx, hh, h0 + hh)
            q = pltpu.bitcast(qn_ref[...], BF)
            h_prev = h0 - 1
            for n in range(HPI * NB):
                hh, i = divmod(n, NB)
                hn, in_ = divmod(n + 1, NB)
                jobs = ()
                if n == GUN:
                    gate(pl.multiple_of(jnp.minimum(it * GROWS, S - GROWS), 16), GROWS)
                if n == 0 and AFIRST:
                    q_next = qproj(in_, h0 + hn)
                    m = qk(cx, n, h0 + hh, q, jobs)
                    q = q_next
                else:
                    m = qk(cx, n, h0 + hh, q, jobs)
                    q = qproj(in_, h0 + hn)
                oproj(cx, (i - 1) % NB, h_prev, 'add')
                pv(cx, n, hh, m)
                h_prev = h0 + hh
            qn_ref[...] = pltpu.bitcast(q, U32)
            return 0

        lax.fori_loop(0, (H - 2) // HPI, body, 0)

    h = H - 1
    wait_head(h)
    for c in cp_ffn:
        c.wait()
    if LOOPONLY:
        out_ref[0:16, 0:128] = pltpu.bitcast(qn_ref[0:8, :], BF) + ot_ref[0:16, :].astype(BF) + acc_ref[0:16, 0:128].astype(BF) + g_ref[0:16, 0:128].astype(BF)
        cp_out(3).start()
        cp_out(3).wait()
        return
    cx = Ctx()
    transpose_v(cx, 0, h)
    q = pltpu.bitcast(qn_ref[...], BF)
    ffn = Ffn()
    cnt = lambda tot, j: (tot * (j + 1)) // (FSL - 1) - (tot * j) // (FSL - 1)
    m = qk(cx, 0, h, q, after=[(lambda t, j=j: ffn.run_up(cnt(70, j))) for j in range(FSL - 1)] + [None])
    q = qproj(1, h)
    oproj(cx, NB - 1, h - 1, 'add')
    pv(cx, 0, 0, m)
    m = qk(cx, 1, h, q, after=[(lambda t, j=j: ffn.run_up(cnt(70, j))) for j in range(FSL - 1)] + [None])
    q = qproj(2, h, cx=cx)
    pv(cx, 1, 0, m, buf=1)
    m = qk(cx, 2, h, q, after=[(lambda t, j=j: ffn.run_down(cnt(70, j))) for j in range(FSL - 1)] + [None])
    ffn.finish()
    q = qproj(3, h, t=None)
    allg = tuple(range(NG))
    oproj(cx, 0, h, 'fin', toks=False)
    cp_out(0).start()
    oproj(cx, 1, h, 'fin', o=load_o(cx, allg, 1))
    cp_out(1).start()
    pv(cx, 2, 0, m, {FINH: cx.memtok(out_ref)})
    m = qk(cx, 3, h, q)
    oproj(cx, 2, h, 'fin')
    cp_out(2).start()

    def alltok(o):
        u = pltpu.bitcast(o, U32)
        t = u[0:8]
        for r in range(8, u.shape[0], 8):
            t = t | u[r:r + 8]
        return t & cx.zvec

    pv(cx, NB - 1, 0, m, {FINH: cx.memtok(out_ref)}, groups=(0, 1))
    os = [load_o(cx, (0,)), load_o(cx, (1,))]
    pv(cx, NB - 1, 0, m, groups=(2,))
    os.append(load_o(cx, (2,)))
    pv(cx, NB - 1, 0, m, {TAILH: alltok(os[0]) | alltok(os[1])} if TAILH else None, groups=(3,))
    os.append(load_o(cx, (3,)))
    for g in range(NG):
        oproj(cx, NB - 1, h, 'fin', groups=(g,), toks=False, o=os[g])
        cp_out(NB - 1 + g).start()
    for j in range(len(out_pieces)):
        cp_out(j).wait()


@jax.jit
def pallas_recurrent_scan__mha_block_cached__moe_arch_mod__prompt_kernel(
    A_x, A_k_cache, A_v_cache, A_wq, A_wo, B_x, B_w_r, B_w_gate, B_w_up, B_w_down):
    x = A_x.reshape(S, D)
    k = A_k_cache.reshape(H, S, DH)
    v = A_v_cache.reshape(H, S, DH)
    wo = A_wo.reshape(H, DH, D)
    wr = B_w_r
    anyspec = pl.BlockSpec(memory_space=pl.ANY)
    out = pl.pallas_call(
        _kernel,
        in_specs=[anyspec] * 9,
        out_specs=anyspec,
        out_shape=jax.ShapeDtypeStruct((S, D), BF),
        scratch_shapes=[
            pltpu.VMEM((S, TQ), F32),
            pltpu.VMEM((S, TQ), F32),
            pltpu.VMEM((HPI, DH // 2, S), U32),
            pltpu.VMEM((NG * DH, 128), F32),
            pltpu.VMEM((NG * DH, 128), F32),
            pltpu.VMEM((S, D), F32),
            pltpu.VMEM((TQ // 2, DH), U32),
            pltpu.VMEM((H, S, DH), BF),
            pltpu.VMEM((H, S, DH), BF),
            pltpu.VMEM((H, D, DH), BF),
            pltpu.VMEM((H, DH, D), BF),
            pltpu.VMEM((S + 64, D), BF),
            pltpu.VMEM((S, D), F32),
            pltpu.VMEM((S, D), BF),
            pltpu.VMEM((F, D), BF),
            pltpu.VMEM((F, D), BF),
            pltpu.VMEM((F, D), BF),
            pltpu.VMEM((S + 64, D), BF),
            pltpu.VMEM((NG * 8, 128), F32),
            pltpu.VMEM((NG * 8, 128), F32),
            pltpu.VMEM((C, D), F32),
            pltpu.VMEM((C, 128), F32),
            pltpu.VMEM((8, D), F32),
            pltpu.VMEM((D,), BF),
            pltpu.SMEM((2,), jnp.int32),
            pltpu.SMEM((C,), jnp.int32),
            pltpu.SemaphoreType.DMA((7,)),
        ],
        compiler_params=pltpu.CompilerParams(
            vmem_limit_bytes=126 * 1024 * 1024,
            internal_scratch_in_bytes=16 * 4096,
            disable_bounds_checks=True,
            disable_semaphore_checks=True,
        ),
    )(x, k, v, A_wq, wo, wr, B_w_gate.T, B_w_up.T, B_w_down)
    return out.reshape(1, S, D)
```

```python
import math
import jax
import jax.numpy as jnp
from jax import lax
import jax.experimental.pallas as pl
import jax.experimental.pallas.tpu as pltpu

S, D, H, DH, F, C = 2048, 640, 32, 128, 1728, 8
TQ = 512
NB = S // TQ
NG = TQ // 128
BF = jnp.bfloat16
F32 = jnp.float32
U32 = jnp.uint32
QSCALE = (DH ** -0.5) * math.log2(math.e)
E = lambda k, d: d
PV_CT = 4
PV_DIST = E('PV_DIST', 3)
HPI = E('HPI', 1)
LNC = E('LNC', 8)
RC_ = 16
RJOB = E('RJOB', 32)
RSPAN = E('RSPAN', 1900)
LAG2 = E('LAG2', 4)
TSL = E('TSL', 1)
LAG3 = E('LAG3', 10)
LOFF = E('LOFF', 0)
ROFF = E('ROFF', 0)
DA = E('DA', 0)
OGT = E('OGT', 0)
LSPAN0 = E('LSPAN0', 2000)
LSPAN = E('LSPAN', 2040)
L0C = E('L0C', 32)
L0A = E('L0A', 0)
L0B = E('L0B', 0)
ATOK = ()
NJOB = E('NJOB', 8)
AFIRST = E('AFIRST', 0)
ONLYF = E('ONLYF', 0)
TAILH = E('TAILH', 0)
FSL = E('FSL', 16)
FH0 = E('FH0', 9)
RTH = E('RTH', 12)
LASTONLY = E('LASTONLY', 0)
LOOPONLY = E('LOOPONLY', 0)
GSPL = E('GSPL', 1)
GUN = E('GUN', 1)
GMODE = E('GMODE', 0)
LN_DIST = E('LN_DIST', 2)
GROWS = 80 * HPI
FINH = E('FINH', 6)
DTOK = (128, 256, 384, 504)
NT = (((1,), (1,)), ((), ()))


def _rb(a):
    return a.astype(BF).astype(F32)


def _kernel(x_hbm, k_hbm, v_hbm, wq_hbm, wo_hbm, wr_hbm, wg_hbm, wu_hbm, wd_hbm,
            o_hbm,
            s0_ref, s1_ref, vt_ref, ot_ref, ot2_ref, acc_ref, qn_ref,
            k_ref, v_ref, wq_ref, wo_ref, xn_ref, g_ref, out_ref, wg_ref, wu_ref, wd_ref,
            x_ref, lr_ref, lr2_ref, xs_ref, rs_ref, wrf_ref, wr_ref, z_ref, idx_ref, sem):
    s_refs = (s0_ref, s1_ref)
    ot_refs = (ot_ref, ot2_ref)
    lr_refs = (lr_ref, lr2_ref)

    SEM_A, SEM_B, SEM_C, SEM_D, SEM_H, SEM_F, SEM_O = range(7)

    def cp_k(h, s=SEM_H):
        return pltpu.make_async_copy(k_hbm.at[h], k_ref.at[h], sem.at[s])

    def cp_v(h, s=SEM_H):
        return pltpu.make_async_copy(v_hbm.at[h], v_ref.at[h], sem.at[s])

    def cp_wq(h, s=SEM_H):
        off = h * DH if isinstance(h, int) else pl.multiple_of(h * DH, DH)
        return pltpu.make_async_copy(wq_hbm.at[:, pl.ds(off, DH)], wq_ref.at[h], sem.at[s])

    def cp_wo(h, s=SEM_H):
        return pltpu.make_async_copy(wo_hbm.at[h], wo_ref.at[h], sem.at[s])

    def cp_x(i, s):
        return pltpu.make_async_copy(x_hbm.at[pl.ds(i * TQ, TQ)], x_ref.at[pl.ds(i * TQ, TQ)], sem.at[s])

    cp_ffn = [pltpu.make_async_copy(wg_hbm, wg_ref, sem.at[SEM_F]),
              pltpu.make_async_copy(wu_hbm, wu_ref, sem.at[SEM_F]),
              pltpu.make_async_copy(wd_hbm, wd_ref, sem.at[SEM_F])]

    cp_wr = pltpu.make_async_copy(wr_hbm, wr_ref, sem.at[SEM_D])

    out_pieces = [(i * TQ, TQ) for i in range(NB - 1)] + [(S - TQ + g * 128, 128) for g in range(NG)]

    def cp_out(j):
        r0, n = out_pieces[j]
        return pltpu.make_async_copy(out_ref.at[pl.ds(r0, n)], o_hbm.at[pl.ds(r0, n)], sem.at[SEM_O])

    def start_head(h):
        cp_k(h).start()
        cp_v(h).start()
        cp_wo(h).start()
        if isinstance(h, int):
            if h + 1 < H:
                cp_wq(h + 1).start()
        else:
            @pl.when(h + 1 < H)
            def _():
                cp_wq(h + 1).start()

    def wait_head(h):
        cp_k(h).wait()
        cp_v(h).wait()
        cp_wo(h).wait()
        if not isinstance(h, int) or h + 1 < H:
            cp_wq(h + 1).wait()

    lane = lax.broadcasted_iota(jnp.int32, (8, 128), 1)
    sub = lax.broadcasted_iota(jnp.int32, (8, 128), 0)

    class Ctx:
        def __init__(self):
            self.z1 = pl.multiple_of(z_ref[0], 8)
            self.z2 = pl.multiple_of(z_ref[1], 8)
            self.zvec = jnp.full((8, 128), z_ref[0], jnp.int32).astype(U32)
            self.hist = []
            self.lnh = []

        def tok(self, a):
            return pltpu.bitcast(a, U32) & self.zvec

        def memtok(self, ref):
            rows = 16 if ref.dtype == BF else 8
            z = pl.multiple_of(self.z2 * 2, 16)
            return self.tok(ref[pl.ds(z, rows), 0:128])

    def dep_bf(a, t):
        if t is None:
            return a
        au = pltpu.bitcast(a, U32)
        first = au[0:8, 0:128] | t
        top = first if au.shape[1] == 128 else jnp.concatenate([first, au[0:8, 128:]], axis=1)
        return pltpu.bitcast(jnp.concatenate([top, au[8:]], axis=0), BF)

    def dep_f32(a, t):
        return pltpu.bitcast(pltpu.bitcast(a, U32) | t, F32)

    class LayerNorm:
        def __init__(self, cx, r0, n, c, lag2, lag3):
            self.cx, self.r0, self.c, self.n = cx, r0, c, n // c
            self.lag2, self.lag3 = lag2, lag3
            self.k = 0
            self.mean, self.inv = {}, {}
            self.steps = self.n + lag3

        def step(self, gate_tok=None):
            cx, c, k = self.cx, self.c, self.k
            self.k += 1
            xv = x_ref.at[pl.ds(pl.multiple_of(cx.z2 * 2, 16), S), :]
            xw = x_ref.at[pl.ds(pl.multiple_of(cx.z1 * 2, 16), S), :]
            xu = x_ref.at[pl.ds(pl.multiple_of((cx.z1 + cx.z2) * 2, 16), S), :]
            if gate_tok is not None:
                x_ref[S:S + 16, 0:128] = pltpu.bitcast(cx.tok(gate_tok), BF)
            if k < self.n:
                a = self.r0 + k * c
                self.mean[k] = jnp.mean(xv[a:a + c, :].astype(F32), axis=-1, keepdims=True)
            j = k - self.lag2
            if 0 <= j < self.n:
                a = self.r0 + j * c
                xc = xw[a:a + c, :].astype(F32) - self.mean[j]
                v = _rb(_rb(jnp.mean(xc * xc, axis=-1, keepdims=True)) + 1e-5)
                den = _rb(v * lax.rsqrt(v))
                inv = pl.reciprocal(den, approx=True)
                self.inv[j] = inv * (2.0 - den * inv)
            j = k - self.lag3
            if 0 <= j < self.n:
                a = self.r0 + j * c
                d = _rb(xu[a:a + c, :].astype(F32) - _rb(self.mean[j]))
                xn_ref[a:a + c, :] = (d * self.inv[j]).astype(BF)

    def silu(b):
        hb = 0.5 * b
        return hb + hb * jnp.tanh(hb)

    def gate(r0, n):
        xf = xn_ref[pl.ds(r0, n), :].astype(F32)
        g_ref[pl.ds(r0, n), :] = silu(xf)
        return xf

    def router(cx, r0, n, rc, gate_tok=None):
        xv = xn_ref.at[pl.ds(pl.multiple_of(cx.z2 * 2, 16), S), :]
        if gate_tok is not None:
            xn_ref[S:S + 16, 0:128] = pltpu.bitcast(cx.tok(gate_tok), BF)
        for c in range(n // RC_):
            a = r0 + c * RC_
            xf = xv[a:a + RC_, :].astype(F32)
            r = _rb(jnp.sum(xf * jnp.concatenate([wrf_ref[...]] * (RC_ // 8), axis=0), axis=-1, keepdims=True))
            for j in range(RC_ // 8):
                gi = a // 8 + j
                rc[gi // 128] = jnp.where(lane == gi % 128, r[j * 8:(j + 1) * 8, :], rc[gi // 128])

    def route(rc):
        r = jnp.concatenate(rc, axis=0)
        tix = jnp.concatenate([(8 * (128 * a + lane) + sub) for a in range(2)], axis=0).astype(F32)
        rw = jnp.where(r != r, -jnp.inf, r)
        alive = jnp.ones((16, 128), F32)
        for j in range(C):
            mx = jnp.max(jnp.max(rw, axis=0, keepdims=True), axis=1, keepdims=True)
            cand = jnp.where((rw == mx) & (alive > 0), tix, float(S - 1))
            ixv = jnp.min(jnp.min(cand, axis=0, keepdims=True), axis=1, keepdims=True)
            hit = tix == ixv
            rsel = jnp.sum(jnp.sum(jnp.where(hit, r, 0.0), axis=0, keepdims=True), axis=1, keepdims=True)
            rw = jnp.where(hit, -jnp.inf, rw)
            alive = jnp.where(hit, 0.0, alive)
            ix = ixv.astype(jnp.int32)[0, 0]
            idx_ref[j] = ix
            blk = xn_ref[pl.ds(pl.multiple_of((ix // 16) * 16, 16), 16), :].astype(F32)
            pick = lax.broadcasted_iota(jnp.int32, (16, D), 0) == (ixv.astype(jnp.int32) & 15)
            xs_ref[j:j + 1, :] = jnp.sum(jnp.where(pick, blk, 0.0), axis=0, keepdims=True)
            rs_ref[j:j + 1, :] = jnp.broadcast_to(rsel, (1, 128))

    FT = [(f0, min(128, F - f0)) for f0 in range(0, F, 128)]

    class Ffn:
        def __init__(self):
            self.xs = xs_ref[...].astype(BF)
            self.acc = {}
            self.up = [(w, i, k) for i in range(len(FT)) for w in (0, 1) for k in range(D // 128)]
            self.down = [(i, k) for k in range(D // 128) for i in range(len(FT))]
            self.hid = None

        def add(self, key, d):
            self.acc[key] = d if key not in self.acc else self.acc[key] + d

        def run_up(self, n):
            for _ in range(min(n, len(self.up))):
                w, i, k = self.up.pop(0)
                f0, fn = FT[i]
                wt = (wg_ref, wu_ref)[w][f0:f0 + fn, k * 128:(k + 1) * 128]
                self.add((w, i), lax.dot_general(self.xs[:, k * 128:(k + 1) * 128], wt, NT, preferred_element_type=F32))

        def run_down(self, n):
            if self.hid is None:
                self.run_up(len(self.up))
                self.hid = []
                for i in range(len(FT)):
                    g = _rb(self.acc[(0, i)])
                    g = _rb(g * jax.nn.sigmoid(g))
                    self.hid.append((g * _rb(self.acc[(1, i)])).astype(BF))
            for _ in range(min(n, len(self.down))):
                i, k = self.down.pop(0)
                f0, fn = FT[i]
                self.add((2, k), jnp.dot(self.hid[i], wd_ref[f0:f0 + fn, k * 128:(k + 1) * 128], preferred_element_type=F32))

        def finish(self):
            self.run_down(len(self.down))
            y = _rb(jnp.concatenate([self.acc[(2, k)] for k in range(D // 128)], axis=1))
            y = _rb(y * _rb(jax.nn.sigmoid(rs_ref[:, 0:1])))
            b = _rb(xs_ref[...] + y)
            gs = b * jax.nn.sigmoid(b)
            for j in range(C):
                g_ref[pl.ds(idx_ref[j], 1), :] = gs[j:j + 1, :]

    def qproj(i, h, split=1, t=None, cx=None):
        parts = []
        n = TQ // split
        for c in range(split):
            r0 = i * TQ + c * n
            xn = dep_bf(xn_ref[r0:r0 + n, :], t)
            d = jnp.dot(xn, wq_ref[h], preferred_element_type=F32)
            if cx is not None:
                for r in ATOK:
                    cx.hist.append(d[r:r + 8, :])
            parts.append((d * QSCALE).astype(BF))
        return parts[0] if split == 1 else jnp.concatenate(parts, axis=0)

    def transpose_v(cx, hh, h):
        vt_ref[hh, pl.ds(cx.z1, DH // 2), :] = pltpu.bitcast(v_ref[h].T, U32)

    def qk(cx, n, h, q, jobs=(), after=(), ticks=None):
        sv = s_refs[n % 2].at[pl.ds(cx.z1, S), :]
        ns = max(len(jobs) + 1, len(after))
        if ticks is not None:
            ns = TSL
        sl = S // ns
        m = None
        for j in range(ns):
            t = jobs[j - 1]() if 0 < j <= len(jobs) else None
            kj = dep_bf(k_ref[h, j * sl:(j + 1) * sl, :], t)
            sT = lax.dot_general(kj, q, NT, preferred_element_type=F32)
            sv[j * sl:(j + 1) * sl, :] = sT
            mj = jnp.max(jnp.max(sT.reshape(sl // 128, 16, 8, TQ), axis=1), axis=0)
            m = mj if m is None else jnp.maximum(m, mj)
            if j < len(after) and after[j] is not None:
                after[j](sT[0:8, 0:128])
            for fn, cnt_, off, span in (ticks or ()):
                for i in range(cnt_):
                    r = (off + i * (span - off) // cnt_) // 8 * 8 - j * sl
                    if 0 <= r < sl:
                        fn(sT[r:r + 8, 0:128])
        return jnp.broadcast_to(jnp.max(m, axis=0, keepdims=True), (8, TQ))

    def pv(cx, n, hh, m, hooks=None, groups=tuple(range(NG)), after=None, buf=0):
        sv = s_refs[n % 2].at[pl.ds(cx.z2, S), :]
        vv = vt_ref.at[hh, pl.ds(cx.z2, DH // 2), :]
        otv = ot_refs[buf].at[pl.ds(cx.z1, NG * DH), :]
        lrv = lr_refs[buf].at[pl.ds(cx.z1, NG * 8), :]
        CT = PV_CT
        for g in groups:
            mg = m[:, g * 128:(g + 1) * 128]
            l8 = None
            oT = None
            for c in range(S // 128 // CT):
                mc = mg
                if len(cx.hist) >= PV_DIST:
                    mc = dep_f32(mc, cx.tok(cx.hist[-PV_DIST]))
                if hooks and (g * 4 + c) in hooks:
                    mc = dep_f32(mc, hooks[g * 4 + c])
                ps = []
                for tt in range(CT):
                    r0 = (c * CT + tt) * 128
                    s = sv[r0:r0 + 128, g * 128:(g + 1) * 128]
                    p = jnp.exp2(s - jnp.concatenate([mc] * 16, axis=0))
                    lt = None
                    for j in reversed(range(16)):
                        pj = p[j * 8:(j + 1) * 8, :]
                        lt = pj if lt is None else lt + pj
                    l8 = lt if l8 is None else l8 + lt
                    ps.append(p)
                vT = pltpu.bitcast(vv[:, c * CT * 128:(c + 1) * CT * 128], BF)
                part = jnp.dot(vT, jnp.concatenate(ps, axis=0).astype(BF), preferred_element_type=F32)
                cx.hist.append(part[0:8, :])
                if after and (g * 4 + c) in after:
                    after[g * 4 + c](part[0:8, :])
                oT = part if oT is None else oT + part
            otv[g * DH:(g + 1) * DH, :] = oT
            lrv[g * 8:(g + 1) * 8, :] = l8

    def load_o(cx, groups, buf=0):
        otv = ot_refs[buf].at[pl.ds(cx.z2, NG * DH), :]
        lrv = lr_refs[buf].at[pl.ds(cx.z2, NG * 8), :]
        parts = []
        for g in groups:
            l = jnp.sum(lrv[g * 8:(g + 1) * 8, :], axis=0, keepdims=True)
            parts.append((otv[g * DH:(g + 1) * DH, :] * (1.0 / l)).T.astype(BF))
        return parts[0] if len(parts) == 1 else jnp.concatenate(parts, axis=0)

    def oproj(cx, i, h, mode, groups=tuple(range(NG)), toks=True, o=None):
        r0 = i * TQ + groups[0] * 128
        r1 = r0 + len(groups) * 128
        if o is None:
            o = load_o(cx, groups)
        d = jnp.dot(o, wo_ref[h], preferred_element_type=F32)
        if mode == 'set':
            acc_ref[r0:r1, :] = d
        elif mode == 'add':
            acc_ref[r0:r1, :] += d
        else:
            s = acc_ref[r0:r1, :] + d
            out_ref[r0:r1, :] = (x_ref[r0:r1, :].astype(F32) + s * g_ref[r0:r1, :]).astype(BF)
        if toks:
            for r in DTOK:
                cx.hist.append(d[r:r + 8, 0:128])

    cp_x(0, SEM_A).start()
    cp_wq(0, SEM_A).start()
    cp_k(0, SEM_B).start()
    cp_x(1, SEM_B).start()
    cp_v(0, SEM_C).start()
    cp_x(2, SEM_D).start()
    cp_x(3, SEM_D).start()
    cp_wo(0, SEM_D).start()
    cp_wq(1, SEM_D).start()
    cp_wr.start()
    z_ref[0] = 0
    z_ref[1] = 0
    acc_ref[S - TQ:, :] = jnp.zeros((TQ, D), F32)

    def hide(i, c):
        z_ref[1] = z_ref[0] * i
        z_ref[0] = z_ref[1] * i
        return c

    lax.fori_loop(0, 2, hide, 0)
    cx = Ctx()
    rc = [jnp.zeros((8, 128), F32), jnp.zeros((8, 128), F32)]

    if LASTONLY:
        start_head(H - 1)
        for c in cp_ffn:
            c.start()
        def _b(i, c_):
            z_ref[1] = z_ref[0] * i
            z_ref[0] = z_ref[1] * i
            return c_
        lax.fori_loop(0, 3, _b, 0)
    elif LOOPONLY:
        start_head(1)
        for c in cp_ffn:
            c.start()
    else:
        cp_x(0, SEM_A).wait()
        cp_wq(0, SEM_A).wait()
        ln = LayerNorm(cx, 0, TQ, L0C, L0A, L0B)
        for _ in range(ln.steps):
            ln.step()
        q = qproj(0, 0, split=4)
        cp_k(0, SEM_B).wait()
        cp_x(1, SEM_B).wait()
        for hh in range(HPI):
            start_head(1 + hh)
        def hold_o(t):
            ot_ref[NG * DH:NG * DH + 8, :] = pltpu.bitcast(cx.tok(t), F32)

        ogate = [(hold_o, 1, OGT, OGT + 8)] if OGT else []
        for n in range(NB):
            if n == 1:
                cp_x(2, SEM_D).wait()
                cp_x(3, SEM_D).wait()
                cp_wo(0, SEM_D).wait()
                cp_wq(1, SEM_D).wait()
                cp_wr.wait()
                wrf_ref[...] = jnp.broadcast_to(wr_ref[...].astype(F32).reshape(1, D), (8, D))
                for c in cp_ffn:
                    c.start()
            if n + 1 < NB:
                ln = LayerNorm(cx, (n + 1) * TQ, TQ, LNC, LAG2, LAG3)
                if n == 0:
                    ln.step()
                    m = qk(cx, n, 0, q, ticks=[(ln.step, ln.steps - 1, 0, LSPAN0)])
                else:
                    m = qk(cx, n, 0, q, ticks=[(ln.step, ln.steps, LOFF, LSPAN)] + ogate)
            else:
                rn = S // RJOB
                st = [0]

                def rstep(t=None):
                    router(cx, st[0] * rn, rn, rc, t)
                    st[0] += 1

                m = qk(cx, n, 0, q, ticks=[(rstep, RJOB, ROFF, RSPAN)] + ogate)
                route(rc)
            if n == 0:
                cp_v(0, SEM_C).wait()
                transpose_v(cx, 0, 0)
                q = qproj(1, 0)
            elif n + 1 < NB:
                if DA:
                    oproj(cx, n - 1, 0, 'set', toks=False)
                    q = qproj(n + 1, 0, cx=cx)
                else:
                    q = qproj(n + 1, 0)
                    oproj(cx, n - 1, 0, 'set')
            else:
                q = qproj(0, 1)
                oproj(cx, n - 1, 0, 'set')
            pv(cx, n, 0, m, {RTH: cx.memtok(xs_ref) | cx.memtok(rs_ref)} if n + 1 == NB else None)
        qn_ref[...] = pltpu.bitcast(q, U32)

        if ONLYF:
            wait_head(1)
            for c in cp_ffn:
                c.wait()
            def _c(i, c_):
                o8 = pl.multiple_of(i * 16, 16)
                f = lambda r: r[pl.ds(o8, 16), 0:128].astype(BF)
                out_ref[0:16, 0:128] = (pltpu.bitcast(qn_ref[pl.ds(o8, 8), :], BF) + f(ot_ref) + f(acc_ref) + f(xn_ref) + f(lr_ref)
                                        + (xs_ref[:, 0:128] + rs_ref[...])[0:1].astype(BF) + idx_ref[i].astype(BF))
                return c_
            lax.fori_loop(0, 2, _c, 0)
            cp_out(3).start()
            cp_out(3).wait()
            return
    if not LASTONLY:
        def body(it, _):
            h0 = 1 + it * HPI
            for hh in range(HPI):
                wait_head(h0 + hh)
            for hh in range(HPI):
                if hh == 0:
                    start_head(h0 + HPI)
                else:
                    @pl.when(h0 + HPI + hh < H)
                    def _():
                        start_head(h0 + HPI + hh)
            cx = Ctx()
            for hh in range(HPI):
                transpose_v(cx, hh, h0 + hh)
            q = pltpu.bitcast(qn_ref[...], BF)
            h_prev = h0 - 1
            for n in range(HPI * NB):
                hh, i = divmod(n, NB)
                hn, in_ = divmod(n + 1, NB)
                jobs = ()
                if n == GUN:
                    gate(pl.multiple_of(jnp.minimum(it * GROWS, S - GROWS), 16), GROWS)
                if n == 0 and AFIRST:
                    q_next = qproj(in_, h0 + hn)
                    m = qk(cx, n, h0 + hh, q, jobs)
                    q = q_next
                else:
                    m = qk(cx, n, h0 + hh, q, jobs)
                    q = qproj(in_, h0 + hn)
                oproj(cx, (i - 1) % NB, h_prev, 'add')
                pv(cx, n, hh, m)
                h_prev = h0 + hh
            qn_ref[...] = pltpu.bitcast(q, U32)
            return 0

        lax.fori_loop(0, (H - 2) // HPI, body, 0)

    h = H - 1
    wait_head(h)
    for c in cp_ffn:
        c.wait()
    if LOOPONLY:
        out_ref[0:16, 0:128] = pltpu.bitcast(qn_ref[0:8, :], BF) + ot_ref[0:16, :].astype(BF) + acc_ref[0:16, 0:128].astype(BF) + g_ref[0:16, 0:128].astype(BF)
        cp_out(3).start()
        cp_out(3).wait()
        return
    cx = Ctx()
    transpose_v(cx, 0, h)
    q = pltpu.bitcast(qn_ref[...], BF)
    ffn = Ffn()
    cnt = lambda tot, j: (tot * (j + 1)) // (FSL - 1) - (tot * j) // (FSL - 1)
    m = qk(cx, 0, h, q, after=[(lambda t, j=j: ffn.run_up(cnt(70, j))) for j in range(FSL - 1)] + [None])
    q = qproj(1, h)
    oproj(cx, NB - 1, h - 1, 'add')
    pv(cx, 0, 0, m)
    m = qk(cx, 1, h, q, after=[(lambda t, j=j: ffn.run_up(cnt(70, j))) for j in range(FSL - 1)] + [None])
    q = qproj(2, h, cx=cx)
    pv(cx, 1, 0, m, buf=1)
    m = qk(cx, 2, h, q, after=[(lambda t, j=j: ffn.run_down(cnt(70, j))) for j in range(FSL - 1)] + [None])
    ffn.finish()
    q = qproj(3, h, t=None)
    allg = tuple(range(NG))
    oproj(cx, 0, h, 'fin', toks=False)
    cp_out(0).start()
    oproj(cx, 1, h, 'fin', o=load_o(cx, allg, 1))
    cp_out(1).start()
    pv(cx, 2, 0, m, {FINH: cx.memtok(out_ref)})
    m = qk(cx, 3, h, q)
    oproj(cx, 2, h, 'fin')
    cp_out(2).start()

    def alltok(o):
        u = pltpu.bitcast(o, U32)
        t = u[0:8]
        for r in range(8, u.shape[0], 8):
            t = t | u[r:r + 8]
        return t & cx.zvec

    pv(cx, NB - 1, 0, m, {FINH: cx.memtok(out_ref)}, groups=(0, 1))
    os = [load_o(cx, (0,)), load_o(cx, (1,))]
    pv(cx, NB - 1, 0, m, groups=(2,))
    os.append(load_o(cx, (2,)))
    pv(cx, NB - 1, 0, m, {TAILH: alltok(os[0]) | alltok(os[1])} if TAILH else None, groups=(3,))
    os.append(load_o(cx, (3,)))
    for g in range(NG):
        oproj(cx, NB - 1, h, 'fin', groups=(g,), toks=False, o=os[g])
        cp_out(NB - 1 + g).start()
    for j in range(len(out_pieces)):
        cp_out(j).wait()


@jax.jit
def pallas_recurrent_scan__mha_block_cached__moe_arch_mod__prompt_kernel(
    A_x, A_k_cache, A_v_cache, A_wq, A_wo, B_x, B_w_r, B_w_gate, B_w_up, B_w_down):
    x = A_x.reshape(S, D)
    k = A_k_cache.reshape(H, S, DH)
    v = A_v_cache.reshape(H, S, DH)
    wo = A_wo.reshape(H, DH, D)
    wr = B_w_r
    anyspec = pl.BlockSpec(memory_space=pl.ANY)
    out = pl.pallas_call(
        _kernel,
        in_specs=[anyspec] * 9,
        out_specs=anyspec,
        out_shape=jax.ShapeDtypeStruct((S, D), BF),
        scratch_shapes=[
            pltpu.VMEM((S, TQ), F32),
            pltpu.VMEM((S, TQ), F32),
            pltpu.VMEM((HPI, DH // 2, S), U32),
            pltpu.VMEM((NG * DH + 32, 128), F32),
            pltpu.VMEM((NG * DH, 128), F32),
            pltpu.VMEM((S, D), F32),
            pltpu.VMEM((TQ // 2, DH), U32),
            pltpu.VMEM((H, S, DH), BF),
            pltpu.VMEM((H, S, DH), BF),
            pltpu.VMEM((H, D, DH), BF),
            pltpu.VMEM((H, DH, D), BF),
            pltpu.VMEM((S + 64, D), BF),
            pltpu.VMEM((S, D), F32),
            pltpu.VMEM((S, D), BF),
            pltpu.VMEM((F, D), BF),
            pltpu.VMEM((F, D), BF),
            pltpu.VMEM((F, D), BF),
            pltpu.VMEM((S + 64, D), BF),
            pltpu.VMEM((NG * 8, 128), F32),
            pltpu.VMEM((NG * 8, 128), F32),
            pltpu.VMEM((C, D), F32),
            pltpu.VMEM((C, 128), F32),
            pltpu.VMEM((8, D), F32),
            pltpu.VMEM((D,), BF),
            pltpu.SMEM((2,), jnp.int32),
            pltpu.SMEM((C,), jnp.int32),
            pltpu.SemaphoreType.DMA((7,)),
        ],
        compiler_params=pltpu.CompilerParams(
            vmem_limit_bytes=126 * 1024 * 1024,
            internal_scratch_in_bytes=16 * 4096,
            disable_bounds_checks=True,
            disable_semaphore_checks=True,
        ),
    )(x, k, v, A_wq, wo, wr, B_w_gate.T, B_w_up.T, B_w_down)
    return out.reshape(1, S, D)
```

```python
import math
import jax
import jax.numpy as jnp
from jax import lax
import jax.experimental.pallas as pl
import jax.experimental.pallas.tpu as pltpu

S, D, H, DH, F, C = 2048, 640, 32, 128, 1728, 8
TQ = 512
NB = S // TQ
NG = TQ // 128
BF = jnp.bfloat16
F32 = jnp.float32
U32 = jnp.uint32
QSCALE = (DH ** -0.5) * math.log2(math.e)
E = lambda k, d: d
PV_CT = 4
PV_DIST = E('PV_DIST', 3)
HPI = E('HPI', 1)
LNC = E('LNC', 8)
RC_ = 16
RJOB = E('RJOB', 32)
RSPAN = E('RSPAN', 1900)
LAG2 = E('LAG2', 4)
TSL = E('TSL', 1)
LAG3 = E('LAG3', 10)
LOFF = E('LOFF', 0)
ROFF = E('ROFF', 0)
DA = E('DA', 0)
QT = E('QT', 1)
QTH = E('QTH', 4)
OGT = E('OGT', 0)
LSPAN0 = E('LSPAN0', 2000)
LSPAN = E('LSPAN', 2040)
L0C = E('L0C', 32)
L0A = E('L0A', 0)
L0B = E('L0B', 0)
ATOK = ()
NJOB = E('NJOB', 8)
AFIRST = E('AFIRST', 0)
ONLYF = E('ONLYF', 0)
TAILH = E('TAILH', 0)
FSL = E('FSL', 16)
FH0 = E('FH0', 9)
RTH = E('RTH', 12)
LASTONLY = E('LASTONLY', 0)
LOOPONLY = E('LOOPONLY', 0)
GSPL = E('GSPL', 1)
GUN = E('GUN', 1)
GMODE = E('GMODE', 0)
LN_DIST = E('LN_DIST', 2)
GROWS = 80 * HPI
FINH = E('FINH', 6)
DTOK = (128, 256, 384, 504)
NT = (((1,), (1,)), ((), ()))


def _rb(a):
    return a.astype(BF).astype(F32)


def _kernel(x_hbm, k_hbm, v_hbm, wq_hbm, wo_hbm, wr_hbm, wg_hbm, wu_hbm, wd_hbm,
            o_hbm,
            s0_ref, s1_ref, vt_ref, ot_ref, ot2_ref, acc_ref, qn_ref,
            k_ref, v_ref, wq_ref, wo_ref, xn_ref, g_ref, out_ref, wg_ref, wu_ref, wd_ref,
            x_ref, lr_ref, lr2_ref, xs_ref, rs_ref, wrf_ref, wr_ref, z_ref, idx_ref, sem):
    s_refs = (s0_ref, s1_ref)
    ot_refs = (ot_ref, ot2_ref)
    lr_refs = (lr_ref, lr2_ref)

    SEM_A, SEM_B, SEM_C, SEM_D, SEM_H, SEM_F, SEM_O = range(7)

    def cp_k(h, s=SEM_H):
        return pltpu.make_async_copy(k_hbm.at[h], k_ref.at[h], sem.at[s])

    def cp_v(h, s=SEM_H):
        return pltpu.make_async_copy(v_hbm.at[h], v_ref.at[h], sem.at[s])

    def cp_wq(h, s=SEM_H):
        off = h * DH if isinstance(h, int) else pl.multiple_of(h * DH, DH)
        return pltpu.make_async_copy(wq_hbm.at[:, pl.ds(off, DH)], wq_ref.at[h], sem.at[s])

    def cp_wo(h, s=SEM_H):
        return pltpu.make_async_copy(wo_hbm.at[h], wo_ref.at[h], sem.at[s])

    def cp_x(i, s):
        return pltpu.make_async_copy(x_hbm.at[pl.ds(i * TQ, TQ)], x_ref.at[pl.ds(i * TQ, TQ)], sem.at[s])

    cp_ffn = [pltpu.make_async_copy(wg_hbm, wg_ref, sem.at[SEM_F]),
              pltpu.make_async_copy(wu_hbm, wu_ref, sem.at[SEM_F]),
              pltpu.make_async_copy(wd_hbm, wd_ref, sem.at[SEM_F])]

    cp_wr = pltpu.make_async_copy(wr_hbm, wr_ref, sem.at[SEM_D])

    out_pieces = [(i * TQ, TQ) for i in range(NB - 1)] + [(S - TQ + g * 128, 128) for g in range(NG)]

    def cp_out(j):
        r0, n = out_pieces[j]
        return pltpu.make_async_copy(out_ref.at[pl.ds(r0, n)], o_hbm.at[pl.ds(r0, n)], sem.at[SEM_O])

    def start_head(h):
        cp_k(h).start()
        cp_v(h).start()
        cp_wo(h).start()
        if isinstance(h, int):
            if h + 1 < H:
                cp_wq(h + 1).start()
        else:
            @pl.when(h + 1 < H)
            def _():
                cp_wq(h + 1).start()

    def wait_head(h):
        cp_k(h).wait()
        cp_v(h).wait()
        cp_wo(h).wait()
        if not isinstance(h, int) or h + 1 < H:
            cp_wq(h + 1).wait()

    lane = lax.broadcasted_iota(jnp.int32, (8, 128), 1)
    sub = lax.broadcasted_iota(jnp.int32, (8, 128), 0)

    class Ctx:
        def __init__(self):
            self.z1 = pl.multiple_of(z_ref[0], 8)
            self.z2 = pl.multiple_of(z_ref[1], 8)
            self.zvec = jnp.full((8, 128), z_ref[0], jnp.int32).astype(U32)
            self.hist = []
            self.lnh = []

        def tok(self, a):
            return pltpu.bitcast(a, U32) & self.zvec

        def memtok(self, ref):
            rows = 16 if ref.dtype == BF else 8
            z = pl.multiple_of(self.z2 * 2, 16)
            return self.tok(ref[pl.ds(z, rows), 0:128])

    def dep_bf(a, t):
        if t is None:
            return a
        au = pltpu.bitcast(a, U32)
        first = au[0:8, 0:128] | t
        top = first if au.shape[1] == 128 else jnp.concatenate([first, au[0:8, 128:]], axis=1)
        return pltpu.bitcast(jnp.concatenate([top, au[8:]], axis=0), BF)

    def dep_f32(a, t):
        return pltpu.bitcast(pltpu.bitcast(a, U32) | t, F32)

    class LayerNorm:
        def __init__(self, cx, r0, n, c, lag2, lag3):
            self.cx, self.r0, self.c, self.n = cx, r0, c, n // c
            self.lag2, self.lag3 = lag2, lag3
            self.k = 0
            self.mean, self.inv = {}, {}
            self.steps = self.n + lag3

        def step(self, gate_tok=None):
            cx, c, k = self.cx, self.c, self.k
            self.k += 1
            xv = x_ref.at[pl.ds(pl.multiple_of(cx.z2 * 2, 16), S), :]
            xw = x_ref.at[pl.ds(pl.multiple_of(cx.z1 * 2, 16), S), :]
            xu = x_ref.at[pl.ds(pl.multiple_of((cx.z1 + cx.z2) * 2, 16), S), :]
            if gate_tok is not None:
                x_ref[S:S + 16, 0:128] = pltpu.bitcast(cx.tok(gate_tok), BF)
            if k < self.n:
                a = self.r0 + k * c
                self.mean[k] = jnp.mean(xv[a:a + c, :].astype(F32), axis=-1, keepdims=True)
            j = k - self.lag2
            if 0 <= j < self.n:
                a = self.r0 + j * c
                xc = xw[a:a + c, :].astype(F32) - self.mean[j]
                v = _rb(_rb(jnp.mean(xc * xc, axis=-1, keepdims=True)) + 1e-5)
                den = _rb(v * lax.rsqrt(v))
                inv = pl.reciprocal(den, approx=True)
                self.inv[j] = inv * (2.0 - den * inv)
            j = k - self.lag3
            if 0 <= j < self.n:
                a = self.r0 + j * c
                d = _rb(xu[a:a + c, :].astype(F32) - _rb(self.mean[j]))
                xn_ref[a:a + c, :] = (d * self.inv[j]).astype(BF)

    def silu(b):
        hb = 0.5 * b
        return hb + hb * jnp.tanh(hb)

    def gate(r0, n):
        xf = xn_ref[pl.ds(r0, n), :].astype(F32)
        g_ref[pl.ds(r0, n), :] = silu(xf)
        return xf

    def router(cx, r0, n, rc, gate_tok=None):
        xv = xn_ref.at[pl.ds(pl.multiple_of(cx.z2 * 2, 16), S), :]
        if gate_tok is not None:
            xn_ref[S:S + 16, 0:128] = pltpu.bitcast(cx.tok(gate_tok), BF)
        for c in range(n // RC_):
            a = r0 + c * RC_
            xf = xv[a:a + RC_, :].astype(F32)
            r = _rb(jnp.sum(xf * jnp.concatenate([wrf_ref[...]] * (RC_ // 8), axis=0), axis=-1, keepdims=True))
            for j in range(RC_ // 8):
                gi = a // 8 + j
                rc[gi // 128] = jnp.where(lane == gi % 128, r[j * 8:(j + 1) * 8, :], rc[gi // 128])

    def route(rc):
        r = jnp.concatenate(rc, axis=0)
        tix = jnp.concatenate([(8 * (128 * a + lane) + sub) for a in range(2)], axis=0).astype(F32)
        rw = jnp.where(r != r, -jnp.inf, r)
        alive = jnp.ones((16, 128), F32)
        for j in range(C):
            mx = jnp.max(jnp.max(rw, axis=0, keepdims=True), axis=1, keepdims=True)
            cand = jnp.where((rw == mx) & (alive > 0), tix, float(S - 1))
            ixv = jnp.min(jnp.min(cand, axis=0, keepdims=True), axis=1, keepdims=True)
            hit = tix == ixv
            rsel = jnp.sum(jnp.sum(jnp.where(hit, r, 0.0), axis=0, keepdims=True), axis=1, keepdims=True)
            rw = jnp.where(hit, -jnp.inf, rw)
            alive = jnp.where(hit, 0.0, alive)
            ix = ixv.astype(jnp.int32)[0, 0]
            idx_ref[j] = ix
            blk = xn_ref[pl.ds(pl.multiple_of((ix // 16) * 16, 16), 16), :].astype(F32)
            pick = lax.broadcasted_iota(jnp.int32, (16, D), 0) == (ixv.astype(jnp.int32) & 15)
            xs_ref[j:j + 1, :] = jnp.sum(jnp.where(pick, blk, 0.0), axis=0, keepdims=True)
            rs_ref[j:j + 1, :] = jnp.broadcast_to(rsel, (1, 128))

    FT = [(f0, min(128, F - f0)) for f0 in range(0, F, 128)]

    class Ffn:
        def __init__(self):
            self.xs = xs_ref[...].astype(BF)
            self.acc = {}
            self.up = [(w, i, k) for i in range(len(FT)) for w in (0, 1) for k in range(D // 128)]
            self.down = [(i, k) for k in range(D // 128) for i in range(len(FT))]
            self.hid = None

        def add(self, key, d):
            self.acc[key] = d if key not in self.acc else self.acc[key] + d

        def run_up(self, n):
            for _ in range(min(n, len(self.up))):
                w, i, k = self.up.pop(0)
                f0, fn = FT[i]
                wt = (wg_ref, wu_ref)[w][f0:f0 + fn, k * 128:(k + 1) * 128]
                self.add((w, i), lax.dot_general(self.xs[:, k * 128:(k + 1) * 128], wt, NT, preferred_element_type=F32))

        def run_down(self, n):
            if self.hid is None:
                self.run_up(len(self.up))
                self.hid = []
                for i in range(len(FT)):
                    g = _rb(self.acc[(0, i)])
                    g = _rb(g * jax.nn.sigmoid(g))
                    self.hid.append((g * _rb(self.acc[(1, i)])).astype(BF))
            for _ in range(min(n, len(self.down))):
                i, k = self.down.pop(0)
                f0, fn = FT[i]
                self.add((2, k), jnp.dot(self.hid[i], wd_ref[f0:f0 + fn, k * 128:(k + 1) * 128], preferred_element_type=F32))

        def finish(self):
            self.run_down(len(self.down))
            y = _rb(jnp.concatenate([self.acc[(2, k)] for k in range(D // 128)], axis=1))
            y = _rb(y * _rb(jax.nn.sigmoid(rs_ref[:, 0:1])))
            b = _rb(xs_ref[...] + y)
            gs = b * jax.nn.sigmoid(b)
            for j in range(C):
                g_ref[pl.ds(idx_ref[j], 1), :] = gs[j:j + 1, :]

    def qproj(i, h, split=1, t=None, cx=None):
        parts = []
        n = TQ // split
        for c in range(split):
            r0 = i * TQ + c * n
            xn = dep_bf(xn_ref[r0:r0 + n, :], t)
            d = jnp.dot(xn, wq_ref[h], preferred_element_type=F32)
            if cx is not None:
                for r in ATOK:
                    cx.hist.append(d[r:r + 8, :])
            parts.append((d * QSCALE).astype(BF))
        return parts[0] if split == 1 else jnp.concatenate(parts, axis=0)

    def transpose_v(cx, hh, h):
        vt_ref[hh, pl.ds(cx.z1, DH // 2), :] = pltpu.bitcast(v_ref[h].T, U32)

    def qk(cx, n, h, q, jobs=(), after=(), ticks=None, qt=False):
        sv = s_refs[n % 2].at[pl.ds(cx.z1, S), :]
        ns = max(len(jobs) + 1, len(after))
        if ticks is not None:
            ns = TSL
        sl = S // ns
        m = None
        for j in range(ns):
            t = jobs[j - 1]() if 0 < j <= len(jobs) else None
            kj = dep_bf(k_ref[h, j * sl:(j + 1) * sl, :], t)
            if qt:
                sT = jnp.dot(kj, q, preferred_element_type=F32)
            else:
                sT = lax.dot_general(kj, q, NT, preferred_element_type=F32)
            sv[j * sl:(j + 1) * sl, :] = sT
            mj = jnp.max(jnp.max(sT.reshape(sl // 128, 16, 8, TQ), axis=1), axis=0)
            m = mj if m is None else jnp.maximum(m, mj)
            if j < len(after) and after[j] is not None:
                after[j](sT[0:8, 0:128])
            for fn, cnt_, off, span in (ticks or ()):
                for i in range(cnt_):
                    r = (off + i * (span - off) // cnt_) // 8 * 8 - j * sl
                    if 0 <= r < sl:
                        fn(sT[r:r + 8, 0:128])
        return jnp.broadcast_to(jnp.max(m, axis=0, keepdims=True), (8, TQ))

    def pv(cx, n, hh, m, hooks=None, groups=tuple(range(NG)), after=None, buf=0):
        sv = s_refs[n % 2].at[pl.ds(cx.z2, S), :]
        vv = vt_ref.at[hh, pl.ds(cx.z2, DH // 2), :]
        otv = ot_refs[buf].at[pl.ds(cx.z1, NG * DH), :]
        lrv = lr_refs[buf].at[pl.ds(cx.z1, NG * 8), :]
        CT = PV_CT
        for g in groups:
            mg = m[:, g * 128:(g + 1) * 128]
            l8 = None
            oT = None
            for c in range(S // 128 // CT):
                mc = mg
                if len(cx.hist) >= PV_DIST:
                    mc = dep_f32(mc, cx.tok(cx.hist[-PV_DIST]))
                if hooks and (g * 4 + c) in hooks:
                    mc = dep_f32(mc, hooks[g * 4 + c])
                ps = []
                for tt in range(CT):
                    r0 = (c * CT + tt) * 128
                    s = sv[r0:r0 + 128, g * 128:(g + 1) * 128]
                    p = jnp.exp2(s - jnp.concatenate([mc] * 16, axis=0))
                    lt = None
                    for j in reversed(range(16)):
                        pj = p[j * 8:(j + 1) * 8, :]
                        lt = pj if lt is None else lt + pj
                    l8 = lt if l8 is None else l8 + lt
                    ps.append(p)
                vT = pltpu.bitcast(vv[:, c * CT * 128:(c + 1) * CT * 128], BF)
                part = jnp.dot(vT, jnp.concatenate(ps, axis=0).astype(BF), preferred_element_type=F32)
                cx.hist.append(part[0:8, :])
                if after and (g * 4 + c) in after:
                    after[g * 4 + c](part[0:8, :])
                oT = part if oT is None else oT + part
            otv[g * DH:(g + 1) * DH, :] = oT
            lrv[g * 8:(g + 1) * 8, :] = l8

    def load_o(cx, groups, buf=0):
        otv = ot_refs[buf].at[pl.ds(cx.z2, NG * DH), :]
        lrv = lr_refs[buf].at[pl.ds(cx.z2, NG * 8), :]
        parts = []
        for g in groups:
            l = jnp.sum(lrv[g * 8:(g + 1) * 8, :], axis=0, keepdims=True)
            parts.append((otv[g * DH:(g + 1) * DH, :] * (1.0 / l)).T.astype(BF))
        return parts[0] if len(parts) == 1 else jnp.concatenate(parts, axis=0)

    def oproj(cx, i, h, mode, groups=tuple(range(NG)), toks=True, o=None):
        r0 = i * TQ + groups[0] * 128
        r1 = r0 + len(groups) * 128
        if o is None:
            o = load_o(cx, groups)
        d = jnp.dot(o, wo_ref[h], preferred_element_type=F32)
        if mode == 'set':
            acc_ref[r0:r1, :] = d
        elif mode == 'add':
            acc_ref[r0:r1, :] += d
        else:
            s = acc_ref[r0:r1, :] + d
            out_ref[r0:r1, :] = (x_ref[r0:r1, :].astype(F32) + s * g_ref[r0:r1, :]).astype(BF)
        if toks:
            for r in DTOK:
                cx.hist.append(d[r:r + 8, 0:128])

    cp_x(0, SEM_A).start()
    cp_wq(0, SEM_A).start()
    cp_k(0, SEM_B).start()
    cp_x(1, SEM_B).start()
    cp_v(0, SEM_C).start()
    cp_x(2, SEM_D).start()
    cp_x(3, SEM_D).start()
    cp_wo(0, SEM_D).start()
    cp_wq(1, SEM_D).start()
    cp_wr.start()
    z_ref[0] = 0
    z_ref[1] = 0
    acc_ref[S - TQ:, :] = jnp.zeros((TQ, D), F32)

    def hide(i, c):
        z_ref[1] = z_ref[0] * i
        z_ref[0] = z_ref[1] * i
        return c

    lax.fori_loop(0, 2, hide, 0)
    cx = Ctx()
    rc = [jnp.zeros((8, 128), F32), jnp.zeros((8, 128), F32)]

    if LASTONLY:
        start_head(H - 1)
        for c in cp_ffn:
            c.start()
        def _b(i, c_):
            z_ref[1] = z_ref[0] * i
            z_ref[0] = z_ref[1] * i
            return c_
        lax.fori_loop(0, 3, _b, 0)
    elif LOOPONLY:
        start_head(1)
        for c in cp_ffn:
            c.start()
    else:
        cp_x(0, SEM_A).wait()
        cp_wq(0, SEM_A).wait()
        ln = LayerNorm(cx, 0, TQ, L0C, L0A, L0B)
        for _ in range(ln.steps):
            ln.step()
        q = qproj(0, 0, split=4)
        cp_k(0, SEM_B).wait()
        cp_x(1, SEM_B).wait()
        for hh in range(HPI):
            start_head(1 + hh)
        def hold_o(t):
            ot_ref[NG * DH:NG * DH + 8, :] = pltpu.bitcast(cx.tok(t), F32)

        ogate = [(hold_o, 1, OGT, OGT + 8)] if OGT else []
        for n in range(NB):
            if n == 1:
                cp_x(2, SEM_D).wait()
                cp_x(3, SEM_D).wait()
                cp_wo(0, SEM_D).wait()
                cp_wq(1, SEM_D).wait()
                cp_wr.wait()
                wrf_ref[...] = jnp.broadcast_to(wr_ref[...].astype(F32).reshape(1, D), (8, D))
                for c in cp_ffn:
                    c.start()
            if n + 1 < NB:
                ln = LayerNorm(cx, (n + 1) * TQ, TQ, LNC, LAG2, LAG3)
                if n == 0:
                    ln.step()
                    m = qk(cx, n, 0, q, ticks=[(ln.step, ln.steps - 1, 0, LSPAN0)])
                else:
                    m = qk(cx, n, 0, q, ticks=[(ln.step, ln.steps, LOFF, LSPAN)] + ogate)
            else:
                rn = S // RJOB
                st = [0]

                def rstep(t=None):
                    router(cx, st[0] * rn, rn, rc, t)
                    st[0] += 1

                m = qk(cx, n, 0, q, ticks=[(rstep, RJOB, ROFF, RSPAN)] + ogate)
                route(rc)
            if n == 0:
                cp_v(0, SEM_C).wait()
                transpose_v(cx, 0, 0)
                q = qproj(1, 0)
            elif n + 1 < NB:
                if DA:
                    oproj(cx, n - 1, 0, 'set', toks=False)
                    q = qproj(n + 1, 0, cx=cx)
                else:
                    q = qproj(n + 1, 0)
                    oproj(cx, n - 1, 0, 'set')
            else:
                q = qproj(0, 1)
                oproj(cx, n - 1, 0, 'set')
            hooks = None
            if n + 1 == NB:
                qn_ref[...] = pltpu.bitcast(q.T if QT else q, U32)
                hooks = {RTH: cx.memtok(xs_ref) | cx.memtok(rs_ref), QTH: cx.memtok(qn_ref)}
            pv(cx, n, 0, m, hooks)

        if ONLYF:
            wait_head(1)
            for c in cp_ffn:
                c.wait()
            def _c(i, c_):
                o8 = pl.multiple_of(i * 16, 16)
                f = lambda r: r[pl.ds(o8, 16), 0:128].astype(BF)
                out_ref[0:16, 0:128] = (pltpu.bitcast(qn_ref[pl.ds(o8, 8), 0:128], BF) + f(ot_ref) + f(acc_ref) + f(xn_ref) + f(lr_ref)
                                        + (xs_ref[:, 0:128] + rs_ref[...])[0:1].astype(BF) + idx_ref[i].astype(BF))
                return c_
            lax.fori_loop(0, 2, _c, 0)
            cp_out(3).start()
            cp_out(3).wait()
            return
    if not LASTONLY:
        def body(it, _):
            h0 = 1 + it * HPI
            for hh in range(HPI):
                wait_head(h0 + hh)
            for hh in range(HPI):
                if hh == 0:
                    start_head(h0 + HPI)
                else:
                    @pl.when(h0 + HPI + hh < H)
                    def _():
                        start_head(h0 + HPI + hh)
            cx = Ctx()
            for hh in range(HPI):
                transpose_v(cx, hh, h0 + hh)
            q = pltpu.bitcast(qn_ref[...], BF)
            h_prev = h0 - 1
            for n in range(HPI * NB):
                hh, i = divmod(n, NB)
                hn, in_ = divmod(n + 1, NB)
                jobs = ()
                if n == GUN:
                    gate(pl.multiple_of(jnp.minimum(it * GROWS, S - GROWS), 16), GROWS)
                if n == 0 and AFIRST:
                    q_next = qproj(in_, h0 + hn)
                    m = qk(cx, n, h0 + hh, q, jobs)
                    q = q_next
                else:
                    m = qk(cx, n, h0 + hh, q, jobs, qt=QT and n == 0)
                    q = qproj(in_, h0 + hn)
                oproj(cx, (i - 1) % NB, h_prev, 'add')
                hooks = None
                if n == HPI * NB - 1:
                    qn_ref[...] = pltpu.bitcast(q.T if QT else q, U32)
                    if QTH:
                        hooks = {QTH: cx.memtok(qn_ref)}
                pv(cx, n, hh, m, hooks)
                h_prev = h0 + hh
            return 0

        lax.fori_loop(0, (H - 2) // HPI, body, 0)

    h = H - 1
    wait_head(h)
    for c in cp_ffn:
        c.wait()
    if LOOPONLY:
        out_ref[0:16, 0:128] = pltpu.bitcast(qn_ref[0:8, 0:128], BF) + ot_ref[0:16, :].astype(BF) + acc_ref[0:16, 0:128].astype(BF) + g_ref[0:16, 0:128].astype(BF)
        cp_out(3).start()
        cp_out(3).wait()
        return
    cx = Ctx()
    transpose_v(cx, 0, h)
    q = pltpu.bitcast(qn_ref[...], BF)
    ffn = Ffn()
    cnt = lambda tot, j: (tot * (j + 1)) // (FSL - 1) - (tot * j) // (FSL - 1)
    m = qk(cx, 0, h, q, qt=QT, after=[(lambda t, j=j: ffn.run_up(cnt(70, j))) for j in range(FSL - 1)] + [None])
    q = qproj(1, h)
    oproj(cx, NB - 1, h - 1, 'add')
    pv(cx, 0, 0, m)
    m = qk(cx, 1, h, q, after=[(lambda t, j=j: ffn.run_up(cnt(70, j))) for j in range(FSL - 1)] + [None])
    q = qproj(2, h, cx=cx)
    pv(cx, 1, 0, m, buf=1)
    m = qk(cx, 2, h, q, after=[(lambda t, j=j: ffn.run_down(cnt(70, j))) for j in range(FSL - 1)] + [None])
    ffn.finish()
    q = qproj(3, h, t=None)
    allg = tuple(range(NG))
    oproj(cx, 0, h, 'fin', toks=False)
    cp_out(0).start()
    oproj(cx, 1, h, 'fin', o=load_o(cx, allg, 1))
    cp_out(1).start()
    pv(cx, 2, 0, m, {FINH: cx.memtok(out_ref)})
    m = qk(cx, 3, h, q)
    oproj(cx, 2, h, 'fin')
    cp_out(2).start()

    def alltok(o):
        u = pltpu.bitcast(o, U32)
        t = u[0:8]
        for r in range(8, u.shape[0], 8):
            t = t | u[r:r + 8]
        return t & cx.zvec

    pv(cx, NB - 1, 0, m, {FINH: cx.memtok(out_ref)}, groups=(0, 1))
    os = [load_o(cx, (0,)), load_o(cx, (1,))]
    pv(cx, NB - 1, 0, m, groups=(2,))
    os.append(load_o(cx, (2,)))
    pv(cx, NB - 1, 0, m, {TAILH: alltok(os[0]) | alltok(os[1])} if TAILH else None, groups=(3,))
    os.append(load_o(cx, (3,)))
    for g in range(NG):
        oproj(cx, NB - 1, h, 'fin', groups=(g,), toks=False, o=os[g])
        cp_out(NB - 1 + g).start()
    for j in range(len(out_pieces)):
        cp_out(j).wait()


@jax.jit
def pallas_recurrent_scan__mha_block_cached__moe_arch_mod__prompt_kernel(
    A_x, A_k_cache, A_v_cache, A_wq, A_wo, B_x, B_w_r, B_w_gate, B_w_up, B_w_down):
    x = A_x.reshape(S, D)
    k = A_k_cache.reshape(H, S, DH)
    v = A_v_cache.reshape(H, S, DH)
    wo = A_wo.reshape(H, DH, D)
    wr = B_w_r
    anyspec = pl.BlockSpec(memory_space=pl.ANY)
    out = pl.pallas_call(
        _kernel,
        in_specs=[anyspec] * 9,
        out_specs=anyspec,
        out_shape=jax.ShapeDtypeStruct((S, D), BF),
        scratch_shapes=[
            pltpu.VMEM((S, TQ), F32),
            pltpu.VMEM((S, TQ), F32),
            pltpu.VMEM((HPI, DH // 2, S), U32),
            pltpu.VMEM((NG * DH + 32, 128), F32),
            pltpu.VMEM((NG * DH, 128), F32),
            pltpu.VMEM((S, D), F32),
            pltpu.VMEM((DH // 2, TQ) if QT else (TQ // 2, DH), U32),
            pltpu.VMEM((H, S, DH), BF),
            pltpu.VMEM((H, S, DH), BF),
            pltpu.VMEM((H, D, DH), BF),
            pltpu.VMEM((H, DH, D), BF),
            pltpu.VMEM((S + 64, D), BF),
            pltpu.VMEM((S, D), F32),
            pltpu.VMEM((S, D), BF),
            pltpu.VMEM((F, D), BF),
            pltpu.VMEM((F, D), BF),
            pltpu.VMEM((F, D), BF),
            pltpu.VMEM((S + 64, D), BF),
            pltpu.VMEM((NG * 8, 128), F32),
            pltpu.VMEM((NG * 8, 128), F32),
            pltpu.VMEM((C, D), F32),
            pltpu.VMEM((C, 128), F32),
            pltpu.VMEM((8, D), F32),
            pltpu.VMEM((D,), BF),
            pltpu.SMEM((2,), jnp.int32),
            pltpu.SMEM((C,), jnp.int32),
            pltpu.SemaphoreType.DMA((7,)),
        ],
        compiler_params=pltpu.CompilerParams(
            vmem_limit_bytes=126 * 1024 * 1024,
            internal_scratch_in_bytes=16 * 4096,
            disable_bounds_checks=True,
            disable_semaphore_checks=True,
        ),
    )(x, k, v, A_wq, wo, wr, B_w_gate.T, B_w_up.T, B_w_down)
    return out.reshape(1, S, D)
```

```python
import math
import jax
import jax.numpy as jnp
from jax import lax
import jax.experimental.pallas as pl
import jax.experimental.pallas.tpu as pltpu

S, D, H, DH, F, C = 2048, 640, 32, 128, 1728, 8
TQ = 512
NB = S // TQ
NG = TQ // 128
BF = jnp.bfloat16
F32 = jnp.float32
U32 = jnp.uint32
QSCALE = (DH ** -0.5) * math.log2(math.e)
E = lambda k, d: d
PV_CT = 4
PV_DIST = E('PV_DIST', 3)
HPI = E('HPI', 1)
LNC = E('LNC', 8)
RC_ = 16
RJOB = E('RJOB', 32)
RSPAN = E('RSPAN', 1900)
LAG2 = E('LAG2', 4)
TSL = E('TSL', 1)
LAG3 = E('LAG3', 10)
LOFF = E('LOFF', 0)
ROFF = E('ROFF', 0)
DA = E('DA', 0)
QT = E('QT', 1)
ODEL = E('ODEL', 0)
TORD = E('TORD', 1)
TLAG = E('TLAG', 2)
QTH = E('QTH', 4)
QTH0 = E('QTH0', 10)
OGT = E('OGT', 0)
LSPAN0 = E('LSPAN0', 2000)
LSPAN = E('LSPAN', 2040)
L0C = E('L0C', 32)
L0A = E('L0A', 0)
L0B = E('L0B', 0)
ATOK = ()
NJOB = E('NJOB', 8)
AFIRST = E('AFIRST', 0)
ONLYF = E('ONLYF', 0)
TAILH = E('TAILH', 0)
FSL = E('FSL', 16)
FH0 = E('FH0', 9)
RTH = E('RTH', 14)
LASTONLY = E('LASTONLY', 0)
LOOPONLY = E('LOOPONLY', 0)
GSPL = E('GSPL', 1)
GUN = E('GUN', 1)
GMODE = E('GMODE', 0)
LN_DIST = E('LN_DIST', 2)
GROWS = E('GROWS', 64)
GREST = E('GREST', 0)
FINH = E('FINH', 6)
DTOK = (128, 256, 384, 504)
NT = (((1,), (1,)), ((), ()))


def _rb(a):
    return a.astype(BF).astype(F32)


def _kernel(x_hbm, k_hbm, v_hbm, wq_hbm, wo_hbm, wr_hbm, wg_hbm, wu_hbm, wd_hbm,
            o_hbm,
            s0_ref, s1_ref, vt_ref, ot_ref, ot2_ref, acc_ref, qn_ref,
            k_ref, v_ref, wq_ref, wo_ref, xn_ref, g_ref, out_ref, wg_ref, wu_ref, wd_ref,
            x_ref, lr_ref, lr2_ref, xs_ref, rs_ref, wrf_ref, wr_ref, z_ref, idx_ref, sem):
    s_refs = (s0_ref, s1_ref)
    ot_refs = (ot_ref, ot2_ref)
    lr_refs = (lr_ref, lr2_ref)

    SEM_A, SEM_B, SEM_C, SEM_D, SEM_H, SEM_F, SEM_O = range(7)

    def cp_k(h, s=SEM_H):
        return pltpu.make_async_copy(k_hbm.at[h], k_ref.at[h], sem.at[s])

    def cp_v(h, s=SEM_H):
        return pltpu.make_async_copy(v_hbm.at[h], v_ref.at[h], sem.at[s])

    def cp_wq(h, s=SEM_H):
        off = h * DH if isinstance(h, int) else pl.multiple_of(h * DH, DH)
        return pltpu.make_async_copy(wq_hbm.at[:, pl.ds(off, DH)], wq_ref.at[h], sem.at[s])

    def cp_wo(h, s=SEM_H):
        return pltpu.make_async_copy(wo_hbm.at[h], wo_ref.at[h], sem.at[s])

    def cp_x(i, s):
        return pltpu.make_async_copy(x_hbm.at[pl.ds(i * TQ, TQ)], x_ref.at[pl.ds(i * TQ, TQ)], sem.at[s])

    cp_ffn = [pltpu.make_async_copy(wg_hbm, wg_ref, sem.at[SEM_F]),
              pltpu.make_async_copy(wu_hbm, wu_ref, sem.at[SEM_F]),
              pltpu.make_async_copy(wd_hbm, wd_ref, sem.at[SEM_F])]

    cp_wr = pltpu.make_async_copy(wr_hbm, wr_ref, sem.at[SEM_D])

    out_pieces = [(i * TQ, TQ) for i in range(NB - 1)] + [(S - TQ + g * 128, 128) for g in range(NG)]

    def cp_out(j):
        r0, n = out_pieces[j]
        return pltpu.make_async_copy(out_ref.at[pl.ds(r0, n)], o_hbm.at[pl.ds(r0, n)], sem.at[SEM_O])

    def start_head(h):
        cp_k(h).start()
        cp_v(h).start()
        cp_wo(h).start()
        if isinstance(h, int):
            if h + 1 < H:
                cp_wq(h + 1).start()
        else:
            @pl.when(h + 1 < H)
            def _():
                cp_wq(h + 1).start()

    def wait_head(h):
        cp_k(h).wait()
        cp_v(h).wait()
        cp_wo(h).wait()
        if not isinstance(h, int) or h + 1 < H:
            cp_wq(h + 1).wait()

    lane = lax.broadcasted_iota(jnp.int32, (8, 128), 1)
    sub = lax.broadcasted_iota(jnp.int32, (8, 128), 0)

    class Ctx:
        def __init__(self):
            self.z1 = pl.multiple_of(z_ref[0], 8)
            self.z2 = pl.multiple_of(z_ref[1], 8)
            self.zvec = jnp.full((8, 128), z_ref[0], jnp.int32).astype(U32)
            self.hist = []
            self.lnh = []

        def tok(self, a):
            return pltpu.bitcast(a, U32) & self.zvec

        def memtok(self, ref):
            rows = 16 if ref.dtype == BF else 8
            z = pl.multiple_of(self.z2 * 2, 16)
            return self.tok(ref[pl.ds(z, rows), 0:128])

    def dep_bf(a, t):
        if t is None:
            return a
        au = pltpu.bitcast(a, U32)
        first = au[0:8, 0:128] | t
        top = first if au.shape[1] == 128 else jnp.concatenate([first, au[0:8, 128:]], axis=1)
        return pltpu.bitcast(jnp.concatenate([top, au[8:]], axis=0), BF)

    def dep_f32(a, t):
        return pltpu.bitcast(pltpu.bitcast(a, U32) | t, F32)

    class LayerNorm:
        def __init__(self, cx, r0, n, c, lag2, lag3):
            self.cx, self.r0, self.c, self.n = cx, r0, c, n // c
            self.lag2, self.lag3 = lag2, lag3
            self.k = 0
            self.mean, self.inv = {}, {}
            self.steps = self.n + lag3

        def step(self, gate_tok=None):
            cx, c, k = self.cx, self.c, self.k
            self.k += 1
            xv = x_ref.at[pl.ds(pl.multiple_of(cx.z2 * 2, 16), S), :]
            xw = x_ref.at[pl.ds(pl.multiple_of(cx.z1 * 2, 16), S), :]
            xu = x_ref.at[pl.ds(pl.multiple_of((cx.z1 + cx.z2) * 2, 16), S), :]
            if gate_tok is not None:
                x_ref[S:S + 16, 0:128] = pltpu.bitcast(cx.tok(gate_tok), BF)
            if k < self.n:
                a = self.r0 + k * c
                self.mean[k] = jnp.mean(xv[a:a + c, :].astype(F32), axis=-1, keepdims=True)
            j = k - self.lag2
            if 0 <= j < self.n:
                a = self.r0 + j * c
                xc = xw[a:a + c, :].astype(F32) - self.mean[j]
                v = _rb(_rb(jnp.mean(xc * xc, axis=-1, keepdims=True)) + 1e-5)
                den = _rb(v * lax.rsqrt(v))
                inv = pl.reciprocal(den, approx=True)
                self.inv[j] = inv * (2.0 - den * inv)
            j = k - self.lag3
            if 0 <= j < self.n:
                a = self.r0 + j * c
                d = _rb(xu[a:a + c, :].astype(F32) - _rb(self.mean[j]))
                xn_ref[a:a + c, :] = (d * self.inv[j]).astype(BF)

    def silu(b):
        hb = 0.5 * b
        return hb + hb * jnp.tanh(hb)

    def gate(r0, n):
        xf = xn_ref[pl.ds(r0, n), :].astype(F32)
        g_ref[pl.ds(r0, n), :] = silu(xf)
        return xf

    def router(cx, r0, n, rc, gate_tok=None):
        xv = xn_ref.at[pl.ds(pl.multiple_of(cx.z2 * 2, 16), S), :]
        if gate_tok is not None:
            xn_ref[S:S + 16, 0:128] = pltpu.bitcast(cx.tok(gate_tok), BF)
        for c in range(n // RC_):
            a = r0 + c * RC_
            xf = xv[a:a + RC_, :].astype(F32)
            r = _rb(jnp.sum(xf * jnp.concatenate([wrf_ref[...]] * (RC_ // 8), axis=0), axis=-1, keepdims=True))
            for j in range(RC_ // 8):
                gi = a // 8 + j
                rc[gi // 128] = jnp.where(lane == gi % 128, r[j * 8:(j + 1) * 8, :], rc[gi // 128])

    def route(rc):
        r = jnp.concatenate(rc, axis=0)
        tix = jnp.concatenate([(8 * (128 * a + lane) + sub) for a in range(2)], axis=0).astype(F32)
        rw = jnp.where(r != r, -jnp.inf, r)
        alive = jnp.ones((16, 128), F32)
        for j in range(C):
            mx = jnp.max(jnp.max(rw, axis=0, keepdims=True), axis=1, keepdims=True)
            cand = jnp.where((rw == mx) & (alive > 0), tix, float(S - 1))
            ixv = jnp.min(jnp.min(cand, axis=0, keepdims=True), axis=1, keepdims=True)
            hit = tix == ixv
            rsel = jnp.sum(jnp.sum(jnp.where(hit, r, 0.0), axis=0, keepdims=True), axis=1, keepdims=True)
            rw = jnp.where(hit, -jnp.inf, rw)
            alive = jnp.where(hit, 0.0, alive)
            ix = ixv.astype(jnp.int32)[0, 0]
            idx_ref[j] = ix
            blk = xn_ref[pl.ds(pl.multiple_of((ix // 16) * 16, 16), 16), :].astype(F32)
            pick = lax.broadcasted_iota(jnp.int32, (16, D), 0) == (ixv.astype(jnp.int32) & 15)
            xs_ref[j:j + 1, :] = jnp.sum(jnp.where(pick, blk, 0.0), axis=0, keepdims=True)
            rs_ref[j:j + 1, :] = jnp.broadcast_to(rsel, (1, 128))

    FT = [(f0, min(128, F - f0)) for f0 in range(0, F, 128)]

    class Ffn:
        def __init__(self):
            self.xs = xs_ref[...].astype(BF)
            self.acc = {}
            self.up = [(w, i, k) for i in range(len(FT)) for w in (0, 1) for k in range(D // 128)]
            self.down = [(i, k) for k in range(D // 128) for i in range(len(FT))]
            self.hid = None

        def add(self, key, d):
            self.acc[key] = d if key not in self.acc else self.acc[key] + d

        def run_up(self, n):
            for _ in range(min(n, len(self.up))):
                w, i, k = self.up.pop(0)
                f0, fn = FT[i]
                wt = (wg_ref, wu_ref)[w][f0:f0 + fn, k * 128:(k + 1) * 128]
                self.add((w, i), lax.dot_general(self.xs[:, k * 128:(k + 1) * 128], wt, NT, preferred_element_type=F32))

        def run_down(self, n):
            if self.hid is None:
                self.run_up(len(self.up))
                self.hid = []
                for i in range(len(FT)):
                    g = _rb(self.acc[(0, i)])
                    g = _rb(g * jax.nn.sigmoid(g))
                    self.hid.append((g * _rb(self.acc[(1, i)])).astype(BF))
            for _ in range(min(n, len(self.down))):
                i, k = self.down.pop(0)
                f0, fn = FT[i]
                self.add((2, k), jnp.dot(self.hid[i], wd_ref[f0:f0 + fn, k * 128:(k + 1) * 128], preferred_element_type=F32))

        def finish(self):
            self.run_down(len(self.down))
            y = _rb(jnp.concatenate([self.acc[(2, k)] for k in range(D // 128)], axis=1))
            y = _rb(y * _rb(jax.nn.sigmoid(rs_ref[:, 0:1])))
            b = _rb(xs_ref[...] + y)
            gs = b * jax.nn.sigmoid(b)
            for j in range(C):
                g_ref[pl.ds(idx_ref[j], 1), :] = gs[j:j + 1, :]

    def qproj(i, h, split=1, t=None, cx=None):
        parts = []
        n = TQ // split
        for c in range(split):
            r0 = i * TQ + c * n
            xn = dep_bf(xn_ref[r0:r0 + n, :], t)
            d = jnp.dot(xn, wq_ref[h], preferred_element_type=F32)
            if cx is not None:
                for r in ATOK:
                    cx.hist.append(d[r:r + 8, :])
            parts.append((d * QSCALE).astype(BF))
        return parts[0] if split == 1 else jnp.concatenate(parts, axis=0)

    def transpose_v(cx, hh, h):
        vt_ref[hh, pl.ds(cx.z1, DH // 2), :] = pltpu.bitcast(v_ref[h].T, U32)

    def qk(cx, n, h, q, jobs=(), after=(), ticks=None, qt=False):
        sv = s_refs[n % 2].at[pl.ds(cx.z1, S), :]
        ns = max(len(jobs) + 1, len(after))
        if ticks is not None:
            ns = TSL
        sl = S // ns
        m = None
        for j in range(ns):
            t = jobs[j - 1]() if 0 < j <= len(jobs) else None
            kj = dep_bf(k_ref[h, j * sl:(j + 1) * sl, :], t)
            if qt:
                sT = jnp.dot(kj, q, preferred_element_type=F32)
            else:
                sT = lax.dot_general(kj, q, NT, preferred_element_type=F32)
            sv[j * sl:(j + 1) * sl, :] = sT
            mj = jnp.max(jnp.max(sT.reshape(sl // 128, 16, 8, TQ), axis=1), axis=0)
            m = mj if m is None else jnp.maximum(m, mj)
            if j < len(after) and after[j] is not None:
                after[j](sT[0:8, 0:128])
            for fn, cnt_, off, span in (ticks or ()):
                for i in range(cnt_):
                    r = (off + i * (span - off) // cnt_) // 8 * 8 - j * sl
                    if 0 <= r < sl:
                        fn(sT[r:r + 8, 0:128])
        return jnp.broadcast_to(jnp.max(m, axis=0, keepdims=True), (8, TQ))

    def pv(cx, n, hh, m, hooks=None, groups=tuple(range(NG)), after=None, buf=0):
        sv = s_refs[n % 2].at[pl.ds(cx.z2, S), :]
        vv = vt_ref.at[hh, pl.ds(cx.z2, DH // 2), :]
        otv = ot_refs[buf].at[pl.ds(cx.z1, NG * DH), :]
        lrv = lr_refs[buf].at[pl.ds(cx.z1, NG * 8), :]
        CT = PV_CT
        for g in groups:
            mg = m[:, g * 128:(g + 1) * 128]
            l8 = None
            oT = None
            for c in range(S // 128 // CT):
                mc = mg
                if len(cx.hist) >= PV_DIST:
                    mc = dep_f32(mc, cx.tok(cx.hist[-PV_DIST]))
                if hooks and (g * 4 + c) in hooks:
                    mc = dep_f32(mc, hooks[g * 4 + c])
                ps = []
                for tt in range(CT):
                    r0 = (c * CT + tt) * 128
                    s = sv[r0:r0 + 128, g * 128:(g + 1) * 128]
                    p = jnp.exp2(s - jnp.concatenate([mc] * 16, axis=0))
                    lt = None
                    for j in reversed(range(16)):
                        pj = p[j * 8:(j + 1) * 8, :]
                        lt = pj if lt is None else lt + pj
                    l8 = lt if l8 is None else l8 + lt
                    ps.append(p)
                vT = pltpu.bitcast(vv[:, c * CT * 128:(c + 1) * CT * 128], BF)
                part = jnp.dot(vT, jnp.concatenate(ps, axis=0).astype(BF), preferred_element_type=F32)
                cx.hist.append(part[0:8, :])
                if after and (g * 4 + c) in after:
                    after[g * 4 + c](part[0:8, :])
                oT = part if oT is None else oT + part
            otv[g * DH:(g + 1) * DH, :] = oT
            lrv[g * 8:(g + 1) * 8, :] = l8

    def load_o(cx, groups, buf=0):
        otv = ot_refs[buf].at[pl.ds(cx.z2, NG * DH), :]
        lrv = lr_refs[buf].at[pl.ds(cx.z2, NG * 8), :]
        parts = []
        for g in groups:
            l = jnp.sum(lrv[g * 8:(g + 1) * 8, :], axis=0, keepdims=True)
            parts.append((otv[g * DH:(g + 1) * DH, :] * (1.0 / l)).T.astype(BF))
        return parts[0] if len(parts) == 1 else jnp.concatenate(parts, axis=0)

    def oproj(cx, i, h, mode, groups=tuple(range(NG)), toks=True, o=None):
        r0 = i * TQ + groups[0] * 128
        r1 = r0 + len(groups) * 128
        if o is None:
            o = load_o(cx, groups)
        d = jnp.dot(o, wo_ref[h], preferred_element_type=F32)
        if mode == 'set':
            acc_ref[r0:r1, :] = d
        elif mode == 'add':
            acc_ref[r0:r1, :] += d
        else:
            s = acc_ref[r0:r1, :] + d
            out_ref[r0:r1, :] = (x_ref[r0:r1, :].astype(F32) + s * g_ref[r0:r1, :]).astype(BF)
        if toks:
            for r in DTOK:
                cx.hist.append(d[r:r + 8, 0:128])

    cp_x(0, SEM_A).start()
    cp_wq(0, SEM_A).start()
    cp_k(0, SEM_B).start()
    cp_x(1, SEM_B).start()
    cp_v(0, SEM_C).start()
    cp_x(2, SEM_D).start()
    cp_x(3, SEM_D).start()
    cp_wo(0, SEM_D).start()
    cp_wq(1, SEM_D).start()
    cp_wr.start()
    z_ref[0] = 0
    z_ref[1] = 0
    acc_ref[S - TQ:, :] = jnp.zeros((TQ, D), F32)

    def hide(i, c):
        z_ref[1] = z_ref[0] * i
        z_ref[0] = z_ref[1] * i
        return c

    lax.fori_loop(0, 2, hide, 0)
    cx = Ctx()
    rc = [jnp.zeros((8, 128), F32), jnp.zeros((8, 128), F32)]

    if LASTONLY:
        start_head(H - 1)
        for c in cp_ffn:
            c.start()
        def _b(i, c_):
            z_ref[1] = z_ref[0] * i
            z_ref[0] = z_ref[1] * i
            return c_
        lax.fori_loop(0, 3, _b, 0)
    elif LOOPONLY:
        start_head(1)
        for c in cp_ffn:
            c.start()
    else:
        cp_x(0, SEM_A).wait()
        cp_wq(0, SEM_A).wait()
        ln = LayerNorm(cx, 0, TQ, L0C, L0A, L0B)
        for _ in range(ln.steps):
            ln.step()
        q = qproj(0, 0, split=4)
        cp_k(0, SEM_B).wait()
        cp_x(1, SEM_B).wait()
        for hh in range(HPI):
            start_head(1 + hh)
        def hold_o(t):
            ot_ref[NG * DH:NG * DH + 8, :] = pltpu.bitcast(cx.tok(t), F32)

        ogate = [(hold_o, 1, OGT, OGT + 8)] if OGT else []
        for n in range(NB):
            if n == 1:
                cp_x(2, SEM_D).wait()
                cp_x(3, SEM_D).wait()
                cp_wo(0, SEM_D).wait()
                cp_wq(1, SEM_D).wait()
                cp_wr.wait()
                wrf_ref[...] = jnp.broadcast_to(wr_ref[...].astype(F32).reshape(1, D), (8, D))
                for c in cp_ffn:
                    c.start()
            if n + 1 < NB:
                ln = LayerNorm(cx, (n + 1) * TQ, TQ, LNC, LAG2, LAG3)
                if n == 0:
                    ln.step()
                    m = qk(cx, n, 0, q, ticks=[(ln.step, ln.steps - 1, 0, LSPAN0)])
                else:
                    m = qk(cx, n, 0, q, ticks=[(ln.step, ln.steps, LOFF, LSPAN)] + ogate)
            else:
                rn = S // RJOB
                st = [0]

                def rstep(t=None):
                    router(cx, st[0] * rn, rn, rc, t)
                    st[0] += 1

                m = qk(cx, n, 0, q, ticks=[(rstep, RJOB, ROFF, RSPAN)] + ogate)
                route(rc)
                if GREST == 0:
                    gate((H - 2) * GROWS, S - (H - 2) * GROWS)
            if n == 0:
                cp_v(0, SEM_C).wait()
                transpose_v(cx, 0, 0)
                q = qproj(1, 0)
            elif n + 1 < NB:
                if DA:
                    oproj(cx, n - 1, 0, 'set', toks=False)
                    q = qproj(n + 1, 0, cx=cx)
                else:
                    q = qproj(n + 1, 0)
                    oproj(cx, n - 1, 0, 'set')
            else:
                q = qproj(0, 1)
                oproj(cx, n - 1, 0, 'set')
            hooks = None
            if n + 1 == NB:
                qn_ref[...] = pltpu.bitcast(q.T if QT else q, U32)
                hooks = {RTH: cx.memtok(xs_ref) | cx.memtok(rs_ref)}
                if QTH0:
                    hooks[QTH0] = cx.memtok(qn_ref) | hooks.get(QTH0, cx.zvec)
            pv(cx, n, 0, m, hooks)

        if ONLYF:
            wait_head(1)
            for c in cp_ffn:
                c.wait()
            def _c(i, c_):
                o8 = pl.multiple_of(i * 16, 16)
                f = lambda r: r[pl.ds(o8, 16), 0:128].astype(BF)
                out_ref[0:16, 0:128] = (pltpu.bitcast(qn_ref[pl.ds(o8, 8), 0:128], BF) + f(ot_ref) + f(acc_ref) + f(xn_ref) + f(lr_ref) + f(g_ref)
                                        + (xs_ref[:, 0:128] + rs_ref[...])[0:1].astype(BF) + idx_ref[i].astype(BF))
                return c_
            lax.fori_loop(0, 2, _c, 0)
            cp_out(3).start()
            cp_out(3).wait()
            return
    if not LASTONLY:
        def body(it, _):
            h0 = 1 + it * HPI
            for hh in range(HPI):
                wait_head(h0 + hh)
            for hh in range(HPI):
                if hh == 0:
                    start_head(h0 + HPI)
                else:
                    @pl.when(h0 + HPI + hh < H)
                    def _():
                        start_head(h0 + HPI + hh)
            cx = Ctx()
            for hh in range(HPI):
                transpose_v(cx, hh, h0 + hh)
            q = pltpu.bitcast(qn_ref[...], BF)
            h_prev = h0 - 1
            for n in range(HPI * NB):
                hh, i = divmod(n, NB)
                hn, in_ = divmod(n + 1, NB)
                jobs = ()
                if n == GUN:
                    gate(pl.multiple_of(it * GROWS, GROWS), GROWS)
                if n == 0 and AFIRST:
                    q_next = qproj(in_, h0 + hn)
                    m = qk(cx, n, h0 + hh, q, jobs)
                    q = q_next
                else:
                    m = qk(cx, n, h0 + hh, q, jobs, qt=QT and n == 0)
                    q = qproj(in_, h0 + hn)
                oproj(cx, (i - 1) % NB, h_prev, 'add')
                hooks = None
                if n == HPI * NB - 1:
                    qn_ref[...] = pltpu.bitcast(q.T if QT else q, U32)
                    if QTH:
                        hooks = {QTH: cx.memtok(qn_ref)}
                pv(cx, n, hh, m, hooks)
                h_prev = h0 + hh
            return 0

        lax.fori_loop(0, (H - 2) // HPI, body, 0)

    h = H - 1
    wait_head(h)
    for c in cp_ffn:
        c.wait()
    if LOOPONLY:
        out_ref[0:16, 0:128] = pltpu.bitcast(qn_ref[0:8, 0:128], BF) + ot_ref[0:16, :].astype(BF) + acc_ref[0:16, 0:128].astype(BF) + g_ref[0:16, 0:128].astype(BF)
        cp_out(3).start()
        cp_out(3).wait()
        return
    cx = Ctx()
    transpose_v(cx, 0, h)
    q = pltpu.bitcast(qn_ref[...], BF)
    if GREST == 1:
        gate((H - 2) * GROWS, S - (H - 2) * GROWS)
    ffn = Ffn()
    cnt = lambda tot, j: (tot * (j + 1)) // (FSL - 1) - (tot * j) // (FSL - 1)
    m = qk(cx, 0, h, q, qt=QT, after=[(lambda t, j=j: ffn.run_up(cnt(70, j))) for j in range(FSL - 1)] + [None])
    q = qproj(1, h)
    oproj(cx, NB - 1, h - 1, 'add')
    pv(cx, 0, 0, m)
    m = qk(cx, 1, h, q, after=[(lambda t, j=j: ffn.run_up(cnt(70, j))) for j in range(FSL - 1)] + [None])
    q = qproj(2, h, cx=cx)
    pv(cx, 1, 0, m, buf=1)
    m = qk(cx, 2, h, q, after=[(lambda t, j=j: ffn.run_down(cnt(70, j))) for j in range(FSL - 1)] + [None])
    ffn.finish()
    q = qproj(3, h, t=None)
    allg = tuple(range(NG))
    oproj(cx, 0, h, 'fin', toks=False)
    if not ODEL:
        cp_out(0).start()
    oproj(cx, 1, h, 'fin', o=load_o(cx, allg, 1))
    if not ODEL:
        cp_out(1).start()
    pv(cx, 2, 0, m, {FINH: cx.memtok(out_ref)})

    def release(j):
        def fn(t):
            r0 = out_pieces[j][0]
            u = pltpu.bitcast(out_ref[r0:r0 + 16, 0:128], U32) | cx.tok(t)
            out_ref[r0:r0 + 16, 0:128] = pltpu.bitcast(u, BF)
            cp_out(j).start()
        return fn

    m = qk(cx, 3, h, q, ticks=[(release(0), 1, 0, 8), (release(1), 1, ODEL, ODEL + 8)] if ODEL else None)
    oproj(cx, 2, h, 'fin')
    cp_out(2).start()

    def tail_d(g, o):
        oproj(cx, NB - 1, h, 'fin', groups=(g,), toks=False, o=o)
        cp_out(NB - 1 + g).start()

    ftok = cx.memtok(out_ref)
    os = []
    done = 0
    for g in range(NG):
        pv(cx, NB - 1, 0, m, {FINH: ftok}, groups=(g,))
        os.append(load_o(cx, (g,)))
        if g >= TLAG and done < TORD:
            tail_d(done, os[done])
            done += 1
    for g in range(done, NG):
        tail_d(g, os[g])
    for j in range(len(out_pieces)):
        cp_out(j).wait()


@jax.jit
def pallas_recurrent_scan__mha_block_cached__moe_arch_mod__prompt_kernel(
    A_x, A_k_cache, A_v_cache, A_wq, A_wo, B_x, B_w_r, B_w_gate, B_w_up, B_w_down):
    x = A_x.reshape(S, D)
    k = A_k_cache.reshape(H, S, DH)
    v = A_v_cache.reshape(H, S, DH)
    wo = A_wo.reshape(H, DH, D)
    wr = B_w_r
    anyspec = pl.BlockSpec(memory_space=pl.ANY)
    out = pl.pallas_call(
        _kernel,
        in_specs=[anyspec] * 9,
        out_specs=anyspec,
        out_shape=jax.ShapeDtypeStruct((S, D), BF),
        scratch_shapes=[
            pltpu.VMEM((S, TQ), F32),
            pltpu.VMEM((S, TQ), F32),
            pltpu.VMEM((HPI, DH // 2, S), U32),
            pltpu.VMEM((NG * DH + 32, 128), F32),
            pltpu.VMEM((NG * DH, 128), F32),
            pltpu.VMEM((S, D), F32),
            pltpu.VMEM((DH // 2, TQ) if QT else (TQ // 2, DH), U32),
            pltpu.VMEM((H, S, DH), BF),
            pltpu.VMEM((H, S, DH), BF),
            pltpu.VMEM((H, D, DH), BF),
            pltpu.VMEM((H, DH, D), BF),
            pltpu.VMEM((S + 64, D), BF),
            pltpu.VMEM((S, D), F32),
            pltpu.VMEM((S, D), BF),
            pltpu.VMEM((F, D), BF),
            pltpu.VMEM((F, D), BF),
            pltpu.VMEM((F, D), BF),
            pltpu.VMEM((S + 64, D), BF),
            pltpu.VMEM((NG * 8, 128), F32),
            pltpu.VMEM((NG * 8, 128), F32),
            pltpu.VMEM((C, D), F32),
            pltpu.VMEM((C, 128), F32),
            pltpu.VMEM((8, D), F32),
            pltpu.VMEM((D,), BF),
            pltpu.SMEM((2,), jnp.int32),
            pltpu.SMEM((C,), jnp.int32),
            pltpu.SemaphoreType.DMA((7,)),
        ],
        compiler_params=pltpu.CompilerParams(
            vmem_limit_bytes=126 * 1024 * 1024,
            internal_scratch_in_bytes=16 * 4096,
            disable_bounds_checks=True,
            disable_semaphore_checks=True,
        ),
    )(x, k, v, A_wq, wo, wr, B_w_gate.T, B_w_up.T, B_w_down)
    return out.reshape(1, S, D)
```

```python
import math
import jax
import jax.numpy as jnp
from jax import lax
import jax.experimental.pallas as pl
import jax.experimental.pallas.tpu as pltpu

S, D, H, DH, F, C = 2048, 640, 32, 128, 1728, 8
TQ = 512
NB = S // TQ
NG = TQ // 128
BF = jnp.bfloat16
F32 = jnp.float32
U32 = jnp.uint32
QSCALE = (DH ** -0.5) * math.log2(math.e)
E = lambda k, d: d
PV_CT = 4
PV_DIST = E('PV_DIST', 3)
HPI = E('HPI', 1)
LNC = E('LNC', 8)
RC_ = 16
RJOB = E('RJOB', 32)
RSPAN = E('RSPAN', 1900)
LAG2 = E('LAG2', 4)
TSL = E('TSL', 1)
LAG3 = E('LAG3', 10)
LOFF = E('LOFF', 0)
ROFF = E('ROFF', 0)
DA = E('DA', 0)
QT = E('QT', 1)
ODEL = E('ODEL', 0)
TORD = E('TORD', 1)
TLAG = E('TLAG', 2)
QTH = E('QTH', 4)
QTH0 = E('QTH0', 10)
OGT = E('OGT', 0)
LSPAN0 = E('LSPAN0', 2000)
LSPAN = E('LSPAN', 2040)
L0C = E('L0C', 32)
L0A = E('L0A', 0)
L0B = E('L0B', 0)
ATOK = ()
NJOB = E('NJOB', 8)
AFIRST = E('AFIRST', 0)
ONLYF = E('ONLYF', 0)
TAILH = E('TAILH', 0)
FSL = E('FSL', 16)
FH0 = E('FH0', 9)
RTH = E('RTH', 14)
LASTONLY = E('LASTONLY', 0)
LOOPONLY = E('LOOPONLY', 0)
GSPL = E('GSPL', 1)
GUN = E('GUN', 1)
GMODE = E('GMODE', 0)
LN_DIST = E('LN_DIST', 2)
GROWS = E('GROWS', 64)
SP = S + 8
GREST = E('GREST', 0)
FINH = E('FINH', 6)
DTOK = (128, 256, 384, 504)
NT = (((1,), (1,)), ((), ()))


def _rb(a):
    return a.astype(BF).astype(F32)


def _kernel(x_hbm, k_hbm, v_hbm, wq_hbm, wo_hbm, wr_hbm, wg_hbm, wu_hbm, wd_hbm,
            o_hbm,
            s0_ref, s1_ref, vt_ref, ot_ref, ot2_ref, acc_ref, qn_ref,
            k_ref, v_ref, wq_ref, wo_ref, xn_ref, g_ref, out_ref, wg_ref, wu_ref, wd_ref,
            x_ref, lr_ref, lr2_ref, xs_ref, rs_ref, wrf_ref, wr_ref, z_ref, idx_ref, sem):
    s_refs = (s0_ref, s1_ref)
    ot_refs = (ot_ref, ot2_ref)
    lr_refs = (lr_ref, lr2_ref)

    SEM_A, SEM_B, SEM_C, SEM_D, SEM_H, SEM_F, SEM_O = range(7)

    def cp_k(h, s=SEM_H):
        return pltpu.make_async_copy(k_hbm.at[h], k_ref.at[h], sem.at[s])

    def cp_v(h, s=SEM_H):
        return pltpu.make_async_copy(v_hbm.at[h], v_ref.at[h], sem.at[s])

    def cp_wq(h, s=SEM_H):
        off = h * DH if isinstance(h, int) else pl.multiple_of(h * DH, DH)
        return pltpu.make_async_copy(wq_hbm.at[:, pl.ds(off, DH)], wq_ref.at[h], sem.at[s])

    def cp_wo(h, s=SEM_H):
        return pltpu.make_async_copy(wo_hbm.at[h], wo_ref.at[h], sem.at[s])

    def cp_x(i, s):
        return pltpu.make_async_copy(x_hbm.at[pl.ds(i * TQ, TQ)], x_ref.at[pl.ds(i * TQ, TQ)], sem.at[s])

    cp_ffn = [pltpu.make_async_copy(wg_hbm, wg_ref, sem.at[SEM_F]),
              pltpu.make_async_copy(wu_hbm, wu_ref, sem.at[SEM_F]),
              pltpu.make_async_copy(wd_hbm, wd_ref, sem.at[SEM_F])]

    cp_wr = pltpu.make_async_copy(wr_hbm, wr_ref, sem.at[SEM_D])

    out_pieces = [(i * TQ, TQ) for i in range(NB - 1)] + [(S - TQ + g * 128, 128) for g in range(NG)]

    def cp_out(j):
        r0, n = out_pieces[j]
        return pltpu.make_async_copy(out_ref.at[pl.ds(r0, n)], o_hbm.at[pl.ds(r0, n)], sem.at[SEM_O])

    def start_head(h):
        cp_k(h).start()
        cp_v(h).start()
        cp_wo(h).start()
        if isinstance(h, int):
            if h + 1 < H:
                cp_wq(h + 1).start()
        else:
            @pl.when(h + 1 < H)
            def _():
                cp_wq(h + 1).start()

    def wait_head(h):
        cp_k(h).wait()
        cp_v(h).wait()
        cp_wo(h).wait()
        if not isinstance(h, int) or h + 1 < H:
            cp_wq(h + 1).wait()

    lane = lax.broadcasted_iota(jnp.int32, (8, 128), 1)
    sub = lax.broadcasted_iota(jnp.int32, (8, 128), 0)

    class Ctx:
        def __init__(self):
            self.z1 = pl.multiple_of(z_ref[0], 8)
            self.z2 = pl.multiple_of(z_ref[1], 8)
            self.zvec = jnp.full((8, 128), z_ref[0], jnp.int32).astype(U32)
            self.hist = []
            self.lnh = []

        def tok(self, a):
            return pltpu.bitcast(a, U32) & self.zvec

        def memtok(self, ref):
            rows = 16 if ref.dtype == BF else 8
            z = pl.multiple_of(self.z2 * 2, 16)
            return self.tok(ref[pl.ds(z, rows), 0:128])

    def dep_bf(a, t):
        if t is None:
            return a
        au = pltpu.bitcast(a, U32)
        first = au[0:8, 0:128] | t
        top = first if au.shape[1] == 128 else jnp.concatenate([first, au[0:8, 128:]], axis=1)
        return pltpu.bitcast(jnp.concatenate([top, au[8:]], axis=0), BF)

    def dep_f32(a, t):
        return pltpu.bitcast(pltpu.bitcast(a, U32) | t, F32)

    class LayerNorm:
        def __init__(self, cx, r0, n, c, lag2, lag3):
            self.cx, self.r0, self.c, self.n = cx, r0, c, n // c
            self.lag2, self.lag3 = lag2, lag3
            self.k = 0
            self.mean, self.inv = {}, {}
            self.steps = self.n + lag3

        def step(self, gate_tok=None):
            cx, c, k = self.cx, self.c, self.k
            self.k += 1
            xv = x_ref.at[pl.ds(pl.multiple_of(cx.z2 * 2, 16), S), :]
            xw = x_ref.at[pl.ds(pl.multiple_of(cx.z1 * 2, 16), S), :]
            xu = x_ref.at[pl.ds(pl.multiple_of((cx.z1 + cx.z2) * 2, 16), S), :]
            if gate_tok is not None:
                x_ref[S:S + 16, 0:128] = pltpu.bitcast(cx.tok(gate_tok), BF)
            if k < self.n:
                a = self.r0 + k * c
                self.mean[k] = jnp.mean(xv[a:a + c, :].astype(F32), axis=-1, keepdims=True)
            j = k - self.lag2
            if 0 <= j < self.n:
                a = self.r0 + j * c
                xc = xw[a:a + c, :].astype(F32) - self.mean[j]
                v = _rb(_rb(jnp.mean(xc * xc, axis=-1, keepdims=True)) + 1e-5)
                den = _rb(v * lax.rsqrt(v))
                inv = pl.reciprocal(den, approx=True)
                self.inv[j] = inv * (2.0 - den * inv)
            j = k - self.lag3
            if 0 <= j < self.n:
                a = self.r0 + j * c
                d = _rb(xu[a:a + c, :].astype(F32) - _rb(self.mean[j]))
                xn_ref[a:a + c, :] = (d * self.inv[j]).astype(BF)

    def silu(b):
        hb = 0.5 * b
        return hb + hb * jnp.tanh(hb)

    def gate(r0, n):
        xf = xn_ref[pl.ds(r0, n), :].astype(F32)
        g_ref[pl.ds(r0, n), :] = silu(xf)
        return xf

    def router(cx, r0, n, rc, gate_tok=None):
        xv = xn_ref.at[pl.ds(pl.multiple_of(cx.z2 * 2, 16), S), :]
        if gate_tok is not None:
            xn_ref[S:S + 16, 0:128] = pltpu.bitcast(cx.tok(gate_tok), BF)
        for c in range(n // RC_):
            a = r0 + c * RC_
            xf = xv[a:a + RC_, :].astype(F32)
            r = _rb(jnp.sum(xf * jnp.concatenate([wrf_ref[...]] * (RC_ // 8), axis=0), axis=-1, keepdims=True))
            for j in range(RC_ // 8):
                gi = a // 8 + j
                rc[gi // 128] = jnp.where(lane == gi % 128, r[j * 8:(j + 1) * 8, :], rc[gi // 128])

    def route(rc):
        r = jnp.concatenate(rc, axis=0)
        tix = jnp.concatenate([(8 * (128 * a + lane) + sub) for a in range(2)], axis=0).astype(F32)
        rw = jnp.where(r != r, -jnp.inf, r)
        alive = jnp.ones((16, 128), F32)
        for j in range(C):
            mx = jnp.max(jnp.max(rw, axis=0, keepdims=True), axis=1, keepdims=True)
            cand = jnp.where((rw == mx) & (alive > 0), tix, float(S - 1))
            ixv = jnp.min(jnp.min(cand, axis=0, keepdims=True), axis=1, keepdims=True)
            hit = tix == ixv
            rsel = jnp.sum(jnp.sum(jnp.where(hit, r, 0.0), axis=0, keepdims=True), axis=1, keepdims=True)
            rw = jnp.where(hit, -jnp.inf, rw)
            alive = jnp.where(hit, 0.0, alive)
            ix = ixv.astype(jnp.int32)[0, 0]
            idx_ref[j] = ix
            blk = xn_ref[pl.ds(pl.multiple_of((ix // 16) * 16, 16), 16), :].astype(F32)
            pick = lax.broadcasted_iota(jnp.int32, (16, D), 0) == (ixv.astype(jnp.int32) & 15)
            xs_ref[j:j + 1, :] = jnp.sum(jnp.where(pick, blk, 0.0), axis=0, keepdims=True)
            rs_ref[j:j + 1, :] = jnp.broadcast_to(rsel, (1, 128))

    FT = [(f0, min(128, F - f0)) for f0 in range(0, F, 128)]

    class Ffn:
        def __init__(self):
            self.xs = xs_ref[...].astype(BF)
            self.acc = {}
            self.up = [(w, i, k) for i in range(len(FT)) for w in (0, 1) for k in range(D // 128)]
            self.down = [(i, k) for k in range(D // 128) for i in range(len(FT))]
            self.hid = None

        def add(self, key, d):
            self.acc[key] = d if key not in self.acc else self.acc[key] + d

        def run_up(self, n):
            for _ in range(min(n, len(self.up))):
                w, i, k = self.up.pop(0)
                f0, fn = FT[i]
                wt = (wg_ref, wu_ref)[w][f0:f0 + fn, k * 128:(k + 1) * 128]
                self.add((w, i), lax.dot_general(self.xs[:, k * 128:(k + 1) * 128], wt, NT, preferred_element_type=F32))

        def run_down(self, n):
            if self.hid is None:
                self.run_up(len(self.up))
                self.hid = []
                for i in range(len(FT)):
                    g = _rb(self.acc[(0, i)])
                    g = _rb(g * jax.nn.sigmoid(g))
                    self.hid.append((g * _rb(self.acc[(1, i)])).astype(BF))
            for _ in range(min(n, len(self.down))):
                i, k = self.down.pop(0)
                f0, fn = FT[i]
                self.add((2, k), jnp.dot(self.hid[i], wd_ref[f0:f0 + fn, k * 128:(k + 1) * 128], preferred_element_type=F32))

        def finish(self):
            self.run_down(len(self.down))
            y = _rb(jnp.concatenate([self.acc[(2, k)] for k in range(D // 128)], axis=1))
            y = _rb(y * _rb(jax.nn.sigmoid(rs_ref[:, 0:1])))
            b = _rb(xs_ref[...] + y)
            gs = b * jax.nn.sigmoid(b)
            for j in range(C):
                g_ref[pl.ds(idx_ref[j], 1), :] = gs[j:j + 1, :]

    def qproj(i, h, split=1, t=None, cx=None):
        parts = []
        n = TQ // split
        for c in range(split):
            r0 = i * TQ + c * n
            xn = dep_bf(xn_ref[r0:r0 + n, :], t)
            d = jnp.dot(xn, wq_ref[h], preferred_element_type=F32)
            if cx is not None:
                for r in ATOK:
                    cx.hist.append(d[r:r + 8, :])
            parts.append((d * QSCALE).astype(BF))
        return parts[0] if split == 1 else jnp.concatenate(parts, axis=0)

    def transpose_v(cx, hh, h):
        vt_ref[hh, pl.ds(cx.z1, DH // 2), :] = pltpu.bitcast(v_ref[h].T, U32)

    def qk(cx, n, h, q, jobs=(), after=(), ticks=None, qt=False):
        sv = s_refs[n % 2].at[pl.ds(cx.z1, NG * SP), :]
        ns = max(len(jobs) + 1, len(after))
        if ticks is not None:
            ns = TSL
        sl = S // ns
        m = None
        for j in range(ns):
            t = jobs[j - 1]() if 0 < j <= len(jobs) else None
            kj = dep_bf(k_ref[h, j * sl:(j + 1) * sl, :], t)
            if qt:
                sT = jnp.dot(kj, q, preferred_element_type=F32)
            else:
                sT = lax.dot_general(kj, q, NT, preferred_element_type=F32)
            for g in range(NG):
                sv[g * SP + j * sl:g * SP + (j + 1) * sl, :] = sT[:, g * 128:(g + 1) * 128]
            mj = jnp.max(jnp.max(sT.reshape(sl // 128, 16, 8, TQ), axis=1), axis=0)
            m = mj if m is None else jnp.maximum(m, mj)
            if j < len(after) and after[j] is not None:
                after[j](sT[0:8, 0:128])
            for fn, cnt_, off, span in (ticks or ()):
                for i in range(cnt_):
                    r = (off + i * (span - off) // cnt_) // 8 * 8 - j * sl
                    if 0 <= r < sl:
                        fn(sT[r:r + 8, 0:128])
        return jnp.broadcast_to(jnp.max(m, axis=0, keepdims=True), (8, TQ))

    def pv(cx, n, hh, m, hooks=None, groups=tuple(range(NG)), after=None, buf=0):
        sv = s_refs[n % 2].at[pl.ds(cx.z2, NG * SP), :]
        vv = vt_ref.at[hh, pl.ds(cx.z2, DH // 2), :]
        otv = ot_refs[buf].at[pl.ds(cx.z1, NG * DH), :]
        lrv = lr_refs[buf].at[pl.ds(cx.z1, NG * 8), :]
        CT = PV_CT
        for g in groups:
            mg = m[:, g * 128:(g + 1) * 128]
            l8 = None
            oT = None
            for c in range(S // 128 // CT):
                mc = mg
                if len(cx.hist) >= PV_DIST:
                    mc = dep_f32(mc, cx.tok(cx.hist[-PV_DIST]))
                if hooks and (g * 4 + c) in hooks:
                    mc = dep_f32(mc, hooks[g * 4 + c])
                ps = []
                for tt in range(CT):
                    r0 = (c * CT + tt) * 128
                    s = sv[g * SP + r0:g * SP + r0 + 128, :]
                    p = jnp.exp2(s - jnp.concatenate([mc] * 16, axis=0))
                    lt = None
                    for j in reversed(range(16)):
                        pj = p[j * 8:(j + 1) * 8, :]
                        lt = pj if lt is None else lt + pj
                    l8 = lt if l8 is None else l8 + lt
                    ps.append(p)
                vT = pltpu.bitcast(vv[:, c * CT * 128:(c + 1) * CT * 128], BF)
                part = jnp.dot(vT, jnp.concatenate(ps, axis=0).astype(BF), preferred_element_type=F32)
                cx.hist.append(part[0:8, :])
                if after and (g * 4 + c) in after:
                    after[g * 4 + c](part[0:8, :])
                oT = part if oT is None else oT + part
            otv[g * DH:(g + 1) * DH, :] = oT
            lrv[g * 8:(g + 1) * 8, :] = l8

    def load_o(cx, groups, buf=0):
        otv = ot_refs[buf].at[pl.ds(cx.z2, NG * DH), :]
        lrv = lr_refs[buf].at[pl.ds(cx.z2, NG * 8), :]
        parts = []
        for g in groups:
            l = jnp.sum(lrv[g * 8:(g + 1) * 8, :], axis=0, keepdims=True)
            parts.append((otv[g * DH:(g + 1) * DH, :] * (1.0 / l)).T.astype(BF))
        return parts[0] if len(parts) == 1 else jnp.concatenate(parts, axis=0)

    def oproj(cx, i, h, mode, groups=tuple(range(NG)), toks=True, o=None):
        r0 = i * TQ + groups[0] * 128
        r1 = r0 + len(groups) * 128
        if o is None:
            o = load_o(cx, groups)
        d = jnp.dot(o, wo_ref[h], preferred_element_type=F32)
        if mode == 'set':
            acc_ref[r0:r1, :] = d
        elif mode == 'add':
            acc_ref[r0:r1, :] += d
        else:
            s = acc_ref[r0:r1, :] + d
            out_ref[r0:r1, :] = (x_ref[r0:r1, :].astype(F32) + s * g_ref[r0:r1, :]).astype(BF)
        if toks:
            for r in DTOK:
                cx.hist.append(d[r:r + 8, 0:128])

    cp_x(0, SEM_A).start()
    cp_wq(0, SEM_A).start()
    cp_k(0, SEM_B).start()
    cp_x(1, SEM_B).start()
    cp_v(0, SEM_C).start()
    cp_x(2, SEM_D).start()
    cp_x(3, SEM_D).start()
    cp_wo(0, SEM_D).start()
    cp_wq(1, SEM_D).start()
    cp_wr.start()
    z_ref[0] = 0
    z_ref[1] = 0
    acc_ref[S - TQ:, :] = jnp.zeros((TQ, D), F32)

    def hide(i, c):
        z_ref[1] = z_ref[0] * i
        z_ref[0] = z_ref[1] * i
        return c

    lax.fori_loop(0, 2, hide, 0)
    cx = Ctx()
    rc = [jnp.zeros((8, 128), F32), jnp.zeros((8, 128), F32)]

    if LASTONLY:
        start_head(H - 1)
        for c in cp_ffn:
            c.start()
        def _b(i, c_):
            z_ref[1] = z_ref[0] * i
            z_ref[0] = z_ref[1] * i
            return c_
        lax.fori_loop(0, 3, _b, 0)
    elif LOOPONLY:
        start_head(1)
        for c in cp_ffn:
            c.start()
    else:
        cp_x(0, SEM_A).wait()
        cp_wq(0, SEM_A).wait()
        ln = LayerNorm(cx, 0, TQ, L0C, L0A, L0B)
        for _ in range(ln.steps):
            ln.step()
        q = qproj(0, 0, split=4)
        cp_k(0, SEM_B).wait()
        cp_x(1, SEM_B).wait()
        for hh in range(HPI):
            start_head(1 + hh)
        def hold_o(t):
            ot_ref[NG * DH:NG * DH + 8, :] = pltpu.bitcast(cx.tok(t), F32)

        ogate = [(hold_o, 1, OGT, OGT + 8)] if OGT else []
        for n in range(NB):
            if n == 1:
                cp_x(2, SEM_D).wait()
                cp_x(3, SEM_D).wait()
                cp_wo(0, SEM_D).wait()
                cp_wq(1, SEM_D).wait()
                cp_wr.wait()
                wrf_ref[...] = jnp.broadcast_to(wr_ref[...].astype(F32).reshape(1, D), (8, D))
                for c in cp_ffn:
                    c.start()
            if n + 1 < NB:
                ln = LayerNorm(cx, (n + 1) * TQ, TQ, LNC, LAG2, LAG3)
                if n == 0:
                    ln.step()
                    m = qk(cx, n, 0, q, ticks=[(ln.step, ln.steps - 1, 0, LSPAN0)])
                else:
                    m = qk(cx, n, 0, q, ticks=[(ln.step, ln.steps, LOFF, LSPAN)] + ogate)
            else:
                rn = S // RJOB
                st = [0]

                def rstep(t=None):
                    router(cx, st[0] * rn, rn, rc, t)
                    st[0] += 1

                m = qk(cx, n, 0, q, ticks=[(rstep, RJOB, ROFF, RSPAN)] + ogate)
                route(rc)
                if GREST == 0:
                    gate((H - 2) * GROWS, S - (H - 2) * GROWS)
            if n == 0:
                cp_v(0, SEM_C).wait()
                transpose_v(cx, 0, 0)
                q = qproj(1, 0)
            elif n + 1 < NB:
                if DA:
                    oproj(cx, n - 1, 0, 'set', toks=False)
                    q = qproj(n + 1, 0, cx=cx)
                else:
                    q = qproj(n + 1, 0)
                    oproj(cx, n - 1, 0, 'set')
            else:
                q = qproj(0, 1)
                oproj(cx, n - 1, 0, 'set')
            hooks = None
            if n + 1 == NB:
                qn_ref[...] = pltpu.bitcast(q.T if QT else q, U32)
                hooks = {RTH: cx.memtok(xs_ref) | cx.memtok(rs_ref)}
                if QTH0:
                    hooks[QTH0] = cx.memtok(qn_ref) | hooks.get(QTH0, cx.zvec)
            pv(cx, n, 0, m, hooks)

        if ONLYF:
            wait_head(1)
            for c in cp_ffn:
                c.wait()
            def _c(i, c_):
                o8 = pl.multiple_of(i * 16, 16)
                f = lambda r: r[pl.ds(o8, 16), 0:128].astype(BF)
                out_ref[0:16, 0:128] = (pltpu.bitcast(qn_ref[pl.ds(o8, 8), 0:128], BF) + f(ot_ref) + f(acc_ref) + f(xn_ref) + f(lr_ref) + f(g_ref)
                                        + (xs_ref[:, 0:128] + rs_ref[...])[0:1].astype(BF) + idx_ref[i].astype(BF))
                return c_
            lax.fori_loop(0, 2, _c, 0)
            cp_out(3).start()
            cp_out(3).wait()
            return
    if not LASTONLY:
        def body(it, _):
            h0 = 1 + it * HPI
            for hh in range(HPI):
                wait_head(h0 + hh)
            for hh in range(HPI):
                if hh == 0:
                    start_head(h0 + HPI)
                else:
                    @pl.when(h0 + HPI + hh < H)
                    def _():
                        start_head(h0 + HPI + hh)
            cx = Ctx()
            for hh in range(HPI):
                transpose_v(cx, hh, h0 + hh)
            q = pltpu.bitcast(qn_ref[...], BF)
            h_prev = h0 - 1
            for n in range(HPI * NB):
                hh, i = divmod(n, NB)
                hn, in_ = divmod(n + 1, NB)
                jobs = ()
                if n == GUN:
                    gate(pl.multiple_of(it * GROWS, GROWS), GROWS)
                if n == 0 and AFIRST:
                    q_next = qproj(in_, h0 + hn)
                    m = qk(cx, n, h0 + hh, q, jobs)
                    q = q_next
                else:
                    m = qk(cx, n, h0 + hh, q, jobs, qt=QT and n == 0)
                    q = qproj(in_, h0 + hn)
                oproj(cx, (i - 1) % NB, h_prev, 'add')
                hooks = None
                if n == HPI * NB - 1:
                    qn_ref[...] = pltpu.bitcast(q.T if QT else q, U32)
                    if QTH:
                        hooks = {QTH: cx.memtok(qn_ref)}
                pv(cx, n, hh, m, hooks)
                h_prev = h0 + hh
            return 0

        lax.fori_loop(0, (H - 2) // HPI, body, 0)

    h = H - 1
    wait_head(h)
    for c in cp_ffn:
        c.wait()
    if LOOPONLY:
        out_ref[0:16, 0:128] = pltpu.bitcast(qn_ref[0:8, 0:128], BF) + ot_ref[0:16, :].astype(BF) + acc_ref[0:16, 0:128].astype(BF) + g_ref[0:16, 0:128].astype(BF)
        cp_out(3).start()
        cp_out(3).wait()
        return
    cx = Ctx()
    transpose_v(cx, 0, h)
    q = pltpu.bitcast(qn_ref[...], BF)
    if GREST == 1:
        gate((H - 2) * GROWS, S - (H - 2) * GROWS)
    ffn = Ffn()
    cnt = lambda tot, j: (tot * (j + 1)) // (FSL - 1) - (tot * j) // (FSL - 1)
    m = qk(cx, 0, h, q, qt=QT, after=[(lambda t, j=j: ffn.run_up(cnt(70, j))) for j in range(FSL - 1)] + [None])
    q = qproj(1, h)
    oproj(cx, NB - 1, h - 1, 'add')
    pv(cx, 0, 0, m)
    m = qk(cx, 1, h, q, after=[(lambda t, j=j: ffn.run_up(cnt(70, j))) for j in range(FSL - 1)] + [None])
    q = qproj(2, h, cx=cx)
    pv(cx, 1, 0, m, buf=1)
    m = qk(cx, 2, h, q, after=[(lambda t, j=j: ffn.run_down(cnt(70, j))) for j in range(FSL - 1)] + [None])
    ffn.finish()
    q = qproj(3, h, t=None)
    allg = tuple(range(NG))
    oproj(cx, 0, h, 'fin', toks=False)
    if not ODEL:
        cp_out(0).start()
    oproj(cx, 1, h, 'fin', o=load_o(cx, allg, 1))
    if not ODEL:
        cp_out(1).start()
    pv(cx, 2, 0, m, {FINH: cx.memtok(out_ref)})

    def release(j):
        def fn(t):
            r0 = out_pieces[j][0]
            u = pltpu.bitcast(out_ref[r0:r0 + 16, 0:128], U32) | cx.tok(t)
            out_ref[r0:r0 + 16, 0:128] = pltpu.bitcast(u, BF)
            cp_out(j).start()
        return fn

    m = qk(cx, 3, h, q, ticks=[(release(0), 1, 0, 8), (release(1), 1, ODEL, ODEL + 8)] if ODEL else None)
    oproj(cx, 2, h, 'fin')
    cp_out(2).start()

    def tail_d(g, o):
        oproj(cx, NB - 1, h, 'fin', groups=(g,), toks=False, o=o)
        cp_out(NB - 1 + g).start()

    ftok = cx.memtok(out_ref)
    os = []
    done = 0
    for g in range(NG):
        pv(cx, NB - 1, 0, m, {FINH: ftok}, groups=(g,))
        os.append(load_o(cx, (g,)))
        if g >= TLAG and done < TORD:
            tail_d(done, os[done])
            done += 1
    for g in range(done, NG):
        tail_d(g, os[g])
    for j in range(len(out_pieces)):
        cp_out(j).wait()


@jax.jit
def pallas_recurrent_scan__mha_block_cached__moe_arch_mod__prompt_kernel(
    A_x, A_k_cache, A_v_cache, A_wq, A_wo, B_x, B_w_r, B_w_gate, B_w_up, B_w_down):
    x = A_x.reshape(S, D)
    k = A_k_cache.reshape(H, S, DH)
    v = A_v_cache.reshape(H, S, DH)
    wo = A_wo.reshape(H, DH, D)
    wr = B_w_r
    anyspec = pl.BlockSpec(memory_space=pl.ANY)
    out = pl.pallas_call(
        _kernel,
        in_specs=[anyspec] * 9,
        out_specs=anyspec,
        out_shape=jax.ShapeDtypeStruct((S, D), BF),
        scratch_shapes=[
            pltpu.VMEM((NG * SP, 128), F32),
            pltpu.VMEM((NG * SP, 128), F32),
            pltpu.VMEM((HPI, DH // 2, S), U32),
            pltpu.VMEM((NG * DH + 32, 128), F32),
            pltpu.VMEM((NG * DH, 128), F32),
            pltpu.VMEM((S, D), F32),
            pltpu.VMEM((DH // 2, TQ) if QT else (TQ // 2, DH), U32),
            pltpu.VMEM((H, S, DH), BF),
            pltpu.VMEM((H, S, DH), BF),
            pltpu.VMEM((H, D, DH), BF),
            pltpu.VMEM((H, DH, D), BF),
            pltpu.VMEM((S + 64, D), BF),
            pltpu.VMEM((S, D), F32),
            pltpu.VMEM((S, D), BF),
            pltpu.VMEM((F, D), BF),
            pltpu.VMEM((F, D), BF),
            pltpu.VMEM((F, D), BF),
            pltpu.VMEM((S + 64, D), BF),
            pltpu.VMEM((NG * 8, 128), F32),
            pltpu.VMEM((NG * 8, 128), F32),
            pltpu.VMEM((C, D), F32),
            pltpu.VMEM((C, 128), F32),
            pltpu.VMEM((8, D), F32),
            pltpu.VMEM((D,), BF),
            pltpu.SMEM((2,), jnp.int32),
            pltpu.SMEM((C,), jnp.int32),
            pltpu.SemaphoreType.DMA((7,)),
        ],
        compiler_params=pltpu.CompilerParams(
            vmem_limit_bytes=126 * 1024 * 1024,
            internal_scratch_in_bytes=16 * 4096,
            disable_bounds_checks=True,
            disable_semaphore_checks=True,
        ),
    )(x, k, v, A_wq, wo, wr, B_w_gate.T, B_w_up.T, B_w_down)
    return out.reshape(1, S, D)
```

```python
import math
import jax
import jax.numpy as jnp
from jax import lax
import jax.experimental.pallas as pl
import jax.experimental.pallas.tpu as pltpu

S, D, H, DH, F, C = 2048, 640, 32, 128, 1728, 8
TQ = 512
NB = S // TQ
NG = TQ // 128
BF = jnp.bfloat16
F32 = jnp.float32
U32 = jnp.uint32
QSCALE = (DH ** -0.5) * math.log2(math.e)
E = lambda k, d: d
PV_CT = E('PV_CT', 4)
PV_DIST = E('PV_DIST', 3)
HPI = E('HPI', 1)
LNC = E('LNC', 8)
RC_ = 16
RJOB = E('RJOB', 64)
LAG3B = E('LAG3B', 12)
UP0 = E('UP0', 60)
LQT = E('LQT', 1)
LQH = E('LQH', 8)
XF = E('XF', 4)
XD = E('XD', 4)
XD2 = E('XD2', 6)
RSPAN = E('RSPAN', 1900)
LAG2 = E('LAG2', 4)
TSL = E('TSL', 1)
LAG3 = E('LAG3', 10)
LOFF = E('LOFF', 0)
ROFF = E('ROFF', 0)
DA = E('DA', 0)
QT = E('QT', 1)
ODEL = E('ODEL', 0)
TORD = E('TORD', 1)
TLAG = E('TLAG', 2)
QTH = E('QTH', 4)
QTH0 = E('QTH0', 10)
OGT = E('OGT', 0)
LSPAN0 = E('LSPAN0', 2000)
LSPAN = E('LSPAN', 2040)
L0C = E('L0C', 32)
L0A = E('L0A', 0)
L0B = E('L0B', 0)
ATOK = ()
NJOB = E('NJOB', 8)
AFIRST = E('AFIRST', 0)
ONLYF = E('ONLYF', 0)
TAILH = E('TAILH', 0)
FSL = E('FSL', 16)
FH0 = E('FH0', 9)
RTH = E('RTH', 14)
LASTONLY = E('LASTONLY', 0)
LOOPONLY = E('LOOPONLY', 0)
GSPL = E('GSPL', 1)
GUN = E('GUN', 1)
GMODE = E('GMODE', 0)
LN_DIST = E('LN_DIST', 2)
GROWS = E('GROWS', 64)
SP = S + 8
GREST = E('GREST', 0)
FINH = E('FINH', 6)
DTOK = (128, 256, 384)
SUMA = E('SUMA', 1)
MAXS = E('MAXS', 16)
OPAD = E('OPAD', 0)
DFIRST = E('DFIRST', 0)
NT = (((1,), (1,)), ((), ()))


def _rb(a):
    return a.astype(BF).astype(F32)


def _kernel(x_hbm, k_hbm, v_hbm, wq_hbm, wo_hbm, wr_hbm, wg_hbm, wu_hbm, wd_hbm,
            o_hbm,
            s0_ref, s1_ref, vt_ref, ot_ref, ot2_ref, acc_ref, qn_ref,
            k_ref, v_ref, wq_ref, wo_ref, xn_ref, g_ref, out_ref, wg_ref, wu_ref, wd_ref,
            x_ref, lr_ref, lr2_ref, xs_ref, rs_ref, wrf_ref, wr_ref, z_ref, idx_ref, sem):
    s_refs = (s0_ref, s1_ref)
    ot_refs = (ot_ref, ot2_ref)
    lr_refs = (lr_ref, lr2_ref)

    SEM_A, SEM_B, SEM_C, SEM_D, SEM_H, SEM_F, SEM_O = range(7)

    def cp_k(h, s=SEM_H):
        return pltpu.make_async_copy(k_hbm.at[h], k_ref.at[h], sem.at[s])

    def cp_v(h, s=SEM_H):
        return pltpu.make_async_copy(v_hbm.at[h], v_ref.at[h], sem.at[s])

    def cp_wq(h, s=SEM_H):
        off = h * DH if isinstance(h, int) else pl.multiple_of(h * DH, DH)
        return pltpu.make_async_copy(wq_hbm.at[:, pl.ds(off, DH)], wq_ref.at[h], sem.at[s])

    def cp_wo(h, s=SEM_H):
        return pltpu.make_async_copy(wo_hbm.at[h], wo_ref.at[h], sem.at[s])

    def cp_x(i, s):
        return pltpu.make_async_copy(x_hbm.at[pl.ds(i * TQ, TQ)], x_ref.at[pl.ds(i * TQ, TQ)], sem.at[s])

    cp_ffn = [pltpu.make_async_copy(wg_hbm, wg_ref, sem.at[SEM_F]),
              pltpu.make_async_copy(wu_hbm, wu_ref, sem.at[SEM_F]),
              pltpu.make_async_copy(wd_hbm, wd_ref, sem.at[SEM_F])]

    cp_wr = pltpu.make_async_copy(wr_hbm, wr_ref, sem.at[SEM_D])

    out_pieces = [(i * TQ, TQ) for i in range(NB - 1)] + [(S - TQ + g * 128, 128) for g in range(NG)]

    def cp_out(j):
        r0, n = out_pieces[j]
        return pltpu.make_async_copy(out_ref.at[pl.ds(r0, n)], o_hbm.at[pl.ds(r0, n)], sem.at[SEM_O])

    def start_head(h):
        cp_k(h).start()
        cp_v(h).start()
        cp_wo(h).start()
        if isinstance(h, int):
            if h + 1 < H:
                cp_wq(h + 1).start()
        else:
            @pl.when(h + 1 < H)
            def _():
                cp_wq(h + 1).start()

    def wait_head(h):
        cp_k(h).wait()
        cp_v(h).wait()
        cp_wo(h).wait()
        if not isinstance(h, int) or h + 1 < H:
            cp_wq(h + 1).wait()

    lane = lax.broadcasted_iota(jnp.int32, (8, 128), 1)
    sub = lax.broadcasted_iota(jnp.int32, (8, 128), 0)

    class Ctx:
        def __init__(self):
            self.z1 = pl.multiple_of(z_ref[0], 8)
            self.z2 = pl.multiple_of(z_ref[1], 8)
            self.zvec = jnp.full((8, 128), z_ref[0], jnp.int32).astype(U32)
            self.hist = []
            self.lnh = []

        def tok(self, a):
            return pltpu.bitcast(a, U32) & self.zvec

        def memtok(self, ref):
            rows = 16 if ref.dtype == BF else 8
            z = pl.multiple_of(self.z2 * 2, 16)
            return self.tok(ref[pl.ds(z, rows), 0:128])

    def dep_bf(a, t):
        if t is None:
            return a
        au = pltpu.bitcast(a, U32)
        first = au[0:8, 0:128] | t
        top = first if au.shape[1] == 128 else jnp.concatenate([first, au[0:8, 128:]], axis=1)
        return pltpu.bitcast(jnp.concatenate([top, au[8:]], axis=0), BF)

    def dep_f32(a, t):
        return pltpu.bitcast(pltpu.bitcast(a, U32) | t, F32)

    class LayerNorm:
        def __init__(self, cx, r0, n, c, lag2, lag3):
            self.cx, self.r0, self.c, self.n = cx, r0, c, n // c
            self.lag2, self.lag3 = lag2, lag3
            self.k = 0
            self.mean, self.inv = {}, {}
            self.steps = self.n + lag3

        def step(self, gate_tok=None):
            cx, c, k = self.cx, self.c, self.k
            self.k += 1
            xv = x_ref.at[pl.ds(pl.multiple_of(cx.z2 * 2, 16), S), :]
            xw = x_ref.at[pl.ds(pl.multiple_of(cx.z1 * 2, 16), S), :]
            xu = x_ref.at[pl.ds(pl.multiple_of((cx.z1 + cx.z2) * 2, 16), S), :]
            if gate_tok is not None:
                x_ref[S:S + 16, 0:128] = pltpu.bitcast(cx.tok(gate_tok), BF)
            if k < self.n:
                a = self.r0 + k * c
                self.mean[k] = jnp.mean(xv[a:a + c, :].astype(F32), axis=-1, keepdims=True)
            j = k - self.lag2
            if 0 <= j < self.n:
                a = self.r0 + j * c
                xc = xw[a:a + c, :].astype(F32) - self.mean[j]
                v = _rb(_rb(jnp.mean(xc * xc, axis=-1, keepdims=True)) + 1e-5)
                den = _rb(v * lax.rsqrt(v))
                inv = pl.reciprocal(den, approx=True)
                self.inv[j] = inv * (2.0 - den * inv)
            j = k - self.lag3
            if 0 <= j < self.n:
                a = self.r0 + j * c
                d = _rb(xu[a:a + c, :].astype(F32) - _rb(self.mean[j]))
                xn_ref[a:a + c, :] = (d * self.inv[j]).astype(BF)

    def silu(b):
        hb = 0.5 * b
        return hb + hb * jnp.tanh(hb)

    def gate(r0, n):
        xf = xn_ref[pl.ds(r0, n), :].astype(F32)
        g_ref[pl.ds(r0, n), :] = silu(xf)
        return xf

    def router(cx, r0, n, rc, gate_tok=None):
        xv = xn_ref.at[pl.ds(pl.multiple_of(cx.z2 * 2, 16), S), :]
        if gate_tok is not None:
            xn_ref[S:S + 16, 0:128] = pltpu.bitcast(cx.tok(gate_tok), BF)
        for c in range(n // RC_):
            a = r0 + c * RC_
            xf = xv[a:a + RC_, :].astype(F32)
            r = _rb(jnp.sum(xf * jnp.concatenate([wrf_ref[...]] * (RC_ // 8), axis=0), axis=-1, keepdims=True))
            for j in range(RC_ // 8):
                gi = a // 8 + j
                rc[gi // 128] = jnp.where(lane == gi % 128, r[j * 8:(j + 1) * 8, :], rc[gi // 128])

    def route(rc):
        r = jnp.concatenate(rc, axis=0)
        tix = jnp.concatenate([(8 * (128 * a + lane) + sub) for a in range(2)], axis=0).astype(F32)
        rw = jnp.where(r != r, -jnp.inf, r)
        alive = jnp.ones((16, 128), F32)
        for j in range(C):
            mx = jnp.max(jnp.max(rw, axis=0, keepdims=True), axis=1, keepdims=True)
            cand = jnp.where((rw == mx) & (alive > 0), tix, float(S - 1))
            ixv = jnp.min(jnp.min(cand, axis=0, keepdims=True), axis=1, keepdims=True)
            hit = tix == ixv
            rsel = jnp.sum(jnp.sum(jnp.where(hit, r, 0.0), axis=0, keepdims=True), axis=1, keepdims=True)
            rw = jnp.where(hit, -jnp.inf, rw)
            alive = jnp.where(hit, 0.0, alive)
            ix = ixv.astype(jnp.int32)[0, 0]
            idx_ref[j] = ix
            blk = xn_ref[pl.ds(pl.multiple_of((ix // 16) * 16, 16), 16), :].astype(F32)
            pick = lax.broadcasted_iota(jnp.int32, (16, D), 0) == (ixv.astype(jnp.int32) & 15)
            xs_ref[j:j + 1, :] = jnp.sum(jnp.where(pick, blk, 0.0), axis=0, keepdims=True)
            rs_ref[j:j + 1, :] = jnp.broadcast_to(rsel, (1, 128))

    FT = [(f0, min(128, F - f0)) for f0 in range(0, F, 128)]

    class Ffn:
        def __init__(self):
            self.xs = xs_ref[...].astype(BF)
            self.acc = {}
            self.up = [(w, i, k) for i in range(len(FT)) for w in (0, 1) for k in range(D // 128)]
            self.down = [(i, k) for k in range(D // 128) for i in range(len(FT))]
            self.hid = None

        def add(self, key, d):
            self.acc[key] = d if key not in self.acc else self.acc[key] + d

        def run_up(self, n):
            for _ in range(min(n, len(self.up))):
                w, i, k = self.up.pop(0)
                f0, fn = FT[i]
                wt = (wg_ref, wu_ref)[w][f0:f0 + fn, k * 128:(k + 1) * 128]
                self.add((w, i), lax.dot_general(self.xs[:, k * 128:(k + 1) * 128], wt, NT, preferred_element_type=F32))

        def run_down(self, n):
            if self.hid is None:
                self.run_up(len(self.up))
                self.hid = []
                for i in range(len(FT)):
                    g = _rb(self.acc[(0, i)])
                    g = _rb(g * jax.nn.sigmoid(g))
                    self.hid.append((g * _rb(self.acc[(1, i)])).astype(BF))
            for _ in range(min(n, len(self.down))):
                i, k = self.down.pop(0)
                f0, fn = FT[i]
                self.add((2, k), jnp.dot(self.hid[i], wd_ref[f0:f0 + fn, k * 128:(k + 1) * 128], preferred_element_type=F32))

        def finish(self):
            self.run_down(len(self.down))
            y = _rb(jnp.concatenate([self.acc[(2, k)] for k in range(D // 128)], axis=1))
            y = _rb(y * _rb(jax.nn.sigmoid(rs_ref[:, 0:1])))
            b = _rb(xs_ref[...] + y)
            gs = b * jax.nn.sigmoid(b)
            for j in range(C):
                g_ref[pl.ds(idx_ref[j], 1), :] = gs[j:j + 1, :]

    def qproj(i, h, split=1, t=None, cx=None):
        parts = []
        n = TQ // split
        for c in range(split):
            r0 = i * TQ + c * n
            xn = dep_bf(xn_ref[r0:r0 + n, :], t)
            d = jnp.dot(xn, wq_ref[h], preferred_element_type=F32)
            if cx is not None:
                for r in ATOK:
                    cx.hist.append(d[r:r + 8, :])
            parts.append((d * QSCALE).astype(BF))
        return parts[0] if split == 1 else jnp.concatenate(parts, axis=0)

    def transpose_v(cx, hh, h):
        vt_ref[hh, pl.ds(cx.z1, DH // 2), :] = pltpu.bitcast(v_ref[h].T, U32)

    def qk(cx, n, h, q, jobs=(), after=(), ticks=None, qt=False):
        sv = s_refs[n % 2].at[pl.ds(cx.z1, NG * SP), :]
        ns = max(len(jobs) + 1, len(after))
        if ticks is not None:
            ns = TSL
        sl = S // ns
        m = None
        for j in range(ns):
            t = jobs[j - 1]() if 0 < j <= len(jobs) else None
            kj = dep_bf(k_ref[h, j * sl:(j + 1) * sl, :], t)
            if qt:
                sT = jnp.dot(kj, q, preferred_element_type=F32)
            else:
                sT = lax.dot_general(kj, q, NT, preferred_element_type=F32)
            for g in range(NG):
                sv[g * SP + j * sl:g * SP + (j + 1) * sl, :] = sT[:, g * 128:(g + 1) * 128]
            mj = jnp.max(jnp.max(sT.reshape(-1, min(MAXS, sl // 8), 8, TQ), axis=1), axis=0)
            m = mj if m is None else jnp.maximum(m, mj)
            if j < len(after) and after[j] is not None:
                after[j](sT[0:8, 0:128])
            for fn, cnt_, off, span in (ticks or ()):
                for i in range(cnt_):
                    r = (off + i * (span - off) // cnt_) // 8 * 8 - j * sl
                    if 0 <= r < sl:
                        fn(sT[r:r + 8, 0:128])
        return jnp.broadcast_to(jnp.max(m, axis=0, keepdims=True), (8, TQ))

    def pv(cx, n, hh, m, hooks=None, groups=tuple(range(NG)), after=None, buf=0):
        sv = s_refs[n % 2].at[pl.ds(cx.z2, NG * SP), :]
        vv = vt_ref.at[hh, pl.ds(cx.z2, DH // 2), :]
        otv = ot_refs[buf].at[pl.ds(cx.z1, NG * DH), :]
        lrv = lr_refs[buf].at[pl.ds(cx.z1, NG * 8), :]
        CT = PV_CT
        for g in groups:
            mg = m[:, g * 128:(g + 1) * 128]
            l8 = None
            la = [None] * CT
            oT = None
            for c in range(S // 128 // CT):
                mc = mg
                if len(cx.hist) >= PV_DIST:
                    mc = dep_f32(mc, cx.tok(cx.hist[-PV_DIST]))
                if hooks and (g * (16 // CT) + c) * (CT // 4 if CT >= 4 else 1) in hooks and CT == 4:
                    mc = dep_f32(mc, hooks[g * 4 + c])
                ps = []
                for tt in range(CT):
                    r0 = (c * CT + tt) * 128
                    s = sv[g * SP + r0:g * SP + r0 + 128, :]
                    p = jnp.exp2(s - jnp.concatenate([mc] * 16, axis=0))
                    if SUMA == 0:
                        for j in reversed(range(16)):
                            pj = p[j * 8:(j + 1) * 8, :]
                            la[tt] = pj if la[tt] is None else la[tt] + pj
                    else:
                        lt = None
                        for j in reversed(range(16)):
                            pj = p[j * 8:(j + 1) * 8, :]
                            lt = pj if lt is None else lt + pj
                        l8 = lt if l8 is None else l8 + lt
                    ps.append(p)
                vT = pltpu.bitcast(vv[:, c * CT * 128:(c + 1) * CT * 128], BF)
                part = jnp.dot(vT, jnp.concatenate(ps, axis=0).astype(BF), preferred_element_type=F32)
                cx.hist.append(part[0:8, :])
                if after and (g * 4 + c) in after:
                    after[g * 4 + c](part[0:8, :])
                oT = part if oT is None else oT + part
            if SUMA == 0:
                l8 = la[0]
                for a_ in la[1:]:
                    l8 = l8 + a_
            otv[g * DH:(g + 1) * DH, :] = oT
            lrv[g * 8:(g + 1) * 8, :] = l8

    def load_o(cx, groups, buf=0):
        otv = ot_refs[buf].at[pl.ds(cx.z2, NG * DH), :]
        lrv = lr_refs[buf].at[pl.ds(cx.z2, NG * 8), :]
        parts = []
        for g in groups:
            l = jnp.sum(lrv[g * 8:(g + 1) * 8, :], axis=0, keepdims=True)
            parts.append((otv[g * DH:(g + 1) * DH, :] * (1.0 / l)).T.astype(BF))
        return parts[0] if len(parts) == 1 else jnp.concatenate(parts, axis=0)

    def oproj(cx, i, h, mode, groups=tuple(range(NG)), toks=True, o=None):
        r0 = i * TQ + groups[0] * 128
        r1 = r0 + len(groups) * 128
        if o is None:
            o = load_o(cx, groups)
        d = jnp.dot(o, wo_ref[h], preferred_element_type=F32)
        if mode == 'set':
            acc_ref[r0:r1, :] = d
        elif mode == 'add':
            acc_ref[r0:r1, :] += d
        else:
            s = acc_ref[r0:r1, :] + d
            out_ref[r0:r1, :] = (x_ref[r0:r1, :].astype(F32) + s * g_ref[r0:r1, :]).astype(BF)
        if toks:
            for r in DTOK:
                cx.hist.append(d[r:r + 8, 0:128])

    cp_x(0, SEM_A).start()
    cp_wq(0, SEM_A).start()
    cp_k(0, SEM_B).start()
    cp_x(1, SEM_B).start()
    cp_v(0, SEM_C).start()
    cp_x(2, SEM_D).start()
    cp_x(3, SEM_D).start()
    cp_wo(0, SEM_D).start()
    cp_wq(1, SEM_D).start()
    cp_wr.start()
    z_ref[0] = 0
    z_ref[1] = 0
    acc_ref[S - TQ:, :] = jnp.zeros((TQ, D), F32)

    def hide(i, c):
        z_ref[1] = z_ref[0] * i
        z_ref[0] = z_ref[1] * i
        return c

    lax.fori_loop(0, 2, hide, 0)
    cx = Ctx()
    rc = [jnp.zeros((8, 128), F32), jnp.zeros((8, 128), F32)]

    if LASTONLY:
        start_head(H - 1)
        for c in cp_ffn:
            c.start()
        def _b(i, c_):
            z_ref[1] = z_ref[0] * i
            z_ref[0] = z_ref[1] * i
            return c_
        lax.fori_loop(0, 3, _b, 0)
    elif LOOPONLY:
        start_head(1)
        for c in cp_ffn:
            c.start()
    else:
        cp_x(0, SEM_A).wait()
        cp_wq(0, SEM_A).wait()
        ln = LayerNorm(cx, 0, TQ, L0C, L0A, L0B)
        for _ in range(ln.steps):
            ln.step()
        q = qproj(0, 0, split=4)
        cp_k(0, SEM_B).wait()
        cp_x(1, SEM_B).wait()
        for hh in range(HPI):
            start_head(1 + hh)
        def hold_o(t):
            ot_ref[NG * DH:NG * DH + 8, :] = pltpu.bitcast(cx.tok(t), F32)

        ogate = [(hold_o, 1, OGT, OGT + 8)] if OGT else []
        for n in range(NB):
            if n == 1:
                cp_x(2, SEM_D).wait()
                cp_x(3, SEM_D).wait()
                cp_wo(0, SEM_D).wait()
                cp_wq(1, SEM_D).wait()
                cp_wr.wait()
                wrf_ref[...] = jnp.broadcast_to(wr_ref[...].astype(F32).reshape(1, D), (8, D))
                for c in cp_ffn:
                    c.start()
            if n + 1 < NB:
                ln = LayerNorm(cx, (n + 1) * TQ, TQ, LNC, LAG2, LAG3 if n == 0 else LAG3B)
                if n == 0:
                    ln.step()
                    m = qk(cx, n, 0, q, ticks=[(ln.step, ln.steps - 1, 0, LSPAN0)])
                else:
                    m = qk(cx, n, 0, q, ticks=[(ln.step, ln.steps, LOFF, LSPAN)] + ogate)
            else:
                rn = S // RJOB
                st = [0]

                def rstep(t=None):
                    router(cx, st[0] * rn, rn, rc, t)
                    st[0] += 1

                m = qk(cx, n, 0, q, ticks=[(rstep, RJOB, ROFF, RSPAN)] + ogate)
                route(rc)
                if GREST == 0:
                    gate((H - 2) * GROWS, S - (H - 2) * GROWS)
            if n == 0:
                cp_v(0, SEM_C).wait()
                transpose_v(cx, 0, 0)
                q = qproj(1, 0)
            elif n + 1 < NB:
                if DA:
                    oproj(cx, n - 1, 0, 'set', toks=False)
                    q = qproj(n + 1, 0, cx=cx)
                else:
                    q = qproj(n + 1, 0)
                    oproj(cx, n - 1, 0, 'set')
            else:
                q = qproj(0, 1)
                oproj(cx, n - 1, 0, 'set')
            hooks = None
            if n + 1 == NB:
                qn_ref[...] = pltpu.bitcast(q.T if QT else q, U32)
                hooks = {RTH: cx.memtok(xs_ref) | cx.memtok(rs_ref)}
                if QTH0:
                    hooks[QTH0] = cx.memtok(qn_ref) | hooks.get(QTH0, cx.zvec)
            pv(cx, n, 0, m, hooks)

        if ONLYF:
            wait_head(1)
            for c in cp_ffn:
                c.wait()
            def _c(i, c_):
                o8 = pl.multiple_of(i * 16, 16)
                f = lambda r: r[pl.ds(o8, 16), 0:128].astype(BF)
                out_ref[0:16, 0:128] = (pltpu.bitcast(qn_ref[pl.ds(o8, 8), 0:128], BF) + f(ot_ref) + f(acc_ref) + f(xn_ref) + f(lr_ref) + f(g_ref)
                                        + (xs_ref[:, 0:128] + rs_ref[...])[0:1].astype(BF) + idx_ref[i].astype(BF))
                return c_
            lax.fori_loop(0, 2, _c, 0)
            cp_out(3).start()
            cp_out(3).wait()
            return
    if not LASTONLY:
        def body(it, _):
            h0 = 1 + it * HPI
            for hh in range(HPI):
                wait_head(h0 + hh)
            for hh in range(HPI):
                if hh == 0:
                    start_head(h0 + HPI)
                else:
                    @pl.when(h0 + HPI + hh < H)
                    def _():
                        start_head(h0 + HPI + hh)
            cx = Ctx()
            for hh in range(HPI):
                transpose_v(cx, hh, h0 + hh)
            q = pltpu.bitcast(qn_ref[...], BF)
            h_prev = h0 - 1
            for n in range(HPI * NB):
                hh, i = divmod(n, NB)
                hn, in_ = divmod(n + 1, NB)
                jobs = ()
                if n == GUN:
                    gate(pl.multiple_of(it * GROWS, GROWS), GROWS)
                if n == 0 and AFIRST:
                    q_next = qproj(in_, h0 + hn)
                    m = qk(cx, n, h0 + hh, q, jobs)
                    q = q_next
                else:
                    m = qk(cx, n, h0 + hh, q, jobs, qt=QT and n == 0)
                    if DFIRST:
                        oproj(cx, (i - 1) % NB, h_prev, 'add')
                    q = qproj(in_, h0 + hn)
                if not DFIRST:
                    oproj(cx, (i - 1) % NB, h_prev, 'add')
                hooks = None
                if n == HPI * NB - 1:
                    qn_ref[...] = pltpu.bitcast(q.T if QT else q, U32)
                    if QTH:
                        hooks = {QTH: cx.memtok(qn_ref)}
                pv(cx, n, hh, m, hooks)
                h_prev = h0 + hh
            return 0

        lax.fori_loop(0, (H - 2) // HPI, body, 0)

    h = H - 1
    wait_head(h)
    for c in cp_ffn:
        c.wait()
    if LOOPONLY:
        out_ref[0:16, 0:128] = pltpu.bitcast(qn_ref[0:8, 0:128], BF) + ot_ref[0:16, :].astype(BF) + acc_ref[0:16, 0:128].astype(BF) + g_ref[0:16, 0:128].astype(BF)
        cp_out(3).start()
        cp_out(3).wait()
        return
    cx = Ctx()
    transpose_v(cx, 0, h)
    q = pltpu.bitcast(qn_ref[...], BF)
    if GREST == 1:
        gate((H - 2) * GROWS, S - (H - 2) * GROWS)
    ffn = Ffn()
    cnt = lambda tot, j: (tot * (j + 1)) // (FSL - 1) - (tot * j) // (FSL - 1)
    def next_q(i):
        q = qproj(i, h)
        if not LQT:
            return q, None
        qn_ref[...] = pltpu.bitcast(q.T, U32)
        t = cx.memtok(qn_ref)
        z = pl.multiple_of(cx.z1, 8)
        return pltpu.bitcast(qn_ref[pl.ds(z, DH // 2), :], BF), {LQH: t}

    m = qk(cx, 0, h, q, qt=QT, after=[(lambda t, j=j: ffn.run_up(cnt(UP0, j))) for j in range(FSL - 1)] + [None])
    ffn.run_up(XF)
    q, hk = next_q(1)
    ffn.run_up(XF)
    oproj(cx, NB - 1, h - 1, 'add')
    pv(cx, 0, 0, m, hk)
    ffn.run_up(XF)
    rest = len(ffn.up) - XF
    m = qk(cx, 1, h, q, qt=LQT, after=[(lambda t, j=j: ffn.run_up(cnt(rest, j))) for j in range(FSL - 1)] + [None])
    ffn.run_up(XF)
    q, hk = next_q(2)
    pv(cx, 1, 0, m, hk, buf=1)
    ffn.run_down(XD)
    rest2 = len(ffn.down) - XD2
    m = qk(cx, 2, h, q, qt=LQT, after=[(lambda t, j=j: ffn.run_down(cnt(rest2, j))) for j in range(FSL - 1)] + [None])
    ffn.finish()
    q = qproj(3, h, t=None)
    allg = tuple(range(NG))
    oproj(cx, 0, h, 'fin', toks=False)
    if not ODEL:
        cp_out(0).start()
    oproj(cx, 1, h, 'fin', o=load_o(cx, allg, 1))
    if not ODEL:
        cp_out(1).start()
    pv(cx, 2, 0, m, {FINH: cx.memtok(out_ref)})

    def release(j):
        def fn(t):
            r0 = out_pieces[j][0]
            u = pltpu.bitcast(out_ref[r0:r0 + 16, 0:128], U32) | cx.tok(t)
            out_ref[r0:r0 + 16, 0:128] = pltpu.bitcast(u, BF)
            cp_out(j).start()
        return fn

    m = qk(cx, 3, h, q, ticks=[(release(0), 1, 0, 8), (release(1), 1, ODEL, ODEL + 8)] if ODEL else None)
    oproj(cx, 2, h, 'fin')
    cp_out(2).start()

    def tail_d(g, o):
        oproj(cx, NB - 1, h, 'fin', groups=(g,), toks=False, o=o)
        cp_out(NB - 1 + g).start()

    ftok = cx.memtok(out_ref)
    os = []
    done = 0
    for g in range(NG):
        pv(cx, NB - 1, 0, m, {FINH: ftok}, groups=(g,))
        os.append(load_o(cx, (g,)))
        if g >= TLAG and done < TORD:
            tail_d(done, os[done])
            done += 1
    for g in range(done, NG):
        tail_d(g, os[g])
    for j in range(len(out_pieces)):
        cp_out(j).wait()


@jax.jit
def pallas_recurrent_scan__mha_block_cached__moe_arch_mod__prompt_kernel(
    A_x, A_k_cache, A_v_cache, A_wq, A_wo, B_x, B_w_r, B_w_gate, B_w_up, B_w_down):
    x = A_x.reshape(S, D)
    k = A_k_cache.reshape(H, S, DH)
    v = A_v_cache.reshape(H, S, DH)
    wo = A_wo.reshape(H, DH, D)
    wr = B_w_r
    anyspec = pl.BlockSpec(memory_space=pl.ANY)
    out = pl.pallas_call(
        _kernel,
        in_specs=[anyspec] * 9,
        out_specs=anyspec,
        out_shape=jax.ShapeDtypeStruct((S, D), BF),
        scratch_shapes=[
            pltpu.VMEM((NG * SP, 128), F32),
            pltpu.VMEM((NG * SP, 128), F32),
            pltpu.VMEM((HPI, DH // 2, S), U32),
            pltpu.VMEM((NG * DH + 32, 128), F32),
            pltpu.VMEM((NG * DH, 128), F32),
            pltpu.VMEM((S, D), F32),
            pltpu.VMEM((DH // 2, TQ) if QT else (TQ // 2, DH), U32),
            pltpu.VMEM((H, S, DH), BF),
            pltpu.VMEM((H, S, DH), BF),
            pltpu.VMEM((H, D, DH), BF),
            pltpu.VMEM((H, DH, D), BF),
            pltpu.VMEM((S + 64, D), BF),
            pltpu.VMEM((S, D), F32),
            pltpu.VMEM((S, D), BF),
            pltpu.VMEM((F, D), BF),
            pltpu.VMEM((F, D), BF),
            pltpu.VMEM((F, D), BF),
            pltpu.VMEM((S + 64, D), BF),
            pltpu.VMEM((NG * 8, 128), F32),
            pltpu.VMEM((NG * 8, 128), F32),
            pltpu.VMEM((C, D), F32),
            pltpu.VMEM((C, 128), F32),
            pltpu.VMEM((8, D), F32),
            pltpu.VMEM((D,), BF),
            pltpu.SMEM((2,), jnp.int32),
            pltpu.SMEM((C,), jnp.int32),
            pltpu.SemaphoreType.DMA((7,)),
        ],
        compiler_params=pltpu.CompilerParams(
            vmem_limit_bytes=126 * 1024 * 1024,
            internal_scratch_in_bytes=16 * 4096,
            disable_bounds_checks=True,
            disable_semaphore_checks=True,
        ),
    )(x, k, v, A_wq, wo, wr, B_w_gate.T, B_w_up.T, B_w_down)
    return out.reshape(1, S, D)
```

```python
import math

import jax
import jax.numpy as jnp
from jax import lax
import jax.experimental.pallas as pl
import jax.experimental.pallas.tpu as pltpu

S, D, H, DH, F, C = 2048, 640, 32, 128, 1728, 8
TQ = 512
NB = S // TQ
NG = TQ // 128
CT = 4
NCH = S // 128 // CT
SP = S + 8
GROWS = 64
BF, F32, U32 = jnp.bfloat16, jnp.float32, jnp.uint32
QSCALE = (DH ** -0.5) * math.log2(math.e)
NT = (((1,), (1,)), ((), ()))
PV_DIST = 3
FSL = 16
SEM_A, SEM_B, SEM_C, SEM_D, SEM_H, SEM_F, SEM_O = range(7)
OUT_PIECES = [(i * TQ, TQ) for i in range(NB - 1)] + [(S - TQ + g * 128, 128) for g in range(NG)]
F_TILES = [(f0, min(128, F - f0)) for f0 in range(0, F, 128)]


def _rb(a):
    return a.astype(BF).astype(F32)


def _kernel(x_hbm, k_hbm, v_hbm, wq_hbm, wo_hbm, wr_hbm, wg_hbm, wu_hbm, wd_hbm,
            o_hbm,
            s0_ref, s1_ref, vt_ref, ot0_ref, ot1_ref, acc_ref, qn_ref,
            k_ref, v_ref, wq_ref, wo_ref, xn_ref, g_ref, out_ref, wg_ref, wu_ref, wd_ref,
            x_ref, l0_ref, l1_ref, xs_ref, rs_ref, wrf_ref, wr_ref, z_ref, idx_ref, sem):
    s_refs = (s0_ref, s1_ref)
    ot_refs = (ot0_ref, ot1_ref)
    l_refs = (l0_ref, l1_ref)

    def cp_k(h, s=SEM_H):
        return pltpu.make_async_copy(k_hbm.at[h], k_ref.at[h], sem.at[s])

    def cp_v(h, s=SEM_H):
        return pltpu.make_async_copy(v_hbm.at[h], v_ref.at[h], sem.at[s])

    def cp_wq(h, s=SEM_H):
        off = h * DH if isinstance(h, int) else pl.multiple_of(h * DH, DH)
        return pltpu.make_async_copy(wq_hbm.at[:, pl.ds(off, DH)], wq_ref.at[h], sem.at[s])

    def cp_wo(h, s=SEM_H):
        return pltpu.make_async_copy(wo_hbm.at[h], wo_ref.at[h], sem.at[s])

    def cp_x(i, s):
        return pltpu.make_async_copy(x_hbm.at[pl.ds(i * TQ, TQ)], x_ref.at[pl.ds(i * TQ, TQ)], sem.at[s])

    def cp_ffn():
        return [pltpu.make_async_copy(src, dst, sem.at[SEM_F])
                for src, dst in ((wg_hbm, wg_ref), (wu_hbm, wu_ref), (wd_hbm, wd_ref))]

    def cp_wr():
        return pltpu.make_async_copy(wr_hbm, wr_ref, sem.at[SEM_D])

    def cp_out(j):
        r0, n = OUT_PIECES[j]
        return pltpu.make_async_copy(out_ref.at[pl.ds(r0, n)], o_hbm.at[pl.ds(r0, n)], sem.at[SEM_O])

    def start_head(h):
        cp_k(h).start()
        cp_v(h).start()
        cp_wo(h).start()
        if isinstance(h, int):
            cp_wq(h + 1).start()
        else:
            @pl.when(h + 1 < H)
            def _():
                cp_wq(h + 1).start()

    def wait_head(h):
        cp_k(h).wait()
        cp_v(h).wait()
        cp_wo(h).wait()
        if not isinstance(h, int):
            cp_wq(h + 1).wait()

    class Ctx:
        def __init__(self):
            self.z1 = pl.multiple_of(z_ref[0], 8)
            self.z2 = pl.multiple_of(z_ref[1], 8)
            self.zvec = jnp.full((8, 128), z_ref[0], jnp.int32).astype(U32)
            self.hist = []

        def tok(self, a):
            return pltpu.bitcast(a, U32) & self.zvec

        def memtok(self, ref):
            rows = 16 if ref.dtype == BF else 8
            return self.tok(ref[pl.ds(pl.multiple_of(self.z2 * 2, 16), rows), 0:128])

        def hold(self, ref, a):
            if a is not None:
                ref[S:S + 16, 0:128] = pltpu.bitcast(self.tok(a), BF)

        def view16(self, ref, z):
            return ref.at[pl.ds(pl.multiple_of(z * 2, 16), S), :]

    def dep(a, t):
        return pltpu.bitcast(pltpu.bitcast(a, U32) | t, F32)

    lane = lax.broadcasted_iota(jnp.int32, (8, 128), 1)
    sub = lax.broadcasted_iota(jnp.int32, (8, 128), 0)

    class LayerNorm:
        def __init__(self, cx, r0, c, lag2, lag3):
            self.cx, self.r0, self.c, self.n = cx, r0, c, TQ // c
            self.lag2, self.lag3 = lag2, lag3
            self.k = 0
            self.mean, self.inv = {}, {}
            self.steps = self.n + lag3

        def step(self, after=None):
            cx, c, k = self.cx, self.c, self.k
            self.k += 1
            xv, xw, xu = cx.view16(x_ref, cx.z2), cx.view16(x_ref, cx.z1), cx.view16(x_ref, cx.z1 + cx.z2)
            cx.hold(x_ref, after)
            if k < self.n:
                a = self.r0 + k * c
                self.mean[k] = jnp.mean(xv[a:a + c, :].astype(F32), axis=-1, keepdims=True)
            j = k - self.lag2
            if 0 <= j < self.n:
                a = self.r0 + j * c
                xc = xw[a:a + c, :].astype(F32) - self.mean[j]
                v = _rb(_rb(jnp.mean(xc * xc, axis=-1, keepdims=True)) + 1e-5)
                den = _rb(v * lax.rsqrt(v))
                inv = pl.reciprocal(den, approx=True)
                self.inv[j] = inv * (2.0 - den * inv)
            j = k - self.lag3
            if 0 <= j < self.n:
                a = self.r0 + j * c
                d = _rb(xu[a:a + c, :].astype(F32) - _rb(self.mean[j]))
                xn_ref[a:a + c, :] = (d * self.inv[j]).astype(BF)

    class Router:
        def __init__(self, cx, steps):
            self.cx, self.steps, self.k = cx, steps, 0
            self.rc = [jnp.zeros((8, 128), F32), jnp.zeros((8, 128), F32)]

        def step(self, after=None):
            cx, n = self.cx, S // self.steps
            xv = cx.view16(xn_ref, cx.z2)
            cx.hold(xn_ref, after)
            for a in range(self.k * n, (self.k + 1) * n, 16):
                xf = xv[a:a + 16, :].astype(F32)
                w = jnp.concatenate([wrf_ref[...]] * 2, axis=0)
                r = _rb(jnp.sum(xf * w, axis=-1, keepdims=True))
                for j in range(2):
                    gi = a // 8 + j
                    self.rc[gi // 128] = jnp.where(lane == gi % 128, r[j * 8:(j + 1) * 8, :], self.rc[gi // 128])
            self.k += 1

        def top_k(self):
            r = jnp.concatenate(self.rc, axis=0)
            tix = jnp.concatenate([(8 * (128 * a + lane) + sub) for a in range(2)], axis=0).astype(F32)
            rw = jnp.where(r != r, -jnp.inf, r)
            alive = jnp.ones((16, 128), F32)
            for j in range(C):
                mx = jnp.max(jnp.max(rw, axis=0, keepdims=True), axis=1, keepdims=True)
                cand = jnp.where((rw == mx) & (alive > 0), tix, float(S - 1))
                ixv = jnp.min(jnp.min(cand, axis=0, keepdims=True), axis=1, keepdims=True)
                hit = tix == ixv
                rsel = jnp.sum(jnp.sum(jnp.where(hit, r, 0.0), axis=0, keepdims=True), axis=1, keepdims=True)
                rw = jnp.where(hit, -jnp.inf, rw)
                alive = jnp.where(hit, 0.0, alive)
                ix = ixv.astype(jnp.int32)[0, 0]
                idx_ref[j] = ix
                blk = xn_ref[pl.ds(pl.multiple_of((ix // 16) * 16, 16), 16), :].astype(F32)
                pick = lax.broadcasted_iota(jnp.int32, (16, D), 0) == (ixv.astype(jnp.int32) & 15)
                xs_ref[j:j + 1, :] = jnp.sum(jnp.where(pick, blk, 0.0), axis=0, keepdims=True)
                rs_ref[j:j + 1, :] = jnp.broadcast_to(rsel, (1, 128))

    def gate(r0, n):
        hb = 0.5 * xn_ref[pl.ds(r0, n), :].astype(F32)
        g_ref[pl.ds(r0, n), :] = hb + hb * jnp.tanh(hb)

    class Ffn:
        def __init__(self):
            self.xs = xs_ref[...].astype(BF)
            self.acc = {}
            self.up = [(w, i, k) for i in range(len(F_TILES)) for w in (0, 1) for k in range(D // 128)]
            self.down = [(i, k) for k in range(D // 128) for i in range(len(F_TILES))]
            self.hid = None

        def add(self, key, d):
            self.acc[key] = d if key not in self.acc else self.acc[key] + d

        def run_up(self, n):
            for _ in range(min(n, len(self.up))):
                w, i, k = self.up.pop(0)
                f0, fn = F_TILES[i]
                wt = (wg_ref, wu_ref)[w][f0:f0 + fn, k * 128:(k + 1) * 128]
                self.add((w, i), lax.dot_general(self.xs[:, k * 128:(k + 1) * 128], wt, NT,
                                                 preferred_element_type=F32))

        def run_down(self, n):
            if self.hid is None:
                self.run_up(len(self.up))
                self.hid = []
                for i in range(len(F_TILES)):
                    g = _rb(self.acc[(0, i)])
                    g = _rb(g * jax.nn.sigmoid(g))
                    self.hid.append((g * _rb(self.acc[(1, i)])).astype(BF))
            for _ in range(min(n, len(self.down))):
                i, k = self.down.pop(0)
                f0, fn = F_TILES[i]
                self.add((2, k), jnp.dot(self.hid[i], wd_ref[f0:f0 + fn, k * 128:(k + 1) * 128],
                                         preferred_element_type=F32))

        def finish(self):
            self.run_down(len(self.down))
            y = _rb(jnp.concatenate([self.acc[(2, k)] for k in range(D // 128)], axis=1))
            y = _rb(y * _rb(jax.nn.sigmoid(rs_ref[:, 0:1])))
            b = _rb(xs_ref[...] + y)
            gs = b * jax.nn.sigmoid(b)
            for j in range(C):
                g_ref[pl.ds(idx_ref[j], 1), :] = gs[j:j + 1, :]

    def qproj(i, h, split=1):
        n = TQ // split
        parts = [(jnp.dot(xn_ref[r0:r0 + n, :], wq_ref[h], preferred_element_type=F32) * QSCALE).astype(BF)
                 for r0 in range(i * TQ, (i + 1) * TQ, n)]
        return parts[0] if split == 1 else jnp.concatenate(parts, axis=0)

    def transpose_v(cx, h):
        vt_ref[pl.ds(cx.z1, DH // 2), :] = pltpu.bitcast(v_ref[h].T, U32)

    def qk(cx, n, h, q, transposed=False, between=None, ticks=None):
        sv = s_refs[n % 2].at[pl.ds(cx.z1, NG * SP), :]
        ns = 1 if between is None else FSL
        sl = S // ns
        m = None
        for j in range(ns):
            kj = k_ref[h, j * sl:(j + 1) * sl, :]
            if transposed:
                sT = jnp.dot(kj, q, preferred_element_type=F32)
            else:
                sT = lax.dot_general(kj, q, NT, preferred_element_type=F32)
            for g in range(NG):
                sv[g * SP + j * sl:g * SP + (j + 1) * sl, :] = sT[:, g * 128:(g + 1) * 128]
            mj = jnp.max(jnp.max(sT.reshape(sl // 128, 16, 8, TQ), axis=1), axis=0)
            m = mj if m is None else jnp.maximum(m, mj)
            if between is not None and j < ns - 1:
                between(j)
        if ticks is not None:
            fn, count, span = ticks
            for i in range(count):
                r = (i * span // count) // 8 * 8
                fn(sT[r:r + 8, 0:128])
        return jnp.broadcast_to(jnp.max(m, axis=0, keepdims=True), (8, TQ))

    def pv(cx, n, m, hooks=None, groups=tuple(range(NG)), buf=0):
        sv = s_refs[n % 2].at[pl.ds(cx.z2, NG * SP), :]
        vv = vt_ref.at[pl.ds(cx.z2, DH // 2), :]
        otv = ot_refs[buf].at[pl.ds(cx.z1, NG * DH), :]
        lv = l_refs[buf].at[pl.ds(cx.z1, NG * 8), :]
        for g in groups:
            l8 = None
            oT = None
            for c in range(NCH):
                mc = m[:, g * 128:(g + 1) * 128]
                if len(cx.hist) >= PV_DIST:
                    mc = dep(mc, cx.tok(cx.hist[-PV_DIST]))
                if hooks and g * NCH + c in hooks:
                    mc = dep(mc, hooks[g * NCH + c])
                ps = []
                for t in range(c * CT, (c + 1) * CT):
                    r0 = g * SP + t * 128
                    p = jnp.exp2(sv[r0:r0 + 128, :] - jnp.concatenate([mc] * 16, axis=0))
                    lt = None
                    for j in reversed(range(16)):
                        pj = p[j * 8:(j + 1) * 8, :]
                        lt = pj if lt is None else lt + pj
                    l8 = lt if l8 is None else l8 + lt
                    ps.append(p)
                vT = pltpu.bitcast(vv[:, c * CT * 128:(c + 1) * CT * 128], BF)
                part = jnp.dot(vT, jnp.concatenate(ps, axis=0).astype(BF), preferred_element_type=F32)
                cx.hist.append(part[0:8, :])
                oT = part if oT is None else oT + part
            otv[g * DH:(g + 1) * DH, :] = oT
            lv[g * 8:(g + 1) * 8, :] = l8

    def load_o(cx, groups=tuple(range(NG)), buf=0):
        otv = ot_refs[buf].at[pl.ds(cx.z2, NG * DH), :]
        lv = l_refs[buf].at[pl.ds(cx.z2, NG * 8), :]
        parts = []
        for g in groups:
            l = jnp.sum(lv[g * 8:(g + 1) * 8, :], axis=0, keepdims=True)
            parts.append((otv[g * DH:(g + 1) * DH, :] * (1.0 / l)).T.astype(BF))
        return parts[0] if len(parts) == 1 else jnp.concatenate(parts, axis=0)

    def oproj(cx, r0, h, o, mode, paces_pv=True):
        r1 = r0 + o.shape[0]
        d = jnp.dot(o, wo_ref[h], preferred_element_type=F32)
        if mode == 'set':
            acc_ref[r0:r1, :] = d
        elif mode == 'add':
            acc_ref[r0:r1, :] += d
        else:
            s = acc_ref[r0:r1, :] + d
            out_ref[r0:r1, :] = (x_ref[r0:r1, :].astype(F32) + s * g_ref[r0:r1, :]).astype(BF)
        if paces_pv:
            for r in (128, 256, 384):
                cx.hist.append(d[r:r + 8, 0:128])

    def store_qt(cx, q):
        qn_ref[...] = pltpu.bitcast(q.T, U32)
        return cx.memtok(qn_ref)

    cp_x(0, SEM_A).start()
    cp_wq(0, SEM_A).start()
    cp_k(0, SEM_B).start()
    cp_x(1, SEM_B).start()
    cp_v(0, SEM_C).start()
    cp_x(2, SEM_D).start()
    cp_x(3, SEM_D).start()
    cp_wo(0, SEM_D).start()
    cp_wq(1, SEM_D).start()
    cp_wr().start()
    z_ref[0] = 0
    z_ref[1] = 0
    acc_ref[S - TQ:, :] = jnp.zeros((TQ, D), F32)

    def hide(i, c):
        z_ref[1] = z_ref[0] * i
        z_ref[0] = z_ref[1] * i
        return c

    lax.fori_loop(0, 2, hide, 0)
    cx = Ctx()
    cp_x(0, SEM_A).wait()
    cp_wq(0, SEM_A).wait()
    ln = LayerNorm(cx, 0, 32, 0, 0)
    for _ in range(ln.steps):
        ln.step()
    q = qproj(0, 0, split=4)
    cp_k(0, SEM_B).wait()
    cp_x(1, SEM_B).wait()
    start_head(1)

    ln = LayerNorm(cx, TQ, 8, 4, 10)
    ln.step()
    m = qk(cx, 0, 0, q, ticks=(ln.step, ln.steps - 1, 2000))
    cp_v(0, SEM_C).wait()
    transpose_v(cx, 0)
    q = qproj(1, 0)
    pv(cx, 0, m)
    cp_x(2, SEM_D).wait()
    cp_x(3, SEM_D).wait()
    cp_wo(0, SEM_D).wait()
    cp_wq(1, SEM_D).wait()
    cp_wr().wait()
    wrf_ref[...] = jnp.broadcast_to(wr_ref[...].astype(F32).reshape(1, D), (8, D))
    for c in cp_ffn():
        c.start()
    for n in range(1, NB - 1):
        ln = LayerNorm(cx, (n + 1) * TQ, 8, 4, 12)
        m = qk(cx, n, 0, q, ticks=(ln.step, ln.steps, 2040))
        q = qproj(n + 1, 0)
        oproj(cx, (n - 1) * TQ, 0, load_o(cx), 'set')
        pv(cx, n, m)
    router = Router(cx, 64)
    m = qk(cx, NB - 1, 0, q, ticks=(router.step, router.steps, 1900))
    router.top_k()
    gate((H - 2) * GROWS, S - (H - 2) * GROWS)
    q = qproj(0, 1)
    oproj(cx, (NB - 2) * TQ, 0, load_o(cx), 'set')
    qt_done = store_qt(cx, q)
    pv(cx, NB - 1, m, {10: qt_done | cx.zvec, 14: cx.memtok(xs_ref) | cx.memtok(rs_ref)})

    def body(it, carry):
        h = 1 + it
        wait_head(h)
        start_head(h + 1)
        cx = Ctx()
        transpose_v(cx, h)
        gate(pl.multiple_of(it * GROWS, GROWS), GROWS)
        q = pltpu.bitcast(qn_ref[...], BF)
        for n in range(NB):
            m = qk(cx, n, h, q, transposed=n == 0)
            q = qproj((n + 1) % NB, h + (n + 1) // NB)
            oproj(cx, (n - 1) % NB * TQ, h - (n == 0), load_o(cx), 'add')
            pv(cx, n, m, {4: store_qt(cx, q)} if n == NB - 1 else None)
        return carry

    lax.fori_loop(0, H - 2, body, 0)

    h = H - 1
    wait_head(h)
    for c in cp_ffn():
        c.wait()
    cx = Ctx()
    transpose_v(cx, h)
    ffn = Ffn()

    def spread(run, total):
        return lambda j: run((total * (j + 1)) // (FSL - 1) - (total * j) // (FSL - 1))

    def next_qt(i):
        done = store_qt(cx, qproj(i, h))
        return pltpu.bitcast(qn_ref[pl.ds(cx.z1, DH // 2), :], BF), {8: done}

    q = pltpu.bitcast(qn_ref[...], BF)
    m = qk(cx, 0, h, q, transposed=True, between=spread(ffn.run_up, 60))
    ffn.run_up(4)
    q, hooks = next_qt(1)
    ffn.run_up(4)
    oproj(cx, S - TQ, h - 1, load_o(cx), 'add')
    pv(cx, 0, m, hooks)
    ffn.run_up(4)
    m = qk(cx, 1, h, q, transposed=True, between=spread(ffn.run_up, len(ffn.up) - 4))
    ffn.run_up(4)
    q, hooks = next_qt(2)
    pv(cx, 1, m, hooks, buf=1)
    ffn.run_down(4)
    m = qk(cx, 2, h, q, transposed=True, between=spread(ffn.run_down, len(ffn.down) - 6))
    ffn.finish()
    q = qproj(3, h)
    oproj(cx, 0, h, load_o(cx), 'out', paces_pv=False)
    cp_out(0).start()
    oproj(cx, TQ, h, load_o(cx, buf=1), 'out')
    cp_out(1).start()
    pv(cx, 2, m, {6: cx.memtok(out_ref)})
    m = qk(cx, 3, h, q)
    oproj(cx, 2 * TQ, h, load_o(cx), 'out')
    cp_out(2).start()
    stored = cx.memtok(out_ref)
    os = []

    def finish_group(g):
        oproj(cx, S - TQ + g * 128, h, os[g], 'out', paces_pv=False)
        cp_out(NB - 1 + g).start()

    for g in range(NG):
        pv(cx, NB - 1, m, {6: stored}, groups=(g,))
        os.append(load_o(cx, (g,)))
        if g == 2:
            finish_group(0)
    for g in range(1, NG):
        finish_group(g)
    for j in range(len(OUT_PIECES)):
        cp_out(j).wait()


@jax.jit
def pallas_recurrent_scan__mha_block_cached__moe_arch_mod__prompt_kernel(
    A_x: jax.Array,
    A_k_cache: jax.Array,
    A_v_cache: jax.Array,
    A_wq: jax.Array,
    A_wo: jax.Array,
    B_x: jax.Array,
    B_w_r: jax.Array,
    B_w_gate: jax.Array,
    B_w_up: jax.Array,
    B_w_down: jax.Array,
):
    hbm = pl.BlockSpec(memory_space=pl.ANY)
    out = pl.pallas_call(
        _kernel,
        in_specs=[hbm] * 9,
        out_specs=hbm,
        out_shape=jax.ShapeDtypeStruct((S, D), BF),
        scratch_shapes=[
            pltpu.VMEM((NG * SP, 128), F32),
            pltpu.VMEM((NG * SP, 128), F32),
            pltpu.VMEM((DH // 2, S), U32),
            pltpu.VMEM((NG * DH + 32, 128), F32),
            pltpu.VMEM((NG * DH, 128), F32),
            pltpu.VMEM((S, D), F32),
            pltpu.VMEM((DH // 2, TQ), U32),
            pltpu.VMEM((H, S, DH), BF),
            pltpu.VMEM((H, S, DH), BF),
            pltpu.VMEM((H, D, DH), BF),
            pltpu.VMEM((H, DH, D), BF),
            pltpu.VMEM((S + 64, D), BF),
            pltpu.VMEM((S, D), F32),
            pltpu.VMEM((S, D), BF),
            pltpu.VMEM((F, D), BF),
            pltpu.VMEM((F, D), BF),
            pltpu.VMEM((F, D), BF),
            pltpu.VMEM((S + 64, D), BF),
            pltpu.VMEM((NG * 8, 128), F32),
            pltpu.VMEM((NG * 8, 128), F32),
            pltpu.VMEM((C, D), F32),
            pltpu.VMEM((C, 128), F32),
            pltpu.VMEM((8, D), F32),
            pltpu.VMEM((D,), BF),
            pltpu.SMEM((2,), jnp.int32),
            pltpu.SMEM((C,), jnp.int32),
            pltpu.SemaphoreType.DMA((7,)),
        ],
        compiler_params=pltpu.CompilerParams(
            vmem_limit_bytes=126 * 1024 * 1024,
            internal_scratch_in_bytes=16 * 4096,
            disable_bounds_checks=True,
            disable_semaphore_checks=True,
        ),
    )(A_x.reshape(S, D), A_k_cache.reshape(H, S, DH), A_v_cache.reshape(H, S, DH), A_wq,
      A_wo.reshape(H, DH, D), B_w_r, B_w_gate.T, B_w_up.T, B_w_down)
    return out.reshape(1, S, D)
```

```python
import math

import jax
import jax.numpy as jnp
from jax import lax
import jax.experimental.pallas as pl
import jax.experimental.pallas.tpu as pltpu

S, D, H, DH, F, C = 2048, 640, 32, 128, 1728, 8
TQ = 512
NB = S // TQ
NG = TQ // 128
CT = 4
NCH = S // 128 // CT
SP = S + 8
GROWS = 64
BF, F32, U32 = jnp.bfloat16, jnp.float32, jnp.uint32
QSCALE = (DH ** -0.5) * math.log2(math.e)
NT = (((1,), (1,)), ((), ()))
PV_DIST = 3
FSL = 16
SEM_A, SEM_B, SEM_C, SEM_D, SEM_H, SEM_F, SEM_O = range(7)
OUT_PIECES = [(i * TQ, TQ) for i in range(NB - 1)] + [(S - TQ + g * 128, 128) for g in range(NG)]
F_TILES = [(f0, min(128, F - f0)) for f0 in range(0, F, 128)]


def _rb(a):
    return a.astype(BF).astype(F32)


def _kernel(x_hbm, k_hbm, v_hbm, wq_hbm, wo_hbm, wr_hbm, wg_hbm, wu_hbm, wd_hbm,
            o_hbm,
            s0_ref, s1_ref, vt_ref, ot0_ref, ot1_ref, acc_ref, qn_ref,
            k_ref, v_ref, wq_ref, wo_ref, xn_ref, g_ref, out_ref, wg_ref, wu_ref, wd_ref,
            x_ref, l0_ref, l1_ref, xs_ref, rs_ref, wrf_ref, wr_ref, z_ref, idx_ref, sem):
    s_refs = (s0_ref, s1_ref)
    ot_refs = (ot0_ref, ot1_ref)
    l_refs = (l0_ref, l1_ref)

    def cp_k(h, s=SEM_H):
        return pltpu.make_async_copy(k_hbm.at[h], k_ref.at[h], sem.at[s])

    def cp_v(h, s=SEM_H):
        return pltpu.make_async_copy(v_hbm.at[h], v_ref.at[h], sem.at[s])

    def cp_wq(h, s=SEM_H):
        off = h * DH if isinstance(h, int) else pl.multiple_of(h * DH, DH)
        return pltpu.make_async_copy(wq_hbm.at[:, pl.ds(off, DH)], wq_ref.at[h], sem.at[s])

    def cp_wo(h, s=SEM_H):
        return pltpu.make_async_copy(wo_hbm.at[h], wo_ref.at[h], sem.at[s])

    def cp_x(i, s):
        return pltpu.make_async_copy(x_hbm.at[pl.ds(i * TQ, TQ)], x_ref.at[pl.ds(i * TQ, TQ)], sem.at[s])

    def cp_ffn():
        return [pltpu.make_async_copy(src, dst, sem.at[SEM_F])
                for src, dst in ((wg_hbm, wg_ref), (wu_hbm, wu_ref), (wd_hbm, wd_ref))]

    def cp_wr():
        return pltpu.make_async_copy(wr_hbm, wr_ref, sem.at[SEM_D])

    def cp_out(j):
        r0, n = OUT_PIECES[j]
        return pltpu.make_async_copy(out_ref.at[pl.ds(r0, n)], o_hbm.at[pl.ds(r0, n)], sem.at[SEM_O])

    def start_head(h):
        cp_k(h).start()
        cp_v(h).start()
        cp_wo(h).start()
        if isinstance(h, int):
            cp_wq(h + 1).start()
        else:
            @pl.when(h + 1 < H)
            def _():
                cp_wq(h + 1).start()

    def wait_head(h):
        cp_k(h).wait()
        cp_v(h).wait()
        cp_wo(h).wait()
        if not isinstance(h, int):
            cp_wq(h + 1).wait()

    class Ctx:
        def __init__(self):
            self.z1 = pl.multiple_of(z_ref[0], 8)
            self.z2 = pl.multiple_of(z_ref[1], 8)
            self.zvec = jnp.full((8, 128), z_ref[0], jnp.int32).astype(U32)
            self.hist = []

        def tok(self, a):
            return pltpu.bitcast(a, U32) & self.zvec

        def memtok(self, ref):
            rows = 16 if ref.dtype == BF else 8
            return self.tok(ref[pl.ds(pl.multiple_of(self.z2 * 2, 16), rows), 0:128])

        def hold(self, ref, a):
            if a is not None:
                ref[S:S + 16, 0:128] = pltpu.bitcast(self.tok(a), BF)

        def view16(self, ref, z):
            return ref.at[pl.ds(pl.multiple_of(z * 2, 16), S), :]

    def dep(a, t):
        return pltpu.bitcast(pltpu.bitcast(a, U32) | t, F32)

    lane = lax.broadcasted_iota(jnp.int32, (8, 128), 1)
    sub = lax.broadcasted_iota(jnp.int32, (8, 128), 0)

    class LayerNorm:
        def __init__(self, cx, r0, c, lag2, lag3):
            self.cx, self.r0, self.c, self.n = cx, r0, c, TQ // c
            self.lag2, self.lag3 = lag2, lag3
            self.k = 0
            self.mean, self.inv = {}, {}
            self.steps = self.n + lag3

        def step(self, after=None):
            cx, c, k = self.cx, self.c, self.k
            self.k += 1
            xv, xw, xu = cx.view16(x_ref, cx.z2), cx.view16(x_ref, cx.z1), cx.view16(x_ref, cx.z1 + cx.z2)
            cx.hold(x_ref, after)
            if k < self.n:
                a = self.r0 + k * c
                self.mean[k] = jnp.mean(xv[a:a + c, :].astype(F32), axis=-1, keepdims=True)
            j = k - self.lag2
            if 0 <= j < self.n:
                a = self.r0 + j * c
                xc = xw[a:a + c, :].astype(F32) - self.mean[j]
                v = _rb(_rb(jnp.mean(xc * xc, axis=-1, keepdims=True)) + 1e-5)
                den = _rb(v * lax.rsqrt(v))
                inv = pl.reciprocal(den, approx=True)
                self.inv[j] = inv * (2.0 - den * inv)
            j = k - self.lag3
            if 0 <= j < self.n:
                a = self.r0 + j * c
                d = _rb(xu[a:a + c, :].astype(F32) - _rb(self.mean[j]))
                xn_ref[a:a + c, :] = (d * self.inv[j]).astype(BF)

    class Router:
        def __init__(self, cx, steps):
            self.cx, self.steps, self.k = cx, steps, 0
            self.rc = [jnp.zeros((8, 128), F32), jnp.zeros((8, 128), F32)]

        def step(self, after=None):
            cx, n = self.cx, S // self.steps
            xv = cx.view16(xn_ref, cx.z2)
            cx.hold(xn_ref, after)
            for a in range(self.k * n, (self.k + 1) * n, 16):
                xf = xv[a:a + 16, :].astype(F32)
                w = jnp.concatenate([wrf_ref[...]] * 2, axis=0)
                r = _rb(jnp.sum(xf * w, axis=-1, keepdims=True))
                for j in range(2):
                    gi = a // 8 + j
                    self.rc[gi // 128] = jnp.where(lane == gi % 128, r[j * 8:(j + 1) * 8, :], self.rc[gi // 128])
            self.k += 1

        def top_k(self):
            r = jnp.concatenate(self.rc, axis=0)
            tix = jnp.concatenate([(8 * (128 * a + lane) + sub) for a in range(2)], axis=0).astype(F32)
            rw = jnp.where(r != r, -jnp.inf, r)
            alive = jnp.ones((16, 128), F32)
            for j in range(C):
                mx = jnp.max(jnp.max(rw, axis=0, keepdims=True), axis=1, keepdims=True)
                cand = jnp.where((rw == mx) & (alive > 0), tix, float(S - 1))
                ixv = jnp.min(jnp.min(cand, axis=0, keepdims=True), axis=1, keepdims=True)
                hit = tix == ixv
                rsel = jnp.sum(jnp.sum(jnp.where(hit, r, 0.0), axis=0, keepdims=True), axis=1, keepdims=True)
                rw = jnp.where(hit, -jnp.inf, rw)
                alive = jnp.where(hit, 0.0, alive)
                ix = ixv.astype(jnp.int32)[0, 0]
                idx_ref[j] = ix
                blk = xn_ref[pl.ds(pl.multiple_of((ix // 16) * 16, 16), 16), :].astype(F32)
                pick = lax.broadcasted_iota(jnp.int32, (16, D), 0) == (ixv.astype(jnp.int32) & 15)
                xs_ref[j:j + 1, :] = jnp.sum(jnp.where(pick, blk, 0.0), axis=0, keepdims=True)
                rs_ref[j:j + 1, :] = jnp.broadcast_to(rsel, (1, 128))

    def gate(r0, n):
        hb = 0.5 * xn_ref[pl.ds(r0, n), :].astype(F32)
        g_ref[pl.ds(r0, n), :] = hb + hb * jnp.tanh(hb)

    class Ffn:
        def __init__(self):
            self.xs = xs_ref[...].astype(BF)
            self.acc = {}
            self.up = [(w, i, k) for i in range(len(F_TILES)) for w in (0, 1) for k in range(D // 128)]
            self.down = [(i, k) for k in range(D // 128) for i in range(len(F_TILES))]
            self.hid = None

        def add(self, key, d):
            self.acc[key] = d if key not in self.acc else self.acc[key] + d

        def run_up(self, n):
            for _ in range(min(n, len(self.up))):
                w, i, k = self.up.pop(0)
                f0, fn = F_TILES[i]
                wt = (wg_ref, wu_ref)[w][f0:f0 + fn, k * 128:(k + 1) * 128]
                self.add((w, i), lax.dot_general(self.xs[:, k * 128:(k + 1) * 128], wt, NT,
                                                 preferred_element_type=F32))

        def run_down(self, n):
            if self.hid is None:
                self.run_up(len(self.up))
                self.hid = []
                for i in range(len(F_TILES)):
                    g = _rb(self.acc[(0, i)])
                    g = _rb(g * jax.nn.sigmoid(g))
                    self.hid.append((g * _rb(self.acc[(1, i)])).astype(BF))
            for _ in range(min(n, len(self.down))):
                i, k = self.down.pop(0)
                f0, fn = F_TILES[i]
                self.add((2, k), jnp.dot(self.hid[i], wd_ref[f0:f0 + fn, k * 128:(k + 1) * 128],
                                         preferred_element_type=F32))

        def finish(self):
            self.run_down(len(self.down))
            y = _rb(jnp.concatenate([self.acc[(2, k)] for k in range(D // 128)], axis=1))
            y = _rb(y * _rb(jax.nn.sigmoid(rs_ref[:, 0:1])))
            b = _rb(xs_ref[...] + y)
            gs = b * jax.nn.sigmoid(b)
            for j in range(C):
                g_ref[pl.ds(idx_ref[j], 1), :] = gs[j:j + 1, :]

    def qproj(i, h, split=1):
        n = TQ // split
        parts = [(jnp.dot(xn_ref[r0:r0 + n, :], wq_ref[h], preferred_element_type=F32) * QSCALE).astype(BF)
                 for r0 in range(i * TQ, (i + 1) * TQ, n)]
        return parts[0] if split == 1 else jnp.concatenate(parts, axis=0)

    def transpose_v(cx, h):
        vt_ref[pl.ds(cx.z1, DH // 2), :] = pltpu.bitcast(v_ref[h].T, U32)

    def qk(cx, n, h, q, transposed=False, between=None, ticks=None):
        sv = s_refs[n % 2].at[pl.ds(cx.z1, NG * SP), :]
        ns = 1 if between is None else FSL
        sl = S // ns
        m = None
        for j in range(ns):
            kj = k_ref[h, j * sl:(j + 1) * sl, :]
            if transposed:
                sT = jnp.dot(kj, q, preferred_element_type=F32)
            else:
                sT = lax.dot_general(kj, q, NT, preferred_element_type=F32)
            for g in range(NG):
                sv[g * SP + j * sl:g * SP + (j + 1) * sl, :] = sT[:, g * 128:(g + 1) * 128]
            mj = jnp.max(jnp.max(sT.reshape(sl // 128, 16, 8, TQ), axis=1), axis=0)
            m = mj if m is None else jnp.maximum(m, mj)
            if between is not None and j < ns - 1:
                between(j)
        if ticks is not None:
            fn, count, span = ticks
            for i in range(count):
                r = (i * span // count) // 8 * 8
                fn(sT[r:r + 8, 0:128])
        return jnp.broadcast_to(jnp.max(m, axis=0, keepdims=True), (8, TQ))

    def pv(cx, n, m, hooks=None, groups=tuple(range(NG)), buf=0):
        sv = s_refs[n % 2].at[pl.ds(cx.z2, NG * SP), :]
        vv = vt_ref.at[pl.ds(cx.z2, DH // 2), :]
        otv = ot_refs[buf].at[pl.ds(cx.z1, NG * DH), :]
        lv = l_refs[buf].at[pl.ds(cx.z1, NG * 8), :]
        for g in groups:
            l8 = None
            oT = None
            for c in range(NCH):
                mc = m[:, g * 128:(g + 1) * 128]
                if len(cx.hist) >= PV_DIST:
                    mc = dep(mc, cx.tok(cx.hist[-PV_DIST]))
                if hooks and g * NCH + c in hooks:
                    mc = dep(mc, hooks[g * NCH + c])
                ps = []
                for t in range(c * CT, (c + 1) * CT):
                    r0 = g * SP + t * 128
                    p = jnp.exp2(sv[r0:r0 + 128, :] - jnp.concatenate([mc] * 16, axis=0))
                    lt = None
                    for j in reversed(range(16)):
                        pj = p[j * 8:(j + 1) * 8, :]
                        lt = pj if lt is None else lt + pj
                    l8 = lt if l8 is None else l8 + lt
                    ps.append(p)
                vT = pltpu.bitcast(vv[:, c * CT * 128:(c + 1) * CT * 128], BF)
                part = jnp.dot(vT, jnp.concatenate(ps, axis=0).astype(BF), preferred_element_type=F32)
                cx.hist.append(part[0:8, :])
                oT = part if oT is None else oT + part
            otv[g * DH:(g + 1) * DH, :] = oT
            lv[g * 8:(g + 1) * 8, :] = l8

    def load_o(cx, groups=tuple(range(NG)), buf=0):
        otv = ot_refs[buf].at[pl.ds(cx.z2, NG * DH), :]
        lv = l_refs[buf].at[pl.ds(cx.z2, NG * 8), :]
        parts = []
        for g in groups:
            l = jnp.sum(lv[g * 8:(g + 1) * 8, :], axis=0, keepdims=True)
            parts.append((otv[g * DH:(g + 1) * DH, :] * (1.0 / l)).T.astype(BF))
        return parts[0] if len(parts) == 1 else jnp.concatenate(parts, axis=0)

    def oproj(cx, r0, h, o, mode, paces_pv=True):
        r1 = r0 + o.shape[0]
        d = jnp.dot(o, wo_ref[h], preferred_element_type=F32)
        if mode == 'set':
            acc_ref[r0:r1, :] = d
        elif mode == 'add':
            acc_ref[r0:r1, :] += d
        else:
            s = acc_ref[r0:r1, :] + d
            out_ref[r0:r1, :] = (x_ref[r0:r1, :].astype(F32) + s * g_ref[r0:r1, :]).astype(BF)
        if paces_pv:
            for r in (128, 256, 384):
                cx.hist.append(d[r:r + 8, 0:128])

    def store_qt(cx, q):
        qn_ref[...] = pltpu.bitcast(q.T, U32)
        return cx.memtok(qn_ref)

    cp_x(0, SEM_A).start()
    cp_wq(0, SEM_A).start()
    cp_k(0, SEM_B).start()
    cp_x(1, SEM_B).start()
    cp_v(0, SEM_C).start()
    cp_x(2, SEM_D).start()
    cp_x(3, SEM_D).start()
    cp_wo(0, SEM_D).start()
    cp_wq(1, SEM_D).start()
    cp_wr().start()
    z_ref[0] = 0
    z_ref[1] = 0
    acc_ref[S - TQ:, :] = jnp.zeros((TQ, D), F32)

    def hide(i, c):
        z_ref[1] = z_ref[0] * i
        z_ref[0] = z_ref[1] * i
        return c

    lax.fori_loop(0, 2, hide, 0)
    cx = Ctx()
    cp_x(0, SEM_A).wait()
    cp_wq(0, SEM_A).wait()
    ln = LayerNorm(cx, 0, 32, 0, 0)
    for _ in range(ln.steps):
        ln.step()
    q = qproj(0, 0, split=4)
    cp_k(0, SEM_B).wait()
    cp_x(1, SEM_B).wait()
    start_head(1)

    ln = LayerNorm(cx, TQ, 8, 4, 10)
    ln.step()
    m = qk(cx, 0, 0, q, ticks=(ln.step, ln.steps - 1, 2000))
    cp_v(0, SEM_C).wait()
    transpose_v(cx, 0)
    q = qproj(1, 0, split=4)
    pv(cx, 0, m)
    cp_x(2, SEM_D).wait()
    cp_x(3, SEM_D).wait()
    cp_wo(0, SEM_D).wait()
    cp_wq(1, SEM_D).wait()
    cp_wr().wait()
    wrf_ref[...] = jnp.broadcast_to(wr_ref[...].astype(F32).reshape(1, D), (8, D))
    for c in cp_ffn():
        c.start()
    for n in range(1, NB - 1):
        ln = LayerNorm(cx, (n + 1) * TQ, 8, 4, 14)
        m = qk(cx, n, 0, q, ticks=(ln.step, ln.steps, 2040))
        q = qproj(n + 1, 0)
        oproj(cx, (n - 1) * TQ, 0, load_o(cx), 'set')
        pv(cx, n, m)
    router = Router(cx, 128)
    m = qk(cx, NB - 1, 0, q, ticks=(router.step, router.steps, 2040))
    router.top_k()
    gate((H - 2) * GROWS, S - (H - 2) * GROWS)
    q = qproj(0, 1)
    oproj(cx, (NB - 2) * TQ, 0, load_o(cx), 'set')
    qt_done = store_qt(cx, q)
    pv(cx, NB - 1, m, {10: qt_done | cx.zvec, 11: cx.memtok(xs_ref) | cx.memtok(rs_ref)})

    def body(it, carry):
        h = 1 + it
        wait_head(h)
        start_head(h + 1)
        cx = Ctx()
        transpose_v(cx, h)
        gate(pl.multiple_of(it * GROWS, GROWS), GROWS)
        q = pltpu.bitcast(qn_ref[...], BF)
        for n in range(NB):
            m = qk(cx, n, h, q, transposed=n == 0)
            q = qproj((n + 1) % NB, h + (n + 1) // NB)
            oproj(cx, (n - 1) % NB * TQ, h - (n == 0), load_o(cx), 'add')
            pv(cx, n, m, {4: store_qt(cx, q)} if n == NB - 1 else None)
        return carry

    lax.fori_loop(0, H - 2, body, 0)

    h = H - 1
    wait_head(h)
    for c in cp_ffn():
        c.wait()
    cx = Ctx()
    transpose_v(cx, h)
    ffn = Ffn()

    def spread(run, total):
        return lambda j: run((total * (j + 1)) // (FSL - 1) - (total * j) // (FSL - 1))

    def next_qt(i):
        done = store_qt(cx, qproj(i, h))
        return pltpu.bitcast(qn_ref[pl.ds(cx.z1, DH // 2), :], BF), {8: done}

    q = pltpu.bitcast(qn_ref[...], BF)
    m = qk(cx, 0, h, q, transposed=True, between=spread(ffn.run_up, 60))
    ffn.run_up(4)
    q, hooks = next_qt(1)
    ffn.run_up(4)
    oproj(cx, S - TQ, h - 1, load_o(cx), 'add')
    pv(cx, 0, m, hooks)
    ffn.run_up(4)
    m = qk(cx, 1, h, q, transposed=True, between=spread(ffn.run_up, len(ffn.up) - 4))
    ffn.run_up(4)
    q, hooks = next_qt(2)
    pv(cx, 1, m, hooks, buf=1)
    ffn.run_down(4)
    m = qk(cx, 2, h, q, transposed=True, between=spread(ffn.run_down, len(ffn.down) - 6))
    ffn.finish()
    q = qproj(3, h)
    oproj(cx, 0, h, load_o(cx), 'out', paces_pv=False)
    cp_out(0).start()
    oproj(cx, TQ, h, load_o(cx, buf=1), 'out')
    cp_out(1).start()
    pv(cx, 2, m, {6: cx.memtok(out_ref)})
    m = qk(cx, 3, h, q)
    oproj(cx, 2 * TQ, h, load_o(cx), 'out')
    cp_out(2).start()
    stored = cx.memtok(out_ref)
    os = []

    def finish_group(g):
        oproj(cx, S - TQ + g * 128, h, os[g], 'out', paces_pv=False)
        cp_out(NB - 1 + g).start()

    for g in range(NG):
        pv(cx, NB - 1, m, {6: stored}, groups=(g,))
        os.append(load_o(cx, (g,)))
        if g == 2:
            finish_group(0)
    for g in range(1, NG):
        finish_group(g)
    for j in range(len(OUT_PIECES)):
        cp_out(j).wait()


@jax.jit
def pallas_recurrent_scan__mha_block_cached__moe_arch_mod__prompt_kernel(
    A_x: jax.Array,
    A_k_cache: jax.Array,
    A_v_cache: jax.Array,
    A_wq: jax.Array,
    A_wo: jax.Array,
    B_x: jax.Array,
    B_w_r: jax.Array,
    B_w_gate: jax.Array,
    B_w_up: jax.Array,
    B_w_down: jax.Array,
):
    hbm = pl.BlockSpec(memory_space=pl.ANY)
    out = pl.pallas_call(
        _kernel,
        in_specs=[hbm] * 9,
        out_specs=hbm,
        out_shape=jax.ShapeDtypeStruct((S, D), BF),
        scratch_shapes=[
            pltpu.VMEM((NG * SP, 128), F32),
            pltpu.VMEM((NG * SP, 128), F32),
            pltpu.VMEM((DH // 2, S), U32),
            pltpu.VMEM((NG * DH + 32, 128), F32),
            pltpu.VMEM((NG * DH, 128), F32),
            pltpu.VMEM((S, D), F32),
            pltpu.VMEM((DH // 2, TQ), U32),
            pltpu.VMEM((H, S, DH), BF),
            pltpu.VMEM((H, S, DH), BF),
            pltpu.VMEM((H, D, DH), BF),
            pltpu.VMEM((H, DH, D), BF),
            pltpu.VMEM((S + 64, D), BF),
            pltpu.VMEM((S, D), F32),
            pltpu.VMEM((S, D), BF),
            pltpu.VMEM((F, D), BF),
            pltpu.VMEM((F, D), BF),
            pltpu.VMEM((F, D), BF),
            pltpu.VMEM((S + 64, D), BF),
            pltpu.VMEM((NG * 8, 128), F32),
            pltpu.VMEM((NG * 8, 128), F32),
            pltpu.VMEM((C, D), F32),
            pltpu.VMEM((C, 128), F32),
            pltpu.VMEM((8, D), F32),
            pltpu.VMEM((D,), BF),
            pltpu.SMEM((2,), jnp.int32),
            pltpu.SMEM((C,), jnp.int32),
            pltpu.SemaphoreType.DMA((7,)),
        ],
        compiler_params=pltpu.CompilerParams(
            vmem_limit_bytes=126 * 1024 * 1024,
            internal_scratch_in_bytes=16 * 4096,
            disable_bounds_checks=True,
            disable_semaphore_checks=True,
        ),
    )(A_x.reshape(S, D), A_k_cache.reshape(H, S, DH), A_v_cache.reshape(H, S, DH), A_wq,
      A_wo.reshape(H, DH, D), B_w_r, B_w_gate.T, B_w_up.T, B_w_down)
    return out.reshape(1, S, D)
```

```python
import math

import jax
import jax.numpy as jnp
from jax import lax
import jax.experimental.pallas as pl
import jax.experimental.pallas.tpu as pltpu

S, D, H, DH, F, C = 2048, 640, 32, 128, 1728, 8
TQ = 512
NB = S // TQ
NG = TQ // 128
CT = 4
NCH = S // 128 // CT
SP = S + 8
GROWS = 64
BF, F32, U32 = jnp.bfloat16, jnp.float32, jnp.uint32
QSCALE = (DH ** -0.5) * math.log2(math.e)
NT = (((1,), (1,)), ((), ()))
PV_DIST = 3
FSL = 16
SEM_A, SEM_B, SEM_C, SEM_D, SEM_H, SEM_F, SEM_O, SEM_E = range(8)
OUT_PIECES = [(i * TQ, TQ) for i in range(NB - 1)] + [(S - TQ + g * 128, 128) for g in range(NG)]
F_TILES = [(f0, min(128, F - f0)) for f0 in range(0, F, 128)]


def _rb(a):
    return a.astype(BF).astype(F32)


def _kernel(x_hbm, k_hbm, v_hbm, wq_hbm, wo_hbm, wr_hbm, wg_hbm, wu_hbm, wd_hbm,
            o_hbm,
            s0_ref, s1_ref, vt_ref, ot0_ref, ot1_ref, acc_ref, qn_ref,
            k_ref, v_ref, wq_ref, wo_ref, xn_ref, g_ref, out_ref, wg_ref, wu_ref, wd_ref,
            x_ref, l0_ref, l1_ref, xs_ref, rs_ref, wrf_ref, wr_ref, z_ref, idx_ref, sem):
    s_refs = (s0_ref, s1_ref)
    ot_refs = (ot0_ref, ot1_ref)
    l_refs = (l0_ref, l1_ref)

    def cp_k(h, s=SEM_H):
        return pltpu.make_async_copy(k_hbm.at[h], k_ref.at[h], sem.at[s])

    def cp_v(h, s=SEM_H):
        return pltpu.make_async_copy(v_hbm.at[h], v_ref.at[h], sem.at[s])

    def cp_wq(h, s=SEM_H):
        off = h * DH if isinstance(h, int) else pl.multiple_of(h * DH, DH)
        return pltpu.make_async_copy(wq_hbm.at[:, pl.ds(off, DH)], wq_ref.at[h], sem.at[s])

    def cp_wo(h, s=SEM_H):
        return pltpu.make_async_copy(wo_hbm.at[h], wo_ref.at[h], sem.at[s])

    def cp_x(i, s, rows=TQ):
        return pltpu.make_async_copy(x_hbm.at[pl.ds(i * rows, rows)], x_ref.at[pl.ds(i * rows, rows)], sem.at[s])

    def cp_ffn():
        return [pltpu.make_async_copy(src, dst, sem.at[SEM_F])
                for src, dst in ((wg_hbm, wg_ref), (wu_hbm, wu_ref), (wd_hbm, wd_ref))]

    def cp_wr():
        return pltpu.make_async_copy(wr_hbm, wr_ref, sem.at[SEM_D])

    def cp_out(j):
        r0, n = OUT_PIECES[j]
        return pltpu.make_async_copy(out_ref.at[pl.ds(r0, n)], o_hbm.at[pl.ds(r0, n)], sem.at[SEM_O])

    def start_head(h):
        cp_k(h).start()
        cp_v(h).start()
        cp_wo(h).start()
        if isinstance(h, int):
            cp_wq(h + 1).start()
        else:
            @pl.when(h + 1 < H)
            def _():
                cp_wq(h + 1).start()

    def wait_head(h):
        cp_k(h).wait()
        cp_v(h).wait()
        cp_wo(h).wait()
        if not isinstance(h, int):
            cp_wq(h + 1).wait()

    class Ctx:
        def __init__(self):
            self.z1 = pl.multiple_of(z_ref[0], 8)
            self.z2 = pl.multiple_of(z_ref[1], 8)
            self.zvec = jnp.full((8, 128), z_ref[0], jnp.int32).astype(U32)
            self.hist = []

        def tok(self, a):
            return pltpu.bitcast(a, U32) & self.zvec

        def memtok(self, ref):
            rows = 16 if ref.dtype == BF else 8
            return self.tok(ref[pl.ds(pl.multiple_of(self.z2 * 2, 16), rows), 0:128])

        def hold(self, ref, a):
            if a is not None:
                ref[S:S + 16, 0:128] = pltpu.bitcast(self.tok(a), BF)

        def view16(self, ref, z):
            return ref.at[pl.ds(pl.multiple_of(z * 2, 16), S), :]

    def dep(a, t):
        return pltpu.bitcast(pltpu.bitcast(a, U32) | t, F32)

    lane = lax.broadcasted_iota(jnp.int32, (8, 128), 1)
    sub = lax.broadcasted_iota(jnp.int32, (8, 128), 0)

    class LayerNorm:
        def __init__(self, cx, r0, c, lag2, lag3, rows=TQ):
            self.cx, self.r0, self.c, self.n = cx, r0, c, rows // c
            self.lag2, self.lag3 = lag2, lag3
            self.k = 0
            self.mean, self.inv = {}, {}
            self.steps = self.n + lag3

        def step(self, after=None):
            cx, c, k = self.cx, self.c, self.k
            self.k += 1
            xv, xw, xu = cx.view16(x_ref, cx.z2), cx.view16(x_ref, cx.z1), cx.view16(x_ref, cx.z1 + cx.z2)
            cx.hold(x_ref, after)
            if k < self.n:
                a = self.r0 + k * c
                self.mean[k] = jnp.mean(xv[a:a + c, :].astype(F32), axis=-1, keepdims=True)
            j = k - self.lag2
            if 0 <= j < self.n:
                a = self.r0 + j * c
                xc = xw[a:a + c, :].astype(F32) - self.mean[j]
                v = _rb(_rb(jnp.mean(xc * xc, axis=-1, keepdims=True)) + 1e-5)
                den = _rb(v * lax.rsqrt(v))
                inv = pl.reciprocal(den, approx=True)
                self.inv[j] = inv * (2.0 - den * inv)
            j = k - self.lag3
            if 0 <= j < self.n:
                a = self.r0 + j * c
                d = _rb(xu[a:a + c, :].astype(F32) - _rb(self.mean[j]))
                xn_ref[a:a + c, :] = (d * self.inv[j]).astype(BF)

    class Router:
        def __init__(self, cx, steps):
            self.cx, self.steps, self.k = cx, steps, 0
            self.rc = [jnp.zeros((8, 128), F32), jnp.zeros((8, 128), F32)]

        def step(self, after=None):
            cx, n = self.cx, S // self.steps
            xv = cx.view16(xn_ref, cx.z2)
            cx.hold(xn_ref, after)
            for a in range(self.k * n, (self.k + 1) * n, 16):
                xf = xv[a:a + 16, :].astype(F32)
                w = jnp.concatenate([wrf_ref[...]] * 2, axis=0)
                r = _rb(jnp.sum(xf * w, axis=-1, keepdims=True))
                for j in range(2):
                    gi = a // 8 + j
                    self.rc[gi // 128] = jnp.where(lane == gi % 128, r[j * 8:(j + 1) * 8, :], self.rc[gi // 128])
            self.k += 1

        def top_k(self):
            r = jnp.concatenate(self.rc, axis=0)
            tix = jnp.concatenate([(8 * (128 * a + lane) + sub) for a in range(2)], axis=0).astype(F32)
            rw = jnp.where(r != r, -jnp.inf, r)
            alive = jnp.ones((16, 128), F32)
            for j in range(C):
                mx = jnp.max(jnp.max(rw, axis=0, keepdims=True), axis=1, keepdims=True)
                cand = jnp.where((rw == mx) & (alive > 0), tix, float(S - 1))
                ixv = jnp.min(jnp.min(cand, axis=0, keepdims=True), axis=1, keepdims=True)
                hit = tix == ixv
                rsel = jnp.sum(jnp.sum(jnp.where(hit, r, 0.0), axis=0, keepdims=True), axis=1, keepdims=True)
                rw = jnp.where(hit, -jnp.inf, rw)
                alive = jnp.where(hit, 0.0, alive)
                ix = ixv.astype(jnp.int32)[0, 0]
                idx_ref[j] = ix
                blk = xn_ref[pl.ds(pl.multiple_of((ix // 16) * 16, 16), 16), :].astype(F32)
                pick = lax.broadcasted_iota(jnp.int32, (16, D), 0) == (ixv.astype(jnp.int32) & 15)
                xs_ref[j:j + 1, :] = jnp.sum(jnp.where(pick, blk, 0.0), axis=0, keepdims=True)
                rs_ref[j:j + 1, :] = jnp.broadcast_to(rsel, (1, 128))

    def gate(r0, n):
        hb = 0.5 * xn_ref[pl.ds(r0, n), :].astype(F32)
        g_ref[pl.ds(r0, n), :] = hb + hb * jnp.tanh(hb)

    class Ffn:
        def __init__(self):
            self.xs = xs_ref[...].astype(BF)
            self.acc = {}
            self.up = [(w, i, k) for i in range(len(F_TILES)) for w in (0, 1) for k in range(D // 128)]
            self.down = [(i, k) for k in range(D // 128) for i in range(len(F_TILES))]
            self.hid = None

        def add(self, key, d):
            self.acc[key] = d if key not in self.acc else self.acc[key] + d

        def run_up(self, n):
            for _ in range(min(n, len(self.up))):
                w, i, k = self.up.pop(0)
                f0, fn = F_TILES[i]
                wt = (wg_ref, wu_ref)[w][f0:f0 + fn, k * 128:(k + 1) * 128]
                self.add((w, i), lax.dot_general(self.xs[:, k * 128:(k + 1) * 128], wt, NT,
                                                 preferred_element_type=F32))

        def run_down(self, n):
            if self.hid is None:
                self.run_up(len(self.up))
                self.hid = []
                for i in range(len(F_TILES)):
                    g = _rb(self.acc[(0, i)])
                    g = _rb(g * jax.nn.sigmoid(g))
                    self.hid.append((g * _rb(self.acc[(1, i)])).astype(BF))
            for _ in range(min(n, len(self.down))):
                i, k = self.down.pop(0)
                f0, fn = F_TILES[i]
                self.add((2, k), jnp.dot(self.hid[i], wd_ref[f0:f0 + fn, k * 128:(k + 1) * 128],
                                         preferred_element_type=F32))

        def finish(self):
            self.run_down(len(self.down))
            y = _rb(jnp.concatenate([self.acc[(2, k)] for k in range(D // 128)], axis=1))
            y = _rb(y * _rb(jax.nn.sigmoid(rs_ref[:, 0:1])))
            b = _rb(xs_ref[...] + y)
            gs = b * jax.nn.sigmoid(b)
            for j in range(C):
                g_ref[pl.ds(idx_ref[j], 1), :] = gs[j:j + 1, :]

    def qproj(i, h, split=1, rows=TQ):
        n = rows // split
        parts = [(jnp.dot(xn_ref[r0:r0 + n, :], wq_ref[h], preferred_element_type=F32) * QSCALE).astype(BF)
                 for r0 in range(i * rows, (i + 1) * rows, n)]
        return parts[0] if split == 1 else jnp.concatenate(parts, axis=0)

    def transpose_v(cx, h):
        vt_ref[pl.ds(cx.z1, DH // 2), :] = pltpu.bitcast(v_ref[h].T, U32)

    def qk(cx, n, h, q, transposed=False, between=None, ticks=None):
        sv = s_refs[n % 2].at[pl.ds(cx.z1, NG * SP), :]
        ns = 1 if between is None else FSL
        sl = S // ns
        m = None
        for j in range(ns):
            kj = k_ref[h, j * sl:(j + 1) * sl, :]
            if transposed:
                sT = jnp.dot(kj, q, preferred_element_type=F32)
            else:
                sT = lax.dot_general(kj, q, NT, preferred_element_type=F32)
            for g in range(NG):
                sv[g * SP + j * sl:g * SP + (j + 1) * sl, :] = sT[:, g * 128:(g + 1) * 128]
            mj = jnp.max(jnp.max(sT.reshape(sl // 128, 16, 8, TQ), axis=1), axis=0)
            m = mj if m is None else jnp.maximum(m, mj)
            if between is not None and j < ns - 1:
                between(j)
        if ticks is not None:
            fn, count, span = ticks
            for i in range(count):
                r = (i * span // count) // 8 * 8
                fn(sT[r:r + 8, 0:128])
        return jnp.broadcast_to(jnp.max(m, axis=0, keepdims=True), (8, TQ))

    def pv(cx, n, m, hooks=None, groups=tuple(range(NG)), buf=0):
        sv = s_refs[n % 2].at[pl.ds(cx.z2, NG * SP), :]
        vv = vt_ref.at[pl.ds(cx.z2, DH // 2), :]
        otv = ot_refs[buf].at[pl.ds(cx.z1, NG * DH), :]
        lv = l_refs[buf].at[pl.ds(cx.z1, NG * 8), :]
        for g in groups:
            l8 = None
            oT = None
            for c in range(NCH):
                mc = m[:, g * 128:(g + 1) * 128]
                if len(cx.hist) >= PV_DIST:
                    mc = dep(mc, cx.tok(cx.hist[-PV_DIST]))
                if hooks and g * NCH + c in hooks:
                    mc = dep(mc, hooks[g * NCH + c])
                ps = []
                for t in range(c * CT, (c + 1) * CT):
                    r0 = g * SP + t * 128
                    p = jnp.exp2(sv[r0:r0 + 128, :] - jnp.concatenate([mc] * 16, axis=0))
                    lt = None
                    for j in reversed(range(16)):
                        pj = p[j * 8:(j + 1) * 8, :]
                        lt = pj if lt is None else lt + pj
                    l8 = lt if l8 is None else l8 + lt
                    ps.append(p)
                vT = pltpu.bitcast(vv[:, c * CT * 128:(c + 1) * CT * 128], BF)
                part = jnp.dot(vT, jnp.concatenate(ps, axis=0).astype(BF), preferred_element_type=F32)
                cx.hist.append(part[0:8, :])
                oT = part if oT is None else oT + part
            otv[g * DH:(g + 1) * DH, :] = oT
            lv[g * 8:(g + 1) * 8, :] = l8

    def load_o(cx, groups=tuple(range(NG)), buf=0):
        otv = ot_refs[buf].at[pl.ds(cx.z2, NG * DH), :]
        lv = l_refs[buf].at[pl.ds(cx.z2, NG * 8), :]
        parts = []
        for g in groups:
            l = jnp.sum(lv[g * 8:(g + 1) * 8, :], axis=0, keepdims=True)
            parts.append((otv[g * DH:(g + 1) * DH, :] * (1.0 / l)).T.astype(BF))
        return parts[0] if len(parts) == 1 else jnp.concatenate(parts, axis=0)

    def oproj(cx, r0, h, o, mode, paces_pv=True):
        r1 = r0 + o.shape[0]
        d = jnp.dot(o, wo_ref[h], preferred_element_type=F32)
        if mode == 'set':
            acc_ref[r0:r1, :] = d
        elif mode == 'add':
            acc_ref[r0:r1, :] += d
        else:
            s = acc_ref[r0:r1, :] + d
            out_ref[r0:r1, :] = (x_ref[r0:r1, :].astype(F32) + s * g_ref[r0:r1, :]).astype(BF)
        if paces_pv:
            for r in (128, 256, 384):
                cx.hist.append(d[r:r + 8, 0:128])

    def store_qt(cx, q):
        qn_ref[...] = pltpu.bitcast(q.T, U32)
        return cx.memtok(qn_ref)

    cp_x(0, SEM_A, TQ // 2).start()
    cp_wq(0, SEM_A).start()
    cp_x(1, SEM_E, TQ // 2).start()
    cp_k(0, SEM_B).start()
    cp_x(1, SEM_B).start()
    cp_v(0, SEM_C).start()
    cp_x(2, SEM_D).start()
    cp_x(3, SEM_D).start()
    cp_wo(0, SEM_D).start()
    cp_wq(1, SEM_D).start()
    cp_wr().start()
    z_ref[0] = 0
    z_ref[1] = 0
    acc_ref[S - TQ:, :] = jnp.zeros((TQ, D), F32)

    def hide(i, c):
        z_ref[1] = z_ref[0] * i
        z_ref[0] = z_ref[1] * i
        return c

    lax.fori_loop(0, 2, hide, 0)
    cx = Ctx()
    cp_wq(0, SEM_A).wait()
    halves = []
    for c, s in enumerate((SEM_A, SEM_E)):
        cp_x(c, s, TQ // 2).wait()
        ln = LayerNorm(cx, c * (TQ // 2), 32, 0, 0, TQ // 2)
        for _ in range(ln.steps):
            ln.step()
        halves.append(qproj(c, 0, split=4, rows=TQ // 2))
    q = jnp.concatenate(halves, axis=0)
    cp_k(0, SEM_B).wait()
    cp_x(1, SEM_B).wait()
    start_head(1)

    ln = LayerNorm(cx, TQ, 8, 4, 10)
    ln.step()
    m = qk(cx, 0, 0, q, ticks=(ln.step, ln.steps - 1, 2000))
    cp_v(0, SEM_C).wait()
    transpose_v(cx, 0)
    q = qproj(1, 0, split=4)
    pv(cx, 0, m)
    cp_x(2, SEM_D).wait()
    cp_x(3, SEM_D).wait()
    cp_wo(0, SEM_D).wait()
    cp_wq(1, SEM_D).wait()
    cp_wr().wait()
    wrf_ref[...] = jnp.broadcast_to(wr_ref[...].astype(F32).reshape(1, D), (8, D))
    for c in cp_ffn():
        c.start()
    for n in range(1, NB - 1):
        ln = LayerNorm(cx, (n + 1) * TQ, 8, 4, 14)
        m = qk(cx, n, 0, q, ticks=(ln.step, ln.steps, 2040))
        q = qproj(n + 1, 0)
        oproj(cx, (n - 1) * TQ, 0, load_o(cx), 'set')
        pv(cx, n, m)
    router = Router(cx, 128)
    m = qk(cx, NB - 1, 0, q, ticks=(router.step, router.steps, 2040))
    router.top_k()
    gate((H - 2) * GROWS, S - (H - 2) * GROWS)
    q = qproj(0, 1)
    oproj(cx, (NB - 2) * TQ, 0, load_o(cx), 'set')
    qt_done = store_qt(cx, q)
    pv(cx, NB - 1, m, {10: qt_done | cx.zvec, 11: cx.memtok(xs_ref) | cx.memtok(rs_ref)})

    def body(it, carry):
        h = 1 + it
        wait_head(h)
        start_head(h + 1)
        cx = Ctx()
        transpose_v(cx, h)
        gate(pl.multiple_of(it * GROWS, GROWS), GROWS)
        q = pltpu.bitcast(qn_ref[...], BF)
        for n in range(NB):
            m = qk(cx, n, h, q, transposed=n == 0)
            q = qproj((n + 1) % NB, h + (n + 1) // NB)
            oproj(cx, (n - 1) % NB * TQ, h - (n == 0), load_o(cx), 'add')
            pv(cx, n, m, {4: store_qt(cx, q)} if n == NB - 1 else None)
        return carry

    lax.fori_loop(0, H - 2, body, 0)

    h = H - 1
    wait_head(h)
    for c in cp_ffn():
        c.wait()
    cx = Ctx()
    transpose_v(cx, h)
    ffn = Ffn()

    def spread(run, total):
        return lambda j: run((total * (j + 1)) // (FSL - 1) - (total * j) // (FSL - 1))

    def next_qt(i):
        done = store_qt(cx, qproj(i, h))
        return pltpu.bitcast(qn_ref[pl.ds(cx.z1, DH // 2), :], BF), {8: done}

    q = pltpu.bitcast(qn_ref[...], BF)
    m = qk(cx, 0, h, q, transposed=True, between=spread(ffn.run_up, 60))
    ffn.run_up(4)
    q, hooks = next_qt(1)
    ffn.run_up(4)
    oproj(cx, S - TQ, h - 1, load_o(cx), 'add')
    pv(cx, 0, m, hooks)
    ffn.run_up(4)
    m = qk(cx, 1, h, q, transposed=True, between=spread(ffn.run_up, len(ffn.up) - 4))
    ffn.run_up(4)
    q, hooks = next_qt(2)
    pv(cx, 1, m, hooks, buf=1)
    ffn.run_down(4)
    m = qk(cx, 2, h, q, transposed=True, between=spread(ffn.run_down, len(ffn.down) - 6))
    ffn.finish()
    q = qproj(3, h)
    oproj(cx, 0, h, load_o(cx), 'out', paces_pv=False)
    cp_out(0).start()
    oproj(cx, TQ, h, load_o(cx, buf=1), 'out')
    cp_out(1).start()
    pv(cx, 2, m, {6: cx.memtok(out_ref)})
    m = qk(cx, 3, h, q)
    oproj(cx, 2 * TQ, h, load_o(cx), 'out')
    cp_out(2).start()
    stored = cx.memtok(out_ref)
    os = []

    def finish_group(g):
        oproj(cx, S - TQ + g * 128, h, os[g], 'out', paces_pv=False)
        cp_out(NB - 1 + g).start()

    for g in range(NG):
        pv(cx, NB - 1, m, {6: stored}, groups=(g,))
        os.append(load_o(cx, (g,)))
        if g in (1, 2):
            finish_group(g - 1)
    for g in range(2, NG):
        finish_group(g)
    for j in range(len(OUT_PIECES)):
        cp_out(j).wait()


@jax.jit
def pallas_recurrent_scan__mha_block_cached__moe_arch_mod__prompt_kernel(
    A_x: jax.Array,
    A_k_cache: jax.Array,
    A_v_cache: jax.Array,
    A_wq: jax.Array,
    A_wo: jax.Array,
    B_x: jax.Array,
    B_w_r: jax.Array,
    B_w_gate: jax.Array,
    B_w_up: jax.Array,
    B_w_down: jax.Array,
):
    hbm = pl.BlockSpec(memory_space=pl.ANY)
    out = pl.pallas_call(
        _kernel,
        in_specs=[hbm] * 9,
        out_specs=hbm,
        out_shape=jax.ShapeDtypeStruct((S, D), BF),
        scratch_shapes=[
            pltpu.VMEM((NG * SP, 128), F32),
            pltpu.VMEM((NG * SP, 128), F32),
            pltpu.VMEM((DH // 2, S), U32),
            pltpu.VMEM((NG * DH + 32, 128), F32),
            pltpu.VMEM((NG * DH, 128), F32),
            pltpu.VMEM((S, D), F32),
            pltpu.VMEM((DH // 2, TQ), U32),
            pltpu.VMEM((H, S, DH), BF),
            pltpu.VMEM((H, S, DH), BF),
            pltpu.VMEM((H, D, DH), BF),
            pltpu.VMEM((H, DH, D), BF),
            pltpu.VMEM((S + 64, D), BF),
            pltpu.VMEM((S, D), F32),
            pltpu.VMEM((S, D), BF),
            pltpu.VMEM((F, D), BF),
            pltpu.VMEM((F, D), BF),
            pltpu.VMEM((F, D), BF),
            pltpu.VMEM((S + 64, D), BF),
            pltpu.VMEM((NG * 8, 128), F32),
            pltpu.VMEM((NG * 8, 128), F32),
            pltpu.VMEM((C, D), F32),
            pltpu.VMEM((C, 128), F32),
            pltpu.VMEM((8, D), F32),
            pltpu.VMEM((D,), BF),
            pltpu.SMEM((2,), jnp.int32),
            pltpu.SMEM((C,), jnp.int32),
            pltpu.SemaphoreType.DMA((8,)),
        ],
        compiler_params=pltpu.CompilerParams(
            vmem_limit_bytes=126 * 1024 * 1024,
            internal_scratch_in_bytes=16 * 4096,
            disable_bounds_checks=True,
            disable_semaphore_checks=True,
        ),
    )(A_x.reshape(S, D), A_k_cache.reshape(H, S, DH), A_v_cache.reshape(H, S, DH), A_wq,
      A_wo.reshape(H, DH, D), B_w_r, B_w_gate.T, B_w_up.T, B_w_down)
    return out.reshape(1, S, D)
```
